```python
import jax
import jax.numpy as jnp

def _softmax(x, axis=-1):
    return jax.nn.softmax(x, axis=axis)
def _gelu(x):
    return jax.nn.gelu(x, approximate=True)
def _silu(x):
    return jax.nn.silu(x)
def _sigmoid(x):
    return jax.nn.sigmoid(x)
def _layernorm(x, axis=-1, eps=1e-5):
    m = jnp.mean(x, axis=axis, keepdims=True)
    v = jnp.var(x, axis=axis, keepdims=True)
    return (x - m) / jnp.sqrt(v + eps)
def _scatter_add(tgt, idx, src, axis=0):
    return tgt.at[idx].add(src)
def _segment_sum(src, seg, n):
    return jax.ops.segment_sum(src, seg, n)
class _Rng:
    def __init__(self, key):
        self._k = key
    def _next(self):
        self._k, sub = jax.random.split(self._k)
        return sub
    def normal(self, shape):
        return jax.random.normal(self._next(), shape, dtype=jnp.bfloat16)
    def randint(self, lo, hi, shape):
        return jax.random.randint(self._next(), shape, lo, hi, dtype=jnp.int32)
    def uniform(self, shape, lo=0.0, hi=1.0):
        return jax.random.uniform(self._next(), shape, jnp.bfloat16, lo, hi)
    def permutation(self, n):
        return jax.random.permutation(self._next(), n)


kernel_name = 'standalone__layernorm_linear__sampling'

def setup_inputs():
    _rng = _Rng(jax.random.key(int.from_bytes(__import__("os").urandom(4), "little")))
    _w = (lambda a: (lambda t: t.astype(jnp.bfloat16) if jnp.issubdtype(t.dtype, jnp.floating) else t)(jnp.asarray(a)))
    B, S, D = 1024, 32, 576
    return {
        "x": _w((lambda *s: _rng.normal(s) * 0.05)(B, S, D)),
        "g": _w((lambda *s: _rng.normal(s) * 0.05)(D) + 1.0),
        "b": _w((lambda *s: _rng.normal(s) * 0.05)(D)),
        "w": _w((lambda *s: _rng.normal(s) * 0.05)(D, D)),
    }

def reference(x, g, b, w):
    return (_layernorm(x, axis=-1) * g + b) @ w
```

```python
import jax
import jax.numpy as jnp
from jax import lax
import jax.experimental.pallas as pl
import jax.experimental.pallas.tpu as pltpu

EPS = 1e-5


def _kernel(x_ref, g_ref, b_ref, w_ref, o_ref, wt_ref, bias_ref):
    @pl.when(pl.program_id(0) == 0)
    def _():
        wt = w_ref[...].astype(jnp.float32).T
        g = g_ref[...].astype(jnp.float32)
        b = b_ref[...].astype(jnp.float32)
        wt_ref[...] = (wt * g).astype(jnp.bfloat16)
        bias = jnp.sum(wt * b, axis=1, keepdims=True)
        bias_ref[...] = jnp.broadcast_to(bias, bias_ref.shape)

    x = x_ref[0].astype(jnp.float32)
    d, tb = x.shape
    m = jnp.sum(x, axis=0, keepdims=True) * (1.0 / d)
    xc = x - m
    v = jnp.sum(xc * xc, axis=0, keepdims=True) * (1.0 / d)
    r = lax.rsqrt(v + EPS)
    xn = (xc * r).astype(jnp.bfloat16)
    acc = jnp.dot(wt_ref[...], xn, preferred_element_type=jnp.float32)
    bias = bias_ref[...]
    acc = acc + jnp.concatenate([bias] * (tb // 128), axis=1)
    o_ref[0] = acc.astype(o_ref.dtype)


@jax.jit
def pallas_standalone__layernorm_linear__sampling_kernel(
    x: jax.Array,
    g: jax.Array,
    b: jax.Array,
    w: jax.Array,
):
    B, S, D = x.shape
    xt = jnp.transpose(x, (1, 2, 0))
    out = pl.pallas_call(
        _kernel,
        grid=(S,),
        in_specs=[
            pl.BlockSpec((1, D, B), lambda i: (i, 0, 0)),
            pl.BlockSpec((1, D), lambda i: (0, 0)),
            pl.BlockSpec((1, D), lambda i: (0, 0)),
            pl.BlockSpec((D, D), lambda i: (0, 0)),
        ],
        out_specs=pl.BlockSpec((1, D, B), lambda i: (i, 0, 0)),
        out_shape=jax.ShapeDtypeStruct((S, D, B), x.dtype),
        scratch_shapes=[
            pltpu.VMEM((D, D), jnp.bfloat16),
            pltpu.VMEM((D, 128), jnp.float32),
        ],
        compiler_params=pltpu.CompilerParams(
            dimension_semantics=("arbitrary",),
            vmem_limit_bytes=64 * 1024 * 1024,
        ),
    )(xt, g.reshape(1, D), b.reshape(1, D), w)
    return jnp.transpose(out, (2, 0, 1))
```

```python
import jax
import jax.numpy as jnp
from jax import lax
import jax.experimental.pallas as pl
import jax.experimental.pallas.tpu as pltpu

EPS = 1e-5
D = 576
S = 32
B = 1024
H = D // 2
KH = 256
KR = 80
PW = 128
W2 = 2 * PW
NP = B // W2
F = 3
NB = 8
DEFER = 13
f32 = jnp.float32
bf16 = jnp.bfloat16
u32 = jnp.uint32


def _dup(z):
    return jnp.concatenate([z, z], axis=1)


def _stats(x, gates):
    ng = max(len(gates), 1)
    bounds = [round((D // 8) * k / ng) for k in range(ng + 1)]
    c = jnp.broadcast_to(x[0:1, :], (8, W2))
    a1 = a2 = None
    for k in range(ng):
        ck = c + _dup(gates[k]) if gates else c
        for i in range(bounds[k], bounds[k + 1]):
            v = x[i * 8:(i + 1) * 8] - ck
            a1 = v if a1 is None else a1 + v
            a2 = v * v if a2 is None else a2 + v * v
    a1 = jnp.sum(a1, axis=0, keepdims=True) * (1.0 / D)
    a2 = jnp.sum(a2, axis=0, keepdims=True) * (1.0 / D)
    m = c[0:1] + a1
    var = jnp.maximum(a2 - a1 * a1, 0.0)
    r = lax.rsqrt(var + EPS)
    return jnp.broadcast_to(m, (8, W2)), jnp.broadcast_to(r, (8, W2))


def _normalize(x, m, r):
    n = x.shape[0]
    return ((x.reshape(n // 8, 8, W2) - m[None]) * r[None]).reshape(n, W2)


def _events(v):
    return [v[r:r + 8, 0:PW] for r in (0, 72, 144, 216)]


def _kernel(x_hbm, g_hbm, b_hbm, w_hbm, o_hbm,
            xbuf, obuf, st_ref, hd_ref, g_ref, b_ref, w_ref, a_ref, ar_ref,
            zs, sin, sout):
    zs[0] = 0
    zs[1] = 0
    zs[2] = 0

    def cin(i):
        return pltpu.make_async_copy(x_hbm.at[i], xbuf.at[i], sin.at[i])

    pieces = [(0, 256), (256, 512), (512, 1024)]

    def cin0(k):
        c0, c1 = pieces[k]
        return pltpu.make_async_copy(
            x_hbm.at[0, :, c0:c1], xbuf.at[0, :, c0:c1], sin.at[S + k])

    def cout(i):
        return pltpu.make_async_copy(obuf.at[i], o_hbm.at[i], sout.at[0])

    def cout_part(i, p, r0=0, r1=D):
        return pltpu.make_async_copy(
            obuf.at[i, r0:r1, p * W2:(p + 1) * W2],
            o_hbm.at[i, r0:r1, p * W2:(p + 1) * W2], sout.at[0])

    cw = pltpu.make_async_copy(w_hbm, w_ref, sin.at[S + 3])
    cg = pltpu.make_async_copy(g_hbm, g_ref, sin.at[S + 4])
    cb = pltpu.make_async_copy(b_hbm, b_ref, sin.at[S + 5])
    cg.start()
    cb.start()
    cw.start()
    for k in range(len(pieces)):
        cin0(k).start()
    for i in range(1, S):
        cin(i).start()

    cg.wait()
    cb.wait()
    cw.wait()
    g = g_ref[...].astype(f32).reshape(1, D)
    w = w_ref[...]
    b16 = jnp.broadcast_to(b_ref[...].reshape(1, D), (16, D))
    bias = jnp.dot(b16, w, preferred_element_type=f32)[0:8]
    bh = bias.astype(bf16).astype(f32)
    bl = (bias - bh).astype(bf16).astype(f32)
    bl2 = bias - bh - bl
    row8 = lax.broadcasted_iota(jnp.int32, (8, D), 0)
    ext = jnp.where(row8 == 0, bh,
                    jnp.where(row8 == 1, bl, jnp.where(row8 == 2, bl2, 0.0)))
    wf = w.astype(f32)
    wr = jnp.concatenate([wf[2 * KH:], ext, jnp.zeros((56, D), f32)], axis=0)
    wg = wf[:2 * KH].T * g[:, :2 * KH]
    gr = jnp.concatenate([g[:, 2 * KH:], jnp.ones((1, 64), f32)], axis=1)
    a11, a12 = wg[0:H, 0:KH], wg[0:H, KH:]
    a21, a22 = wg[H:, 0:KH], wg[H:, KH:]
    aops = [a11 + a22, a21 + a22, a11, a22, a11 + a12, a21 - a11, a12 - a22]
    for i, o in enumerate(aops):
        a_ref[i * 144:(i + 1) * 144, :] = pltpu.bitcast(o.astype(bf16), u32)
    ar_ref[...] = pltpu.bitcast((wr.T * gr).astype(bf16), u32)

    def store_head(xh, m, r, gates):
        ng = max(len(gates), 1)
        bounds = [16 * round(16 * k / ng) for k in range(ng + 1)]
        for k in range(ng):
            r0, r1 = bounds[k], bounds[k + 1]
            if r0 == r1:
                continue
            mk = m + _dup(gates[k]) if gates else m
            top = _normalize(xh[r0:r1], mk, r)
            bot = _normalize(xh[KH + r0:KH + r1], mk, r)
            hd_ref[r0 // 2:r1 // 2, :] = pltpu.bitcast(
                (top[:, 0:PW] + bot[:, PW:]).astype(bf16), u32)
            hd_ref[128 + r0 // 2:128 + r1 // 2, :] = pltpu.bitcast(
                (bot[:, 0:PW] - top[:, 0:PW]).astype(bf16), u32)

    cin0(0).wait()
    x0 = xbuf[0, :, 0:W2].astype(f32)
    m0, r0 = _stats(x0, [])
    st_ref[0, 0:8, :] = m0
    st_ref[0, 8:16, :] = r0
    store_head(x0, m0, r0, [])

    def run(s, n, have, tasks, cuts, head_span):
        k1 = s + zs[0]
        k2 = s + zs[2]
        never = lax.broadcasted_iota(jnp.int32, (8, PW), 0) < zs[1]
        stats = {p: (st_ref[p, 0:8, :], st_ref[p, 8:16, :]) for p in have}
        h1 = pltpu.bitcast(hd_ref[0:128, :], bf16)
        h4 = pltpu.bitcast(hd_ref[128:256, :], bf16)
        row16 = lax.broadcasted_iota(jnp.int32, (16, W2), 0)
        ones = jnp.where(row16 < 3, 1.0, 0.0)
        events = []
        loaded = {}

        def gates(p0, p1):
            return [jnp.where(never, e, 0.0) for (pp, e) in events
                    if p0 < pp <= p1]

        def load(k, q):
            tq, cq = divmod(q, NP)
            return xbuf[jnp.minimum(k + tq, S - 1), :,
                        cq * W2:(cq + 1) * W2].astype(f32)

        def at(pos):
            if pos in cuts:
                cuts[pos]()
            for (q, p0, p1) in tasks:
                if p0 == pos:
                    loaded[q] = load(k1, q)
            for (q, p0, p1) in tasks:
                if p1 == pos:
                    stats[q] = _stats(loaded.pop(q), gates(p0, p1))
            if head_span and pos == head_span[1]:
                store_head(load(k2, n), *stats[n], gates(*head_span))

        for p in range(n):
            t, c = divmod(p, NP)
            c0 = c * W2
            at((p, -1))
            m, r = stats.pop(p)
            xn = _normalize(xbuf[s + t, :, c0:c0 + W2].astype(f32), m, r)
            b11, b12 = xn[0:KH, 0:PW], xn[0:KH, PW:]
            b21, b22 = xn[KH:2 * KH, 0:PW], xn[KH:2 * KH, PW:]
            ops = [b11 + b22, b11, b12 - b22, b21 - b11, b22, b11 + b12,
                   b21 + b22]
            ops = [o.astype(bf16) for o in ops]
            if p == 0:
                ops[0], ops[3] = h1, h4
            rr = jnp.concatenate([xn[2 * KH:], ones], axis=0).astype(bf16)
            dot_no = [0]

            def post(v, p=p, dot_no=dot_no):
                for e in _events(v):
                    events.append(((p, dot_no[0]), e))
                at((p, dot_no[0]))
                dot_no[0] += 1
                return v

            def prod(i, ops=ops, post=post):
                a = pltpu.bitcast(a_ref[(i - 1) * 144:i * 144, :], bf16)
                return post(jnp.dot(a, ops[i - 1], preferred_element_type=f32))

            def rem(half, rr=rr):
                ar = pltpu.bitcast(
                    ar_ref[half * 144:(half + 1) * 144, :], bf16)[:, :KR]
                return jnp.dot(ar, rr, preferred_element_type=f32)

            m1 = prod(1)
            m4 = prod(4)
            m5 = prod(5)
            m7 = prod(7)
            m3 = prod(3)
            rt = rem(0)
            c11 = m1 + m4 - m5 + m7 + rt[:, 0:PW]
            c12 = m5 + m3 + rt[:, PW:]
            obuf[s + t, 0:H, c0:c0 + W2] = jnp.concatenate(
                [c11, c12], axis=1).astype(bf16)
            post(rt)
            m2 = prod(2)
            m6 = prod(6)
            rb = rem(1)
            c21 = m4 + m2 + rb[:, 0:PW]
            c22 = m1 + m3 - m2 + m6 + rb[:, PW:]
            obuf[s + t, H:, c0:c0 + W2] = jnp.concatenate(
                [c21, c22], axis=1).astype(bf16)
            post(rb)
        for q in sorted(stats):
            m, r = stats[q]
            st_ref[q - n, 0:8, :] = m
            st_ref[q - n, 8:16, :] = r

    ca, cb_, cc, cd = (0, 7), (2, 5), (4, 5), (7, 6)
    cuts = {(0, -1): lambda: cin0(1).wait(),
            ca: lambda: cin0(2).wait(),
            cb_: lambda: cin(1).wait(),
            cc: lambda: cin(2).wait(),
            cd: lambda: (cin(3).wait(), cin(4).wait())}
    spans = [cd, (8, 2), (8, 6), (9, 2), (9, 6), (10, 2), (10, 6), (11, 2),
             (11, 6)]
    tasks = [(1, (0, -1), (0, 2)),
             (2, ca, (1, 4)), (3, (1, 4), cb_),
             (4, cb_, (3, 2)), (5, (3, 2), (3, 6)), (6, (3, 6), (4, 1)),
             (7, (4, 1), cc),
             (8, cc, (5, 4)), (9, (5, 4), (6, 2)), (10, (6, 2), (6, 8)),
             (11, (6, 8), cd)]
    tasks += [(12 + i, spans[i], spans[i + 1]) for i in range(8)]
    run(0, F * NP, [0], tasks, cuts, ((10, 8), (11, 6)))

    n_iter = (S - F - 1) // 2
    j_flush = -(-(DEFER - F) // 2)

    def body(j, carry):
        s = F + 2 * j

        def top():
            cin(s + 2).wait()

            @pl.when(s + 3 < S)
            def _():
                cin(jnp.minimum(s + 3, S - 1)).wait()

        def outs_a():
            @pl.when(j == j_flush)
            def _():
                for i in range(F + 2 * j_flush):
                    cout(i).start()

            @pl.when(j > j_flush)
            def _():
                cout(s - 1).start()

        def outs_b():
            @pl.when(j >= j_flush)
            def _():
                cout(s).start()

        tasks = [(NB + p, (p, -1), (p, 7)) for p in range(NB)]
        run(s, NB, list(range(NB)), tasks,
            {(0, -1): top, (0, 5): outs_a, (4, 5): outs_b}, ((5, 8), (6, 7)))
        return carry

    lax.fori_loop(0, n_iter, body, 0)

    s = S - 1
    cuts = {(0, 3): lambda: cout(s - 1).start(),
            (1, 3): lambda: cout_part(s, 0).start(),
            (2, 3): lambda: cout_part(s, 1).start(),
            (3, 3): lambda: cout_part(s, 2).start(),
            (3, 7): lambda: cout_part(s, 3, 0, H).start(),
            (3, 8): lambda: cout_part(s, 3, H, D).start()}
    run(s, NP, list(range(NP)), [], cuts, None)
    pltpu.make_async_copy(obuf, o_hbm, sout.at[0]).wait()


@jax.jit
def pallas_standalone__layernorm_linear__sampling_kernel(
    x: jax.Array,
    g: jax.Array,
    b: jax.Array,
    w: jax.Array,
):
    assert x.shape == (B, S, D) and w.shape == (D, D)
    xt = jnp.transpose(x, (1, 2, 0))
    out = pl.pallas_call(
        _kernel,
        in_specs=[pl.BlockSpec(memory_space=pl.ANY)] * 4,
        out_specs=pl.BlockSpec(memory_space=pl.ANY),
        out_shape=jax.ShapeDtypeStruct((S, D, B), x.dtype),
        scratch_shapes=[
            pltpu.VMEM((S, D, B), bf16),
            pltpu.VMEM((S, D, B), bf16),
            pltpu.VMEM((NB, 16, W2), f32),
            pltpu.VMEM((256, PW), u32),
            pltpu.VMEM((D,), bf16),
            pltpu.VMEM((D,), bf16),
            pltpu.VMEM((D, D), bf16),
            pltpu.VMEM((7 * H // 2, KH), u32),
            pltpu.VMEM((D // 2, 128), u32),
            pltpu.SMEM((4,), jnp.int32),
            pltpu.SemaphoreType.DMA((S + 6,)),
            pltpu.SemaphoreType.DMA((1,)),
        ],
        compiler_params=pltpu.CompilerParams(
            vmem_limit_bytes=100 * 1024 * 1024,
            disable_bounds_checks=True,
            disable_semaphore_checks=True,
        ),
    )(xt, g, b, w)
    return jnp.transpose(out, (2, 0, 1))
```

```python
import jax
import jax.numpy as jnp
from jax import lax
import jax.experimental.pallas as pl
import jax.experimental.pallas.tpu as pltpu

EPS = 1e-5
D = 576
S = 32
B = 1024
H = D // 2
Q = D // 4
KH = 256
KR = 80
PW = 128
W2 = 2 * PW
W4 = 4 * PW
NH = 10
DEFER = 13
NPER = 6
SG = 18
f32 = jnp.float32
bf16 = jnp.bfloat16
u32 = jnp.uint32
KS = "abcd"
SUB = {"a": (0, 0), "b": (0, 1), "c": (1, 1), "d": (1, 0)}
PERM = (3, 5, 6, 7)
BROWS = 25 * 64 + 80


def _sa(a11, a12, a21, a22):
    return {1: a11 + a22, 2: a21 + a22, 3: a11, 4: a22, 5: a11 + a12,
            6: a21 - a11, 7: a12 - a22}


def _sb(b11, b12, b21, b22):
    return {1: b11 + b22, 2: b11, 3: b12 - b22, 4: b21 - b11, 5: b22,
            6: b11 + b12, 7: b21 + b22}


def _bpos(i, j):
    n = (i - 1) * 7 + (j - 1)
    return (n // 2) * 64, (n % 2) * PW


def _rpos(ct):
    return 25 * 64 + (ct // 2) * 40, (ct % 2) * PW


_LV = [[0, 54, 89, 58, 261, 60, 89, 74, 318, 5, 53, 89, 56, 330, 68, 262],
       [149, 54, 89, 55, 263, 8, 53, 89, 73, 318, 60, 89, 56, 330, 65, 99],
       [313, 56, 89, 55, 263, 8, 53, 89, 73, 318, 60, 89, 56, 330, 65, 95],
       [8, 53, 89, 55, 263, 61, 89, 73, 318, 7, 53, 89, 56, 330, 61, 402]]
_LS = [[71, 23, 61, 48, 87, 27, 64, 58, 87, 74, 24, 61, 35, 35, 34, 20],
       [70, 24, 65, 54, 87, 74, 24, 62, 56, 87, 26, 61, 35, 35, 38, 16],
       [69, 25, 65, 53, 87, 74, 24, 62, 56, 87, 26, 61, 35, 34, 33, 21],
       [74, 23, 62, 50, 87, 27, 64, 58, 87, 74, 24, 61, 35, 34, 28, 35]]
_NCOST = []
for _k in range(8):
    _NCOST += [43, 51, 51, 29, 21, 51, 29] + ([32] if _k % 2 == 0 else [])


def _place(costs, weights, lo, hi):
    tot = sum(weights)
    ctot = sum(costs)
    cum = []
    a = 0.0
    for w in weights:
        cum += [a + w * e / NPER for e in range(NPER)]
        a += w
    out = []
    c = 0
    for x in costs:
        tgt = (lo + (hi - lo) * c / ctot) * tot
        out.append(max(k for k in range(len(cum)) if cum[k] <= tgt + 1e-9))
        c += x
    return out


def _weights(pat, steady):
    t, ts = (360, 85) if steady else (420, 110)
    free = [max(t - v, 0) for v in _LV[pat]]
    if not steady:
        wf = [f + 0.01 for f in free]
        return wf, wf
    wn = [min(f, max(ts - s, 0) * 5.2) + 0.01 for f, s in zip(free, _LS[pat])]
    sc = sum(_NCOST) / sum(wn)
    ws = [max(f - n * sc, 0) + 0.01 for f, n in zip(free, wn)]
    return wn, ws


def _stats_pair(x, gates):
    ng = max(len(gates), 1)
    bounds = [round((D // 8) * k / ng) for k in range(ng + 1)]
    c = jnp.broadcast_to(x[0:1, :], (8, W2))
    a1 = a2 = None
    for k in range(ng):
        ck = gates[k](c) if gates else c
        for i in range(bounds[k], bounds[k + 1]):
            v = x[i * 8:(i + 1) * 8] - ck
            a1 = v if a1 is None else a1 + v
            a2 = v * v if a2 is None else a2 + v * v
    a1 = jnp.sum(a1, axis=0, keepdims=True) * (1.0 / D)
    a2 = jnp.sum(a2, axis=0, keepdims=True) * (1.0 / D)
    m = c[0:1] + a1
    var = jnp.maximum(a2 - a1 * a1, 0.0)
    r = lax.rsqrt(var + EPS)
    return jnp.broadcast_to(m, (8, W2)), jnp.broadcast_to(r, (8, W2))


def _stats_quad(x, gates):
    h = len(gates) // 2
    ma, ra = _stats_pair(x[:, 0:W2], gates[:h])
    mb, rb = _stats_pair(x[:, W2:], gates[h:])
    return (jnp.concatenate([ma, mb], axis=1),
            jnp.concatenate([ra, rb], axis=1))


def _norm_quad(x, m, r, p_ref, gates):
    ms = [m[:, c * PW:(c + 1) * PW] for c in range(4)]
    rs = [r[:, c * PW:(c + 1) * PW] for c in range(4)]
    it = iter(gates)

    def gated_mean():
        g = next(it, None)
        return ms if g is None else [g(v) for v in ms]

    def gated(v):
        g = next(it, None)
        if g is None:
            return v
        v = dict(v)
        for q in ((0, 0), (1, 1)):
            v[q] = jnp.concatenate([g(v[q][0:8]), g(v[q][8:16])], axis=0)
        return v

    def store(r0, c0, v):
        p_ref[r0:r0 + 8, c0:c0 + PW] = pltpu.bitcast(v.astype(bf16), u32)

    def block(r0, ct, mg):
        xx = x[r0:r0 + 16, ct * PW:(ct + 1) * PW].reshape(2, 8, PW)
        return ((xx - mg[ct][None]) * rs[ct][None]).reshape(16, PW)

    def sub(k, kr, tc):
        mg = gated_mean()
        return {(a, b): block((2 * a + kr) * 128 + k * 16, 2 * b + tc, mg)
                for a in range(2) for b in range(2)}

    def emit(k, j, v):
        b1 = _sb(v[(0, 0)], v[(0, 1)], v[(1, 0)], v[(1, 1)])
        for i in range(1, 8):
            rr, cc = _bpos(i, j)
            store(rr + k * 8, cc, b1[i])

    def dsub(u, v):
        return {q: u[q] - v[q] for q in u}

    def dadd(u, v):
        return {q: u[q] + v[q] for q in u}

    for k in range(8):
        b11 = sub(k, 0, 0)
        emit(k, 2, b11)
        b12 = sub(k, 0, 1)
        emit(k, 6, dadd(b11, b12))
        b22 = sub(k, 1, 1)
        emit(k, 1, dadd(b11, b22))
        emit(k, 3, gated(dsub(b12, b22)))
        emit(k, 5, gated(b22))
        b21 = sub(k, 1, 0)
        emit(k, 4, dsub(b21, b11))
        emit(k, 7, gated(dadd(b21, b22)))
        if k % 2 == 0:
            mg = gated_mean()
            for ct in range(4):
                rr, cc = _rpos(ct)
                store(rr + (k // 2) * 8, cc,
                      block(2 * KH + (k // 2) * 16, ct, mg))


def _kernel(x_hbm, g_hbm, b_hbm, w_hbm, o_hbm, xbuf, obuf,
            p0, p1, p2, p3, u0, u1, u2, u3, u4,
            st_ref, g_ref, b_ref, w_ref, a_ref, ar_ref, zs, sin, sout):
    ps = [p0, p1, p2, p3]
    us = [u0, u1, u2, u3, u4]
    for i in range(4):
        zs[i] = 0

    def cin(i):
        return pltpu.make_async_copy(x_hbm.at[i], xbuf.at[i], sin.at[i])

    def cin_quad(n):
        t, c = divmod(n, 2)
        return pltpu.make_async_copy(
            x_hbm.at[t, :, c * W4:(c + 1) * W4],
            xbuf.at[t, :, c * W4:(c + 1) * W4], sin.at[S + 3 + n])

    def cout(sl, r0, r1, ct):
        idx = (sl, slice(r0, r1), slice(ct * PW, (ct + 1) * PW))
        pltpu.make_async_copy(
            obuf.at[idx], o_hbm.at[idx], sout.at[0]).start(priority=ct % 2)

    def cout_quad(t, c):
        for ct in range(4):
            cout(t, 0, D, 4 * c + ct)

    cw = pltpu.make_async_copy(w_hbm, w_ref, sin.at[S])
    cg = pltpu.make_async_copy(g_hbm, g_ref, sin.at[S + 1])
    cb = pltpu.make_async_copy(b_hbm, b_ref, sin.at[S + 2])
    cg.start()
    cb.start()
    cw.start()
    for n in range(NH):
        cin_quad(n).start()
    for i in range(NH // 2, S):
        cin(i).start()

    cg.wait()
    cb.wait()
    cw.wait()
    g = g_ref[...].astype(f32).reshape(1, D)
    w = w_ref[...]
    b16 = jnp.broadcast_to(b_ref[...].reshape(1, D), (16, D))
    bias = jnp.dot(b16, w, preferred_element_type=f32)[0:8]
    bh = bias.astype(bf16).astype(f32)
    bl = (bias - bh).astype(bf16).astype(f32)
    bl2 = bias - bh - bl
    row8 = lax.broadcasted_iota(jnp.int32, (8, D), 0)
    ext = jnp.where(row8 == 0, bh,
                    jnp.where(row8 == 1, bl, jnp.where(row8 == 2, bl2, 0.0)))
    wf = w.astype(f32)
    wr = jnp.concatenate([wf[2 * KH:], ext, jnp.zeros((56, D), f32)], axis=0)
    wg = wf[:2 * KH].T * g[:, :2 * KH]
    gr = jnp.concatenate([g[:, 2 * KH:], jnp.ones((1, 64), f32)], axis=1)
    a1 = _sa(wg[0:H, 0:KH], wg[0:H, KH:], wg[H:, 0:KH], wg[H:, KH:])
    for i in range(1, 8):
        top, bot = a1[i][0:Q], a1[i][Q:]
        if i in PERM:
            top, bot = bot, top
        a2 = _sa(top[:, 0:128], top[:, 128:], bot[:, 0:128], bot[:, 128:])
        for j in range(1, 8):
            n = (i - 1) * 7 + (j - 1)
            a_ref[(n // 2) * 72:(n // 2 + 1) * 72,
                  (n % 2) * PW:(n % 2 + 1) * PW] = pltpu.bitcast(
                      a2[j].astype(bf16), u32)
    arv = (wr.T * gr).astype(bf16)
    ar_ref[:, 0:PW] = pltpu.bitcast(arv[0:H], u32)
    ar_ref[:, PW:] = pltpu.bitcast(arv[H:], u32)

    row16 = lax.broadcasted_iota(jnp.int32, (16, W2), 0)
    ones = pltpu.bitcast(jnp.where(row16 < 3, 1.0, 0.0).astype(bf16), u32)
    for p_ref in ps:
        for ct in (0, 2):
            rr = _rpos(ct)[0] + 32
            p_ref[rr:rr + 8, :] = ones
    cin_quad(0).wait()
    x0 = xbuf[0, :, 0:W4].astype(f32)
    _norm_quad(x0, *_stats_quad(x0, []), ps[0], [])

    def mm_quad(sl, c, p_ref, pat, po, uo, hooks):
        c0 = c * W4
        rem = {}
        ev = []

        def hook(name):
            if name in hooks:
                hooks[name]()

        def rows(r, n):
            if po is None:
                return slice(r, r + n)
            return pl.ds(pl.multiple_of(po + r, 8), n)

        def add(a, b):
            return {k: a[k] + b[k] for k in KS}

        def sub(a, b):
            return {k: a[k] - b[k] for k in KS}

        def mark(v):
            for e in range(NPER):
                r0 = Q * e // NPER // 8 * 8
                ev.append(v[r0:r0 + 8])
            return v

        def dot(i, j):
            n = (i - 1) * 7 + (j - 1)
            a = pltpu.bitcast(a_ref[(n // 2) * 72:(n // 2 + 1) * 72,
                                    (n % 2) * PW:(n % 2 + 1) * PW], bf16)
            rr, cc = _bpos(i, j)
            bb = pltpu.bitcast(p_ref[rows(rr, 64), cc:cc + PW], bf16)
            return jnp.dot(a, bb, preferred_element_type=f32)

        def rp(name):
            half, cc = int(name[0]) - 1, int(name[1]) - 1
            hr, hc = SUB[name[2]]
            ar = pltpu.bitcast(ar_ref[hr * 72:(hr + 1) * 72,
                                      half * PW:(half + 1) * PW], bf16)
            rr, c1 = _rpos(2 * cc + hc)
            rc = pltpu.bitcast(p_ref[rows(rr, KR // 2), c1:c1 + PW], bf16)
            rem[name] = jnp.dot(ar[:, :KR], rc, preferred_element_type=f32)
            return rem[name]

        def rp_round(names):
            for n in names:
                v = rp(n)
            mark(v)

        def prod(i, x):
            m3 = mark(dot(i, 3))
            m5 = dot(i, 5)
            m1 = dot(i, 1)
            m7 = dot(i, 7)
            m4 = mark(dot(i, 4))
            m2 = dot(i, 2)
            m6 = dot(i, 6)
            rp(x)
            c12 = m3 + m5
            c21 = m2 + m4
            c11 = ((m1 + m7) - m5) + m4
            c22 = (m1 + m3) + (m6 - m2)
            if i in PERM:
                return {"a": c21, "b": c22, "c": c12, "d": c11}
            return {"a": c11, "b": c12, "c": c22, "d": c21}

        def out(name, val, plus, minus=()):
            half, cc = int(name[0]) - 1, int(name[1]) - 1
            for k in KS:
                if name + k not in rem:
                    rp(name + k)
            v = {k: val[k] + rem[name + k] for k in KS}
            for o in plus:
                v = add(v, o)
            for o in minus:
                v = sub(v, o)
            r0 = half * H
            cols = slice(c0 + cc * W2, c0 + (cc + 1) * W2)
            obuf[sl, r0:r0 + Q, cols] = jnp.concatenate(
                [v["a"], v["b"]], axis=1).astype(bf16)
            obuf[sl, r0 + Q:r0 + H, cols] = jnp.concatenate(
                [v["d"], v["c"]], axis=1).astype(bf16)

        def put(i, v):
            for n, k in enumerate(KS):
                us[i][(n // 2) * Q:(n // 2 + 1) * Q,
                      (n % 2) * PW:(n % 2 + 1) * PW] = v[k]

        def get(i):
            return {k: us[i][pl.ds(pl.multiple_of(uo + (n // 2) * Q, 8), Q),
                             (n % 2) * PW:(n % 2 + 1) * PW]
                    for n, k in enumerate(KS)}

        pre = [("12b", "12d", "21a", "21d"), ("12b", "12d", "21a"),
               ("12b", "12d"), ("12b", "12d", "21a", "21d", "22c")][pat]
        mid = [("11b", "11d", "22c", "22d"), ("21d", "11b", "11d", "22c"),
               ("21a", "21d", "11b", "11d"), ("11b", "11d", "22b", "22d")][pat]
        rp_round(pre)
        hook("pre")
        put(0, prod(3, "12c"))
        hook("m3")
        m5 = prod(5, "12a")
        out("12", m5, [get(0)])
        put(1, m5)
        if pat in (1, 2):
            rp_round(mid)
        put(2, prod(2, "21b"))
        hook("m2")
        m4 = prod(4, "21c")
        out("21", m4, [get(2)])
        put(3, sub(m4, get(1)))
        if pat in (0, 3):
            rp_round(mid)
        put(4, prod(1, "11c"))
        hook("m1")
        m7 = prod(7, "11a")
        out("11", m7, [get(3), get(4)])
        m6 = prod(6, "22a")
        hook("m6")
        out("22", m6, [get(0), get(4)], minus=[get(2)])
        hook("end")
        return ev

    def run(s, n0, slots, have_st, save_st):
        k1 = s + zs[0]
        k2 = s + zs[2]
        never = lax.broadcasted_iota(jnp.int32, (8, PW), 0) < zs[1]
        never2 = lax.broadcasted_iota(jnp.int32, (8, W2), 0) < zs[1]
        zero = zs[3]

        def xload(k, q):
            t, c = divmod(q, 2)
            return xbuf[jnp.minimum(k + t, S - 1), :,
                        c * W4:(c + 1) * W4].astype(f32)

        mr = {}
        if have_st is not None:
            mr[have_st] = (st_ref[0:8, :], st_ref[8:16, :])
        for p, slot in enumerate(slots):
            t, c = divmod(p, 2)
            pat = p % 4
            hooks = slot.get("hooks", {})
            ev = mm_quad(s + t, c, ps[(n0 + p) % 4], pat,
                         zero if slot.get("fresh") else None, zero, hooks)
            e0 = NPER if "pre" in hooks else 0
            wn, ws = _weights(pat, slot.get("steady", False))
            for (kind, q, lo, hi) in slot.get("tasks", []):
                if kind == "N":
                    gates = [
                        (lambda v, e=ev[max(i, e0)]: jnp.where(never, e, v))
                        for i in _place(_NCOST, wn, lo, hi)]
                    _norm_quad(xload(k2, q), *mr.pop(q), ps[(n0 + q) % 4],
                               gates)
                else:
                    gates = [
                        (lambda v, e=ev[max(i, e0)]: jnp.where(
                            never2, jnp.concatenate([e, e], axis=1), v))
                        for i in _place([1] * (2 * SG), ws, lo, hi)]
                    mr[q] = _stats_quad(xload(k1, q), gates)
        if save_st is not None:
            st_ref[0:8, :] = mr[save_st][0]
            st_ref[8:16, :] = mr[save_st][1]

    def wait_quads(*ns):
        return lambda: [cin_quad(n).wait() for n in ns]

    cin_quad(1).wait()
    run(0, 0, [
        dict(tasks=[("S", 1, 0, .38), ("N", 1, .38, .93)]),
        dict(fresh=True, hooks={"pre": wait_quads(2, 3)},
             tasks=[("S", 2, 0, .28), ("N", 2, .28, .72), ("S", 3, .72, 1)]),
        dict(fresh=True, hooks={"pre": wait_quads(4, 5)},
             tasks=[("N", 3, 0, .45), ("S", 4, .45, .72), ("S", 5, .72, 1)]),
        dict(fresh=True, hooks={"pre": wait_quads(6, 7)},
             tasks=[("N", 4, 0, .38), ("N", 5, .38, .76), ("S", 6, .76, 1)]),
        dict(fresh=True, hooks={"pre": wait_quads(8, 9)},
             tasks=[("N", 6, 0, .45), ("S", 7, .45, .72), ("S", 8, .72, 1)]),
        dict(fresh=True,
             tasks=[("N", 7, 0, .38), ("N", 8, .38, .76), ("S", 9, .76, 1)]),
    ], None, 9)

    j_flush = -(-(DEFER - 3) // 2)

    def body(j, carry):
        s = 3 + 2 * j
        cin(s + 2).wait()

        @pl.when(s + 3 < S)
        def _():
            cin(jnp.minimum(s + 3, S - 1)).wait()

        def write_prev(p):
            t, c = divmod(p - 1, 2)

            def f():
                if p == 0:
                    @pl.when(j == j_flush)
                    def _():
                        for ct in range(8):
                            cout(pl.ds(0, 3 + 2 * j_flush), 0, D, ct)

                @pl.when(j > j_flush if p == 0 else j >= j_flush)
                def _():
                    cout_quad(s + t, c)
            return f

        run(s, 2, [dict(fresh=(p == 3), steady=True,
                        hooks={"m3": write_prev(p)},
                        tasks=[("N", p + 3, 0, 1), ("S", p + 4, 0, 1)])
                   for p in range(4)], 3, 7)
        return carry

    lax.fori_loop(0, (S - 4) // 2, body, 0)

    s = S - 1

    def write_part(half, cc):
        return lambda: [cout(s, half * H, (half + 1) * H, 4 + 2 * cc + k)
                        for k in range(2)]

    run(s, 2, [dict(hooks={"m3": lambda: cout_quad(s - 1, 1)}),
               dict(hooks={"m3": lambda: cout_quad(s, 0),
                           "m2": write_part(0, 1), "m1": write_part(1, 0),
                           "m6": write_part(0, 0), "end": write_part(1, 1)})],
        None, None)
    pltpu.make_async_copy(obuf, o_hbm, sout.at[0]).wait()


@jax.jit
def pallas_standalone__layernorm_linear__sampling_kernel(
    x: jax.Array,
    g: jax.Array,
    b: jax.Array,
    w: jax.Array,
):
    assert x.shape == (B, S, D) and w.shape == (D, D)
    xt = jnp.transpose(x, (1, 2, 0))
    out = pl.pallas_call(
        _kernel,
        in_specs=[pl.BlockSpec(memory_space=pl.ANY)] * 4,
        out_specs=pl.BlockSpec(memory_space=pl.ANY),
        out_shape=jax.ShapeDtypeStruct((S, D, B), x.dtype),
        scratch_shapes=[
            pltpu.VMEM((S, D, B), bf16),
            pltpu.VMEM((S, D, B), bf16),
        ] + [pltpu.VMEM((BROWS, W2), u32)] * 4
        + [pltpu.VMEM((H, W2), f32)] * 5
        + [
            pltpu.VMEM((16, W4), f32),
            pltpu.VMEM((D,), bf16),
            pltpu.VMEM((D,), bf16),
            pltpu.VMEM((D, D), bf16),
            pltpu.VMEM((25 * 72, W2), u32),
            pltpu.VMEM((144, W2), u32),
            pltpu.SMEM((4,), jnp.int32),
            pltpu.SemaphoreType.DMA((S + 3 + NH,)),
            pltpu.SemaphoreType.DMA((1,)),
        ],
        compiler_params=pltpu.CompilerParams(
            vmem_limit_bytes=110 * 1024 * 1024,
            disable_bounds_checks=True,
            disable_semaphore_checks=True,
        ),
    )(xt, g, b, w)
    return jnp.transpose(out, (2, 0, 1))
```

```python
import jax
import jax.numpy as jnp
from jax import lax
import jax.experimental.pallas as pl
import jax.experimental.pallas.tpu as pltpu

EPS = 1e-5
D = 576
S = 32
B = 1024
H = D // 2
Q = D // 4
KH = 256
KR = 80
PW = 128
W2 = 2 * PW
W4 = 4 * PW
NH = 10
FQ = 8
DEFER = 14
NPER = 18
SG = 36
f32 = jnp.float32
bf16 = jnp.bfloat16
u32 = jnp.uint32
cat = jnp.concatenate
PERM = (3, 5, 6, 7)
RROW = 28 * 64
BROWS = RROW + 80


def _sa(a11, a12, a21, a22):
    return [a11 + a22, a21 + a22, a11, a22, a11 + a12, a21 - a11, a12 - a22]


def _sb(b11, b12, b21, b22):
    return [b11 + b22, b11, b12 - b22, b21 - b11, b22, b11 + b12, b21 + b22]


def _ppos(i, j):
    return ((j - 1) * 4 + (i - 1) // 2) * 64, ((i - 1) % 2) * PW


def _rpos(ct):
    return RROW + (ct // 2) * 40, (ct % 2) * PW


_VT = [53, 89, 57, 143, 142, 74, 105, 141, 197, 60, 89, 56, 179, 161, 28, 286,
       172, 125, 38, 140, 146, 73, 108, 70, 206, 105, 122, 38, 158, 198, 60,
       214, 213, 76, 88, 123, 160, 60, 89, 75, 178, 161, 74, 56, 189, 196, 44,
       191, 235, 77, 91, 54, 157, 115, 122, 56, 174, 166, 73, 74, 23, 240, 137,
       219, 233]
_ST = [26, 71, 49, 54, 60, 44, 47, 35, 54, 29, 71, 33, 20, 36, 46, 34, 58, 54,
       45, 58, 39, 42, 80, 61, 51, 50, 53, 28, 25, 36, 36, 34, 53, 43, 47, 34,
       54, 29, 71, 51, 54, 60, 44, 29, 26, 19, 28, 25, 20, 43, 71, 52, 47, 54,
       52, 47, 57, 41, 43, 54, 50, 34, 27, 24, 17]
_NCOST = []
for _k in range(8):
    _NCOST += [43, 51, 51, 29, 21, 51, 29] + ([32] if _k % 2 == 0 else [])

_FIRST_WAITS = {17: (2, 3), 40: (4, 5, 6), 79: (7, 8, 9, 10)}
_FIRST_TASKS = [
    ("S", 1, 0, 5.5), ("N", 1, 5.5, 15), ("S", 2, 17, 21), ("N", 2, 21, 30.5),
    ("S", 3, 21, 30), ("N", 3, 30.5, 40), ("S", 4, 40, 45), ("N", 4, 45, 56),
    ("S", 5, 45, 56), ("N", 5, 56, 67.5), ("S", 6, 56, 67),
    ("N", 6, 67.5, 79), ("S", 7, 79, 83), ("N", 7, 83, 95),
    ("S", 8, 83, 94.5), ("N", 8, 95, 106.5), ("S", 9, 94.5, 106),
    ("N", 9, 106.5, 118), ("S", 10, 106, 118), ("N", 10, 118, 130),
    ("S", 11, 118, 130)]


def _stats_pair(x, gates):
    ng = len(gates) if gates else 18
    n = D // 8 // ng
    c = jnp.broadcast_to(x[0:1, :], (8, W2))
    a1 = a2 = None
    for k in range(ng):
        ck = gates[k](c, 2) if gates else c
        v = x[k * n * 8:(k + 1) * n * 8] - cat([ck] * n, axis=0)
        sq = v * v
        if a1 is not None:
            v = cat([a1, v], axis=0)
            sq = cat([a2, sq], axis=0)
        a1 = jnp.sum(v.reshape(-1, 8, W2), axis=0)
        a2 = jnp.sum(sq.reshape(-1, 8, W2), axis=0)
    a1 = jnp.sum(a1, axis=0, keepdims=True) * (1.0 / D)
    a2 = jnp.sum(a2, axis=0, keepdims=True) * (1.0 / D)
    m = c[0:1] + a1
    var = jnp.maximum(a2 - a1 * a1, 0.0)
    r = lax.rsqrt(var + EPS)
    return jnp.broadcast_to(m, (8, W2)), jnp.broadcast_to(r, (8, W2))


def _stats_quad(x, gates):
    h = len(gates) // 2
    ma, ra = _stats_pair(x[:, 0:W2], gates[:h])
    mb, rb = _stats_pair(x[:, W2:], gates[h:])
    return cat([ma, mb], axis=1), cat([ra, rb], axis=1)


def _norm_quad(x, m, r, p_ref, gates):
    def tiles(v, tc):
        return cat([v[:, tc * PW:(tc + 1) * PW],
                    v[:, (tc + 2) * PW:(tc + 3) * PW]], axis=1)

    def wide(v):
        return cat([cat([v, v], axis=1)] * 2, axis=0)

    xt = [tiles(x, 0), tiles(x, 1)]
    mt = [tiles(m, 0), tiles(m, 1)]
    rt = [wide(tiles(r, 0)), wide(tiles(r, 1))]
    r16 = cat([r, r], axis=0)
    it = iter(gates)

    def sub(k, kr, tc):
        g = next(it, None)
        mg = mt[tc] if g is None else g(mt[tc], 2)
        r0 = kr * 128 + k * 16
        xb = cat([xt[tc][r0:r0 + 16], xt[tc][KH + r0:KH + r0 + 16]], axis=1)
        return (xb - wide(mg)) * rt[tc]

    def emit(k, j, v, gate=False):
        q = [v[:, i * PW:(i + 1) * PW] for i in range(4)]
        g = next(it, None) if gate else None
        if g is not None:
            q[0] = g(q[0], 0)
            q[3] = g(q[3], 0)
        ops = _sb(*q)
        for i0 in range(0, 7, 2):
            grp = ops[i0:i0 + 2]
            r0 = _ppos(i0 + 1, j)[0] + k * 8
            p_ref[r0:r0 + 8, 0:len(grp) * PW] = pltpu.bitcast(
                cat(grp, axis=1).astype(bf16), u32)

    for k in range(8):
        b11 = sub(k, 0, 0)
        emit(k, 2, b11)
        b12 = sub(k, 0, 1)
        emit(k, 6, b11 + b12)
        b22 = sub(k, 1, 1)
        emit(k, 1, b11 + b22)
        emit(k, 3, b12 - b22, True)
        emit(k, 5, b22, True)
        b21 = sub(k, 1, 0)
        emit(k, 4, b21 - b11)
        emit(k, 7, b21 + b22, True)
        if k % 2 == 0:
            g = next(it, None)
            mg = m if g is None else g(m, 4)
            r0 = 2 * KH + k * 8
            v = (x[r0:r0 + 16] - cat([mg, mg], axis=0)) * r16
            for c0 in (0, 2):
                r1 = _rpos(c0)[0] + k * 4
                p_ref[r1:r1 + 8, :] = pltpu.bitcast(
                    v[:, c0 * PW:(c0 + 2) * PW].astype(bf16), u32)


def _kernel(x_hbm, g_hbm, b_hbm, w_hbm, o_hbm, xbuf, obuf,
            p0, p1, p2, p3, u0, u1, u2, u3, u4,
            st_ref, g_ref, b_ref, w_ref, a_ref, ar_ref, zs, sin, sout):
    ps = [p0, p1, p2, p3]
    us = [u0, u1, u2, u3, u4]
    for i in range(4):
        zs[i] = 0

    def cin(i):
        return pltpu.make_async_copy(x_hbm.at[i], xbuf.at[i], sin.at[i])

    def cin_quad(n):
        t, c = divmod(n, 2)
        return pltpu.make_async_copy(
            x_hbm.at[t, :, c * W4:(c + 1) * W4],
            xbuf.at[t, :, c * W4:(c + 1) * W4], sin.at[S + 3 + n])

    def cout(sl, r0, r1, ct):
        idx = (sl, slice(r0, r1), slice(ct * PW, (ct + 1) * PW))
        pltpu.make_async_copy(
            obuf.at[idx], o_hbm.at[idx], sout.at[0]).start(priority=ct % 2)

    def cout_quad(t, c):
        for ct in range(4):
            cout(t, 0, D, 4 * c + ct)

    cw = pltpu.make_async_copy(w_hbm, w_ref, sin.at[S])
    cg = pltpu.make_async_copy(g_hbm, g_ref, sin.at[S + 1])
    cb = pltpu.make_async_copy(b_hbm, b_ref, sin.at[S + 2])
    cg.start()
    cb.start()
    cw.start()
    for n in range(NH):
        cin_quad(n).start()
    for i in range(NH // 2, S):
        cin(i).start()

    row16 = lax.broadcasted_iota(jnp.int32, (16, W2), 0)
    ones = pltpu.bitcast(jnp.where(row16 < 3, 1.0, 0.0).astype(bf16), u32)
    for p_ref in ps:
        for c0 in (0, 2):
            r1 = _rpos(c0)[0] + 32
            p_ref[r1:r1 + 8, :] = ones

    cg.wait()
    cb.wait()
    cw.wait()
    g = g_ref[...].astype(f32).reshape(1, D)
    w = w_ref[...]
    b16 = jnp.broadcast_to(b_ref[...].reshape(1, D), (16, D))
    bias = jnp.dot(b16, w, preferred_element_type=f32)[0:8]
    bh = bias.astype(bf16).astype(f32)
    bl = (bias - bh).astype(bf16).astype(f32)
    bl2 = bias - bh - bl
    row8 = lax.broadcasted_iota(jnp.int32, (8, D), 0)
    ext = jnp.where(row8 == 0, bh,
                    jnp.where(row8 == 1, bl, jnp.where(row8 == 2, bl2, 0.0)))
    wf = w.astype(f32)
    wr = cat([wf[2 * KH:], ext, jnp.zeros((56, D), f32)], axis=0)
    wg = wf[:2 * KH].T * g[:, :2 * KH]
    gr = cat([g[:, 2 * KH:], jnp.ones((1, 64), f32)], axis=1)
    a1 = _sa(wg[0:H, 0:KH], wg[0:H, KH:], wg[H:, 0:KH], wg[H:, KH:])
    for i in range(1, 8):
        top, bot = a1[i - 1][0:Q], a1[i - 1][Q:]
        if i in PERM:
            top, bot = bot, top
        a2 = _sa(top[:, 0:128], top[:, 128:], bot[:, 0:128], bot[:, 128:])
        a_ref[:, (i - 1) * PW:i * PW] = pltpu.bitcast(
            cat(a2, axis=0).astype(bf16), u32)
    arv = (wr.T * gr).astype(bf16)
    ar_ref[:, 0:PW] = pltpu.bitcast(arv[0:H], u32)
    ar_ref[:, PW:] = pltpu.bitcast(arv[H:], u32)

    cin_quad(0).wait()
    _norm_quad(xbuf[zs[2], :, 0:W4].astype(f32),
               *_stats_quad(xbuf[zs[0], :, 0:W4].astype(f32), []), ps[0], [])

    def run(s, nq, fresh, waits, tasks, hooks, have_st, save_st, bubble):
        k1 = s + zs[0]
        k2 = s + zs[2]
        never = {n: lax.broadcasted_iota(
            jnp.int32, (8, n * PW) if n else (16, PW), 0) < zs[1]
                 for n in (0, 2, 4)}
        zero = pl.multiple_of(zs[3], 8)
        nr = -(-65 * nq // 4)
        free = [max(420 - _VT[r % 65], 0) for r in range(nr)]
        wn = [min(free[r], max(110 - _ST[r % 65], 0) * 5.2) + 0.01
              for r in range(nr)]
        sc = sum(_NCOST) * nr / 16.25 / sum(wn)
        ws = [max(free[r] - wn[r] * sc, 0) + 0.01 for r in range(nr)]

        def xload(k, q):
            t, c = divmod(q, 2)
            return xbuf[jnp.minimum(k + t, S - 1), :,
                        c * W4:(c + 1) * W4].astype(f32)

        def make_gate(e):
            if e is None:
                return lambda v, n: v

            def gate(v, n):
                z = e[0][e[1]:e[1] + 8]
                z = cat([z] * n, axis=1) if n else cat([z, z], axis=0)
                return lax.select(never[n], z, v)
            return gate

        mr = {}
        if have_st is not None:
            mr[have_st] = (st_ref[0:8, :], st_ref[8:16, :])
        first = {}
        todo = list(tasks)

        def flush(now):
            for task in [t for t in todo if t[3] <= now + 1e-9]:
                todo.remove(task)
                kind, q, t0, t1 = task
                wt = wn if kind == "N" else ws
                cand = []
                a = 0.0
                if t0 == 0 or t0 in waits:
                    cand.append((0.0, None))
                    a += bubble[kind]
                for r in range(int(t0), nr):
                    for e in range(NPER):
                        if t0 - 1e-9 <= r + e / NPER < t1 - 1e-9:
                            cand.append(
                                (a, (first[r], Q * e // NPER // 8 * 8)))
                            a += wt[r] / NPER
                costs = _NCOST if kind == "N" else [1] * (2 * SG)
                done = 0
                gates = []
                for x in costs:
                    tgt = a * done / sum(costs)
                    gates.append(make_gate(
                        [e for (c, e) in cand if c <= tgt + 1e-9][-1]))
                    done += x
                if kind == "N":
                    _norm_quad(xload(k2, q), *mr.pop(q), ps[q % 4], gates)
                else:
                    mr[q] = _stats_quad(xload(k1, q), gates)

        count = [0]

        def mxu(lhs, rhs):
            r, o = divmod(count[0], 4)
            if o == 0 and r in waits:
                flush(r)
                waits[r]()
            v = jnp.dot(lhs(), rhs(), preferred_element_type=f32)
            if o == 0:
                first[r] = v
            count[0] += 1
            return v

        def get(i):
            return us[i][pl.ds(zero, H), :]

        def quad(p):
            sl = s + p // 2
            c0 = (p % 2) * W4
            p_ref = ps[p % 4]
            if p in fresh:
                p_ref = p_ref.at[pl.ds(zero, BROWS), :]

            def hook(name):
                if (p, name) in hooks:
                    hooks[(p, name)]()

            def dot(i, j):
                r1, c1 = _ppos(i, j)
                return mxu(
                    lambda: pltpu.bitcast(
                        a_ref[(j - 1) * 72:j * 72, (i - 1) * PW:i * PW], bf16),
                    lambda: pltpu.bitcast(
                        p_ref[r1:r1 + 64, c1:c1 + PW], bf16))

            def rem(half, cc, hr, hc):
                r1, c1 = _rpos(2 * cc + hc)
                return mxu(
                    lambda: pltpu.bitcast(
                        ar_ref[hr * 72:(hr + 1) * 72,
                               half * PW:(half + 1) * PW], bf16)[:, :KR],
                    lambda: pltpu.bitcast(
                        p_ref[r1:r1 + 40, c1:c1 + PW], bf16))

            def prod(i, o=None):
                sw = 1 if i in PERM else 0

                def rm(hr, hc):
                    return rem(o[0], o[1], hr ^ sw, hc) if o else None

                def blk(c11, c12, c21, c22):
                    rows = [cat([c11, c12], axis=1), cat([c21, c22], axis=1)]
                    return cat(rows[::-1] if sw else rows, axis=0)

                m3 = dot(i, 3)
                m5 = dot(i, 5)
                r12 = rm(0, 1)
                m1 = dot(i, 1)
                m7 = dot(i, 7)
                m4 = dot(i, 4)
                r11 = rm(0, 0)
                m2 = dot(i, 2)
                r21 = rm(1, 0)
                m6 = dot(i, 6)
                r22 = rm(1, 1)
                c12 = m3 + m5
                c21 = m2 + m4
                c11 = ((m1 + m7) - m5) + m4
                c22 = (m1 + m3) + (m6 - m2)
                return (blk(c11, c12, c21, c22),
                        blk(r11, r12, r21, r22) if o else None)

            def out(i, o, plus, minus=()):
                val, v = prod(i, o)
                if o == (1, 1):
                    hook("m6")
                v = val + v
                for u in plus:
                    v = v + get(u)
                for u in minus:
                    v = v - get(u)
                obuf[sl, o[0] * H:(o[0] + 1) * H,
                     c0 + o[1] * W2:c0 + (o[1] + 1) * W2] = v.astype(bf16)
                return val

            us[0][...] = prod(3)[0]
            hook("m3")
            us[1][...] = out(5, (0, 1), [0])
            us[2][...] = prod(2)[0]
            hook("m2")
            m4 = out(4, (1, 0), [2])
            us[3][...] = m4 - get(1)
            us[4][...] = prod(1)[0]
            hook("m1")
            out(7, (0, 0), [3, 4])
            out(6, (1, 1), [0, 4], [2])
            hook("end")

        for p in range(nq):
            flush(-(-count[0] // 4))
            quad(p)
        flush(nr)
        if save_st is not None:
            st_ref[0:8, :] = mr[save_st][0]
            st_ref[8:16, :] = mr[save_st][1]

    def wait_quads(ns):
        return lambda: [(cin_quad(n) if n < NH else cin(n // 2)).wait()
                        for n in ns]

    cin_quad(1).wait()
    run(0, FQ, range(1, FQ),
        {r: wait_quads(ns) for r, ns in _FIRST_WAITS.items()}, _FIRST_TASKS,
        {}, None, FQ + 3, {"N": 150, "S": 300})

    f = FQ // 2
    j_flush = (DEFER - f) // 2
    bnd = [0, 17, 33, 49, 65]
    no_bubble = {"N": 0.01, "S": 0.01}

    def body(j, carry):
        s = f + 2 * j
        cin(s + 2).wait()
        cin(s + 3).wait()

        def write_prev(p):
            def fn():
                if p == 0:
                    @pl.when(j == j_flush)
                    def _():
                        for ct in range(8):
                            cout(pl.ds(0, DEFER), 0, D, ct)

                @pl.when(j > j_flush if p == 0 else j >= j_flush)
                def _():
                    cout_quad(s + (p - 1) // 2, (p - 1) % 2)
            return fn

        tasks = []
        for p in range(4):
            tasks += [("N", p + 3, bnd[p], bnd[p + 1]),
                      ("S", p + 4, bnd[p], bnd[p + 1])]
        run(s, 4, (3,), {}, tasks,
            {(p, "m3"): write_prev(p) for p in range(4)}, 3, 7, no_bubble)
        return carry

    lax.fori_loop(0, (S - 2 - f) // 2, body, 0)

    s = S - 2

    def write_part(half, cc):
        return lambda: [cout(S - 1, half * H, (half + 1) * H, 4 + 2 * cc + k)
                        for k in range(2)]

    hooks = {(p, "m3"): (lambda p=p: cout_quad(s + (p - 1) // 2, (p - 1) % 2))
             for p in range(4)}
    hooks.update({(3, "m2"): write_part(0, 1), (3, "m1"): write_part(1, 0),
                  (3, "m6"): write_part(0, 0), (3, "end"): write_part(1, 1)})
    run(s, 4, (3,), {}, [("N", 3, 0, 33)], hooks, 3, None, no_bubble)
    pltpu.make_async_copy(obuf, o_hbm, sout.at[0]).wait()


@jax.jit
def pallas_standalone__layernorm_linear__sampling_kernel(
    x: jax.Array,
    g: jax.Array,
    b: jax.Array,
    w: jax.Array,
):
    assert x.shape == (B, S, D) and w.shape == (D, D)
    xt = jnp.transpose(x, (1, 2, 0))
    out = pl.pallas_call(
        _kernel,
        in_specs=[pl.BlockSpec(memory_space=pl.ANY)] * 4,
        out_specs=pl.BlockSpec(memory_space=pl.ANY),
        out_shape=jax.ShapeDtypeStruct((S, D, B), x.dtype),
        scratch_shapes=[
            pltpu.VMEM((S, D, B), bf16),
            pltpu.VMEM((S, D, B), bf16),
        ] + [pltpu.VMEM((BROWS, W2), u32)] * 4
        + [pltpu.VMEM((H, W2), f32)] * 5
        + [
            pltpu.VMEM((16, W4), f32),
            pltpu.VMEM((D,), bf16),
            pltpu.VMEM((D,), bf16),
            pltpu.VMEM((D, D), bf16),
            pltpu.VMEM((7 * 72, 7 * PW), u32),
            pltpu.VMEM((144, W2), u32),
            pltpu.SMEM((4,), jnp.int32),
            pltpu.SemaphoreType.DMA((S + 3 + NH,)),
            pltpu.SemaphoreType.DMA((1,)),
        ],
        compiler_params=pltpu.CompilerParams(
            vmem_limit_bytes=110 * 1024 * 1024,
            disable_bounds_checks=True,
            disable_semaphore_checks=True,
        ),
    )(xt, g, b, w)
    return jnp.transpose(out, (2, 0, 1))
```

```python
import jax
import jax.numpy as jnp
from jax import lax
import jax.experimental.pallas as pl
import jax.experimental.pallas.tpu as pltpu

EPS = 1e-5
D = 576
S = 32
B = 1024
H = D // 2
Q = D // 4
KH = 256
KR = 80
PW = 128
W2 = 2 * PW
W4 = 4 * PW
NH = 10
FQ = 8
DEFER = 14
NPER = 18
SG = 36
f32 = jnp.float32
bf16 = jnp.bfloat16
u32 = jnp.uint32
cat = jnp.concatenate
PERM = (3, 5, 6, 7)
RROW = 28 * 64
BROWS = RROW + 80


def _sa(a11, a12, a21, a22):
    return [a11 + a22, a21 + a22, a11, a22, a11 + a12, a21 - a11, a12 - a22]


def _sb(b11, b12, b21, b22):
    return [b11 + b22, b11, b12 - b22, b21 - b11, b22, b11 + b12, b21 + b22]


def _ppos(i, j):
    return ((j - 1) * 4 + (i - 1) // 2) * 64, ((i - 1) % 2) * PW


def _rpos(ct):
    return RROW + (ct // 2) * 40, (ct % 2) * PW


_VT = [53, 89, 57, 143, 142, 74, 105, 141, 197, 60, 89, 56, 179, 161, 28, 286,
       172, 125, 38, 140, 146, 73, 108, 70, 206, 105, 122, 38, 158, 198, 60,
       214, 213, 76, 88, 123, 160, 60, 89, 75, 178, 161, 74, 56, 189, 196, 44,
       191, 235, 77, 91, 54, 157, 115, 122, 56, 174, 166, 73, 74, 23, 240, 137,
       219, 233]
_ST = [26, 71, 49, 54, 60, 44, 47, 35, 54, 29, 71, 33, 20, 36, 46, 34, 58, 54,
       45, 58, 39, 42, 80, 61, 51, 50, 53, 28, 25, 36, 36, 34, 53, 43, 47, 34,
       54, 29, 71, 51, 54, 60, 44, 29, 26, 19, 28, 25, 20, 43, 71, 52, 47, 54,
       52, 47, 57, 41, 43, 54, 50, 34, 27, 24, 17]
_NCOST = []
for _k in range(8):
    _NCOST += [43, 51, 51, 29, 21, 51, 29] + ([32] if _k % 2 == 0 else [])

_FIRST_WAITS = {17: (2, 3), 40: (4, 5, 6), 79: (7, 8, 9, 10)}
_FIRST_TASKS = [
    ("S", 1, 0, 5.11),
    ("N", 1, 5.11, 14.23),
    ("S", 2, 17, 20.01),
    ("N", 2, 20.01, 31.2044),
    ("S", 3, 20.01, 30.7044),
    ("N", 3, 31.2044, 40),
    ("S", 4, 40, 44.47),
    ("N", 4, 44.47, 55.98),
    ("S", 5, 44.47, 55.98),
    ("N", 5, 55.98, 67.49),
    ("S", 6, 55.98, 67.49),
    ("N", 6, 67.49, 79),
    ("S", 7, 79, 84.4),
    ("N", 7, 84.4, 95.8),
    ("S", 8, 84.4, 95.8),
    ("N", 8, 95.8, 107.2),
    ("S", 9, 95.8, 107.2),
    ("N", 9, 107.2, 118.6),
    ("S", 10, 107.2, 118.6),
    ("N", 10, 118.6, 130.0),
    ("S", 11, 118.6, 130.0),
]


def _stats_pair(x, gates):
    ng = len(gates) if gates else 18
    n = D // 8 // ng
    c = jnp.broadcast_to(x[0:1, :], (8, W2))
    a1 = a2 = None
    for k in range(ng):
        ck = gates[k](c, 2) if gates else c
        v = x[k * n * 8:(k + 1) * n * 8] - cat([ck] * n, axis=0)
        sq = v * v
        if a1 is not None:
            v = cat([a1, v], axis=0)
            sq = cat([a2, sq], axis=0)
        a1 = jnp.sum(v.reshape(-1, 8, W2), axis=0)
        a2 = jnp.sum(sq.reshape(-1, 8, W2), axis=0)
    a1 = jnp.sum(a1, axis=0, keepdims=True) * (1.0 / D)
    a2 = jnp.sum(a2, axis=0, keepdims=True) * (1.0 / D)
    m = c[0:1] + a1
    var = jnp.maximum(a2 - a1 * a1, 0.0)
    r = lax.rsqrt(var + EPS)
    return jnp.broadcast_to(m, (8, W2)), jnp.broadcast_to(r, (8, W2))


def _stats_quad(x, gates):
    h = len(gates) // 2
    ma, ra = _stats_pair(x[:, 0:W2], gates[:h])
    mb, rb = _stats_pair(x[:, W2:], gates[h:])
    return cat([ma, mb], axis=1), cat([ra, rb], axis=1)


def _norm_quad(x, m, r, p_ref, gates):
    def tiles(v, tc):
        return cat([v[:, tc * PW:(tc + 1) * PW],
                    v[:, (tc + 2) * PW:(tc + 3) * PW]], axis=1)

    def wide(v):
        return cat([cat([v, v], axis=1)] * 2, axis=0)

    xt = [tiles(x, 0), tiles(x, 1)]
    mt = [tiles(m, 0), tiles(m, 1)]
    rt = [wide(tiles(r, 0)), wide(tiles(r, 1))]
    r16 = cat([r, r], axis=0)
    it = iter(gates)

    def sub(k, kr, tc):
        g = next(it, None)
        mg = mt[tc] if g is None else g(mt[tc], 2)
        r0 = kr * 128 + k * 16
        xb = cat([xt[tc][r0:r0 + 16], xt[tc][KH + r0:KH + r0 + 16]], axis=1)
        return (xb - wide(mg)) * rt[tc]

    def emit(k, j, v, gate=False):
        q = [v[:, i * PW:(i + 1) * PW] for i in range(4)]
        g = next(it, None) if gate else None
        if g is not None:
            q[0] = g(q[0], 0)
            q[3] = g(q[3], 0)
        ops = _sb(*q)
        for i0 in range(0, 7, 2):
            grp = ops[i0:i0 + 2]
            r0 = _ppos(i0 + 1, j)[0] + k * 8
            p_ref[r0:r0 + 8, 0:len(grp) * PW] = pltpu.bitcast(
                cat(grp, axis=1).astype(bf16), u32)

    for k in range(8):
        b11 = sub(k, 0, 0)
        emit(k, 2, b11)
        b12 = sub(k, 0, 1)
        emit(k, 6, b11 + b12)
        b22 = sub(k, 1, 1)
        emit(k, 1, b11 + b22)
        emit(k, 3, b12 - b22, True)
        emit(k, 5, b22, True)
        b21 = sub(k, 1, 0)
        emit(k, 4, b21 - b11)
        emit(k, 7, b21 + b22, True)
        if k % 2 == 0:
            g = next(it, None)
            mg = m if g is None else g(m, 4)
            r0 = 2 * KH + k * 8
            v = (x[r0:r0 + 16] - cat([mg, mg], axis=0)) * r16
            for c0 in (0, 2):
                r1 = _rpos(c0)[0] + k * 4
                p_ref[r1:r1 + 8, :] = pltpu.bitcast(
                    v[:, c0 * PW:(c0 + 2) * PW].astype(bf16), u32)


def _kernel(x_hbm, g_hbm, b_hbm, w_hbm, o_hbm, xbuf, obuf,
            p0, p1, p2, p3, u0, u1, u2, u3, u4,
            st_ref, g_ref, b_ref, w_ref, a_ref, ar_ref, zs, sin, sout):
    ps = [p0, p1, p2, p3]
    us = [u0, u1, u2, u3, u4]
    for i in range(4):
        zs[i] = 0

    def cin(i):
        return pltpu.make_async_copy(x_hbm.at[i], xbuf.at[i], sin.at[i])

    def cin_quad(n):
        t, c = divmod(n, 2)
        return pltpu.make_async_copy(
            x_hbm.at[t, :, c * W4:(c + 1) * W4],
            xbuf.at[t, :, c * W4:(c + 1) * W4], sin.at[S + 3 + n])

    def cout(sl, r0, r1, ct):
        idx = (sl, slice(r0, r1), slice(ct * PW, (ct + 1) * PW))
        pltpu.make_async_copy(
            obuf.at[idx], o_hbm.at[idx], sout.at[0]).start(priority=ct % 2)

    def cout_quad(t, c):
        for ct in range(4):
            cout(t, 0, D, 4 * c + ct)

    cw = pltpu.make_async_copy(w_hbm, w_ref, sin.at[S])
    cg = pltpu.make_async_copy(g_hbm, g_ref, sin.at[S + 1])
    cb = pltpu.make_async_copy(b_hbm, b_ref, sin.at[S + 2])
    cg.start()
    cb.start()
    cw.start()
    for n in range(NH):
        cin_quad(n).start()
    for i in range(NH // 2, S):
        cin(i).start()

    row16 = lax.broadcasted_iota(jnp.int32, (16, W2), 0)
    ones = pltpu.bitcast(jnp.where(row16 < 3, 1.0, 0.0).astype(bf16), u32)
    for p_ref in ps:
        for c0 in (0, 2):
            r1 = _rpos(c0)[0] + 32
            p_ref[r1:r1 + 8, :] = ones

    cg.wait()
    cb.wait()
    cw.wait()
    g = g_ref[...].astype(f32).reshape(1, D)
    w = w_ref[...]
    b16 = jnp.broadcast_to(b_ref[...].reshape(1, D), (16, D))
    bias = jnp.dot(b16, w, preferred_element_type=f32)[0:8]
    bh = bias.astype(bf16).astype(f32)
    bl = (bias - bh).astype(bf16).astype(f32)
    bl2 = bias - bh - bl
    row8 = lax.broadcasted_iota(jnp.int32, (8, D), 0)
    ext = jnp.where(row8 == 0, bh,
                    jnp.where(row8 == 1, bl, jnp.where(row8 == 2, bl2, 0.0)))
    wf = w.astype(f32)
    wr = cat([wf[2 * KH:], ext, jnp.zeros((56, D), f32)], axis=0)
    wg = wf[:2 * KH].T * g[:, :2 * KH]
    gr = cat([g[:, 2 * KH:], jnp.ones((1, 64), f32)], axis=1)
    a1 = _sa(wg[0:H, 0:KH], wg[0:H, KH:], wg[H:, 0:KH], wg[H:, KH:])
    for i in range(1, 8):
        top, bot = a1[i - 1][0:Q], a1[i - 1][Q:]
        if i in PERM:
            top, bot = bot, top
        a2 = _sa(top[:, 0:128], top[:, 128:], bot[:, 0:128], bot[:, 128:])
        a_ref[:, (i - 1) * PW:i * PW] = pltpu.bitcast(
            cat(a2, axis=0).astype(bf16), u32)
    arv = (wr.T * gr).astype(bf16)
    ar_ref[:, 0:PW] = pltpu.bitcast(arv[0:H], u32)
    ar_ref[:, PW:] = pltpu.bitcast(arv[H:], u32)

    cin_quad(0).wait()
    _norm_quad(xbuf[zs[2], :, 0:W4].astype(f32),
               *_stats_quad(xbuf[zs[0], :, 0:W4].astype(f32), []), ps[0], [])

    def run(s, nq, fresh, waits, tasks, hooks, have_st, save_st, bubble,
            valu=420, vst=110):
        k1 = s + zs[0]
        k2 = s + zs[2]
        never = {n: lax.broadcasted_iota(
            jnp.int32, (8, n * PW) if n else (16, PW), 0) < zs[1]
                 for n in (0, 2, 4)}
        zero = pl.multiple_of(zs[3], 8)
        nr = -(-65 * nq // 4)
        free = [max(valu - _VT[r % 65], 0) for r in range(nr)]
        wn = [min(free[r], max(vst - _ST[r % 65], 0) * 5.2) + 0.01
              for r in range(nr)]
        sc = sum(_NCOST) * nr / 16.25 / sum(wn)
        ws = [max(free[r] - wn[r] * sc, 0) + 0.01 for r in range(nr)]

        def xload(k, q):
            t, c = divmod(q, 2)
            return xbuf[jnp.minimum(k + t, S - 1), :,
                        c * W4:(c + 1) * W4].astype(f32)

        def make_gate(e):
            if e is None:
                return lambda v, n: v

            def gate(v, n):
                z = e[0][e[1]:e[1] + 8]
                z = cat([z] * n, axis=1) if n else cat([z, z], axis=0)
                return lax.select(never[n], z, v)
            return gate

        mr = {}
        if have_st is not None:
            mr[have_st] = (st_ref[0:8, :], st_ref[8:16, :])
        first = {}
        todo = list(tasks)

        def flush(now):
            for task in [t for t in todo if t[3] <= now + 1e-9]:
                todo.remove(task)
                kind, q, t0, t1 = task
                wt = wn if kind == "N" else ws
                cand = []
                a = 0.0
                if t0 == 0 or t0 in waits:
                    cand.append((0.0, None))
                    a += bubble[kind]
                for r in range(int(t0), nr):
                    for e in range(NPER):
                        if t0 - 1e-9 <= r + e / NPER < t1 - 1e-9:
                            cand.append(
                                (a, (first[r], Q * e // NPER // 8 * 8)))
                            a += wt[r] / NPER
                costs = _NCOST if kind == "N" else [1] * (2 * SG)
                done = 0
                gates = []
                for x in costs:
                    tgt = a * done / sum(costs)
                    gates.append(make_gate(
                        [e for (c, e) in cand if c <= tgt + 1e-9][-1]))
                    done += x
                if kind == "N":
                    _norm_quad(xload(k2, q), *mr.pop(q), ps[q % 4], gates)
                else:
                    mr[q] = _stats_quad(xload(k1, q), gates)

        count = [0]

        def mxu(lhs, rhs):
            r, o = divmod(count[0], 4)
            if o == 0 and r in waits:
                flush(r)
                waits[r]()
            v = jnp.dot(lhs(), rhs(), preferred_element_type=f32)
            if o == 0:
                first[r] = v
            count[0] += 1
            return v

        def get(i):
            return us[i][pl.ds(zero, H), :]

        def quad(p):
            sl = s + p // 2
            c0 = (p % 2) * W4
            p_ref = ps[p % 4]
            if p in fresh:
                p_ref = p_ref.at[pl.ds(zero, BROWS), :]

            def hook(name):
                if (p, name) in hooks:
                    hooks[(p, name)]()

            def dot(i, j):
                r1, c1 = _ppos(i, j)
                return mxu(
                    lambda: pltpu.bitcast(
                        a_ref[(j - 1) * 72:j * 72, (i - 1) * PW:i * PW], bf16),
                    lambda: pltpu.bitcast(
                        p_ref[r1:r1 + 64, c1:c1 + PW], bf16))

            def rem(half, cc, hr, hc):
                r1, c1 = _rpos(2 * cc + hc)
                return mxu(
                    lambda: pltpu.bitcast(
                        ar_ref[hr * 72:(hr + 1) * 72,
                               half * PW:(half + 1) * PW], bf16)[:, :KR],
                    lambda: pltpu.bitcast(
                        p_ref[r1:r1 + 40, c1:c1 + PW], bf16))

            def prod(i, o=None):
                sw = 1 if i in PERM else 0

                def rm(hr, hc):
                    return rem(o[0], o[1], hr ^ sw, hc) if o else None

                def blk(c11, c12, c21, c22):
                    rows = [cat([c11, c12], axis=1), cat([c21, c22], axis=1)]
                    return cat(rows[::-1] if sw else rows, axis=0)

                m3 = dot(i, 3)
                m5 = dot(i, 5)
                r12 = rm(0, 1)
                m1 = dot(i, 1)
                m7 = dot(i, 7)
                m4 = dot(i, 4)
                r11 = rm(0, 0)
                m2 = dot(i, 2)
                r21 = rm(1, 0)
                m6 = dot(i, 6)
                r22 = rm(1, 1)
                c12 = m3 + m5
                c21 = m2 + m4
                c11 = ((m1 + m7) - m5) + m4
                c22 = (m1 + m3) + (m6 - m2)
                return (blk(c11, c12, c21, c22),
                        blk(r11, r12, r21, r22) if o else None)

            def out(i, o, plus, minus=()):
                val, v = prod(i, o)
                if o == (1, 1):
                    hook("m6")
                v = val + v
                for u in plus:
                    v = v + get(u)
                for u in minus:
                    v = v - get(u)
                obuf[sl, o[0] * H:(o[0] + 1) * H,
                     c0 + o[1] * W2:c0 + (o[1] + 1) * W2] = v.astype(bf16)
                return val

            us[0][...] = prod(3)[0]
            hook("m3")
            us[1][...] = out(5, (0, 1), [0])
            us[2][...] = prod(2)[0]
            hook("m2")
            m4 = out(4, (1, 0), [2])
            us[3][...] = m4 - get(1)
            us[4][...] = prod(1)[0]
            hook("m1")
            out(7, (0, 0), [3, 4])
            out(6, (1, 1), [0, 4], [2])
            hook("end")

        for p in range(nq):
            flush(-(-count[0] // 4))
            quad(p)
        flush(nr)
        if save_st is not None:
            st_ref[0:8, :] = mr[save_st][0]
            st_ref[8:16, :] = mr[save_st][1]

    def wait_quads(ns):
        return lambda: [(cin_quad(n) if n < NH else cin(n // 2)).wait()
                        for n in ns]

    cin_quad(1).wait()
    run(0, FQ, range(1, FQ),
        {r: wait_quads(ns) for r, ns in _FIRST_WAITS.items()}, _FIRST_TASKS,
        {}, None, FQ + 3, {"N": 371, "S": 215}, 439, 133)

    f = FQ // 2
    j_flush = (DEFER - f) // 2
    bnd = [0, 17, 33, 49, 65]
    no_bubble = {"N": 0.01, "S": 0.01}

    def body(j, carry):
        s = f + 2 * j
        cin(s + 2).wait()
        cin(s + 3).wait()

        def write_prev(p):
            def fn():
                if p == 0:
                    @pl.when(j == j_flush)
                    def _():
                        for ct in range(8):
                            cout(pl.ds(0, DEFER), 0, D, ct)

                @pl.when(j > j_flush if p == 0 else j >= j_flush)
                def _():
                    cout_quad(s + (p - 1) // 2, (p - 1) % 2)
            return fn

        tasks = []
        for p in range(4):
            tasks += [("N", p + 3, bnd[p], bnd[p + 1]),
                      ("S", p + 4, bnd[p], bnd[p + 1])]
        run(s, 4, (3,), {}, tasks,
            {(p, "m3"): write_prev(p) for p in range(4)}, 3, 7, no_bubble)
        return carry

    lax.fori_loop(0, (S - 2 - f) // 2, body, 0)

    s = S - 2

    def write_part(half, cc):
        return lambda: [cout(S - 1, half * H, (half + 1) * H, 4 + 2 * cc + k)
                        for k in range(2)]

    hooks = {(p, "m3"): (lambda p=p: cout_quad(s + (p - 1) // 2, (p - 1) % 2))
             for p in range(4)}
    hooks.update({(3, "m2"): write_part(0, 1), (3, "m1"): write_part(1, 0),
                  (3, "m6"): write_part(0, 0), (3, "end"): write_part(1, 1)})
    run(s, 4, (3,), {}, [("N", 3, 0, 33)], hooks, 3, None, no_bubble)
    pltpu.make_async_copy(obuf, o_hbm, sout.at[0]).wait()


@jax.jit
def pallas_standalone__layernorm_linear__sampling_kernel(
    x: jax.Array,
    g: jax.Array,
    b: jax.Array,
    w: jax.Array,
):
    assert x.shape == (B, S, D) and w.shape == (D, D)
    xt = jnp.transpose(x, (1, 2, 0))
    out = pl.pallas_call(
        _kernel,
        in_specs=[pl.BlockSpec(memory_space=pl.ANY)] * 4,
        out_specs=pl.BlockSpec(memory_space=pl.ANY),
        out_shape=jax.ShapeDtypeStruct((S, D, B), x.dtype),
        scratch_shapes=[
            pltpu.VMEM((S, D, B), bf16),
            pltpu.VMEM((S, D, B), bf16),
        ] + [pltpu.VMEM((BROWS, W2), u32)] * 4
        + [pltpu.VMEM((H, W2), f32)] * 5
        + [
            pltpu.VMEM((16, W4), f32),
            pltpu.VMEM((D,), bf16),
            pltpu.VMEM((D,), bf16),
            pltpu.VMEM((D, D), bf16),
            pltpu.VMEM((7 * 72, 7 * PW), u32),
            pltpu.VMEM((144, W2), u32),
            pltpu.SMEM((4,), jnp.int32),
            pltpu.SemaphoreType.DMA((S + 3 + NH,)),
            pltpu.SemaphoreType.DMA((1,)),
        ],
        compiler_params=pltpu.CompilerParams(
            vmem_limit_bytes=110 * 1024 * 1024,
            disable_bounds_checks=True,
            disable_semaphore_checks=True,
        ),
    )(xt, g, b, w)
    return jnp.transpose(out, (2, 0, 1))
```

```python
import jax
import jax.numpy as jnp
from jax import lax
import jax.experimental.pallas as pl
import jax.experimental.pallas.tpu as pltpu

EPS = 1e-5
D = 576
S = 32
B = 1024
H = D // 2
Q = D // 4
KH = 256
KR = 80
PW = 128
W2 = 2 * PW
W4 = 4 * PW
NH = 10
FQ = 8
DEFER = 14
NPER = 18
SG = 36
f32 = jnp.float32
bf16 = jnp.bfloat16
u32 = jnp.uint32
cat = jnp.concatenate
PERM = (3, 5, 6, 7)
RROW = 28 * 64
BROWS = RROW + 80


def _sa(a11, a12, a21, a22):
    return [a11 + a22, a21 + a22, a11, a22, a11 + a12, a21 - a11, a12 - a22]


def _sb(b11, b12, b21, b22):
    return [b11 + b22, b11, b12 - b22, b21 - b11, b22, b11 + b12, b21 + b22]


def _ppos(i, j):
    return ((j - 1) * 4 + (i - 1) // 2) * 64, ((i - 1) % 2) * PW


def _rpos(ct):
    return RROW + (ct // 2) * 40, (ct % 2) * PW


_VT = [
    69, 74, 88, 142, 97, 108, 86, 159, 180, 74, 74, 71, 177, 165, 54, 224,
    205, 111, 54, 159, 110, 74, 73, 124, 197, 115, 102, 54, 173, 166, 75, 210,
    186, 112, 69, 140, 144, 74, 74, 122, 180, 98, 114, 61, 173, 181, 60, 206,
    202, 79, 73, 90, 160, 108, 108, 71, 196, 128, 74, 90, 53, 190, 169, 207,
    216]
_ST = [
    17, 54, 35, 55, 19, 52, 59, 40, 54, 18, 54, 10, 17, 19, 12, 21, 55, 56,
    23, 55, 39, 40, 41, 73, 53, 44, 56, 2, 16, 18, 12, 17, 19, 53, 56, 40, 54,
    19, 54, 59, 55, 20, 53, 20, 16, 18, 2, 16, 21, 40, 42, 54, 53, 43, 56, 43,
    53, 41, 45, 38, 9, 17, 46, 19, 18]
_TWEAK_N = [
    0.98385, 1.05057, 1.02993, 0.93299, 1.05023, 1.03936, 0.98582, 1.04086,
    0.96472, 1.02730, 0.93143, 0.95776, 1.06158, 1.03496, 0.92494, 1.04946,
    0.97776, 0.99312, 0.95971, 1.05364, 1.01375, 0.95796, 0.92688, 0.99800,
    0.92211, 1.03853, 0.94262, 0.92140, 1.07085, 0.99028, 0.95642, 1.03143,
    0.93503, 1.06471, 0.93201, 1.04749, 1.00629, 0.93629, 1.05207, 0.96283,
    1.00015, 1.07243, 1.00313, 1.00272, 0.98374, 0.97637, 1.07728, 0.94101,
    1.07103, 0.92409, 1.07401, 1.01038, 1.04828, 1.00751, 1.00674, 1.06666,
    0.96143, 1.02789, 0.97589, 1.02624, 0.93122, 1.04412, 0.95866, 1.02311,
    1.04915]
_TWEAK_S = [
    0.94475, 1.01490, 0.92222, 1.06484, 1.01462, 0.97573, 0.94670, 1.03224,
    0.95077, 1.05245, 0.92219, 0.99506, 1.07580, 0.99771, 0.97520, 0.96862,
    0.98735, 0.94918, 0.92983, 1.03025, 1.06141, 0.96667, 1.07439, 1.00876,
    0.93568, 0.99977, 1.04659, 0.94462, 0.93550, 0.95043, 0.93443, 0.95083,
    0.95162, 1.02015, 1.04397, 1.02191, 1.00415, 0.95669, 0.93918, 0.94129,
    0.96809, 0.94784, 0.93512, 1.05237, 0.96457, 1.04345, 0.95907, 1.01603,
    1.04527, 0.92655, 1.02777, 1.06300, 0.93542, 1.02003, 1.00384, 1.07230,
    0.98114, 0.95352, 1.04570, 1.00114, 1.02819, 0.99466, 1.01684, 0.94674,
    1.02499]
_NCOST = []
for _k in range(8):
    _NCOST += [43, 51, 51, 29, 21, 51, 29] + ([32] if _k % 2 == 0 else [])

_FIRST_WAITS = {17: (2, 3), 41: (4, 5, 6), 80: (7, 8, 9, 10)}
_FIRST_TASKS = [
    ("S", 1, 0, 4.56),
    ("N", 1, 4.56, 14.49),
    ("S", 2, 17, 19.92),
    ("N", 2, 19.92, 29.8276),
    ("S", 3, 19.92, 29.3276),
    ("N", 3, 29.8276, 41),
    ("S", 4, 41, 44.83),
    ("N", 4, 44.83, 56.55333),
    ("S", 5, 44.83, 56.55333),
    ("N", 5, 56.55333, 68.27667),
    ("S", 6, 56.55333, 68.27667),
    ("N", 6, 68.27667, 80),
    ("S", 7, 80, 84.1),
    ("N", 7, 84.1, 95.575),
    ("S", 8, 84.1, 95.575),
    ("N", 8, 95.575, 107.05),
    ("S", 9, 95.575, 107.05),
    ("N", 9, 107.05, 118.525),
    ("S", 10, 107.05, 118.525),
    ("N", 10, 118.525, 130.0),
    ("S", 11, 118.525, 130.0),
]

_ORDER = {
    ("put", 0): "m1 m2 m4 m6 m3 m5 m7",
    ("put", 1): "m1 m2 m4 m3 m5 m6 m7",
    ("put", 2): "m1 m6 m2 m3 m4 m5 m7",
    ("put", 3): "m2 m1 m3 m5 m6 m4 m7",
    ("sep", 0): "m1 m2 m4 m7 m3 m5 r11 r12 m6 r21 r22",
    ("sep", 1): "m1 m2 m4 m3 m6 r21 r22 m5 m7 r11 r12",
    ("sep", 2): "m3 m4 m1 m2 m6 r21 m5 m7 r11 r12 r22",
    ("sep", 3): "m3 m1 m2 m4 m6 m5 m7 r11 r12 r21 r22",
    ("merge", 0): "m3 m6 r12 r22 m1 m2 m4 r21 m5 m7 r11",
    ("merge", 1): "m3 m6 r22 m1 m2 m4 r21 m5 m7 r11 r12",
    ("merge", 2): "m6 r22 m4 m7 r11 r21 m1 m3 m5 r12 m2",
    ("merge", 3): "m1 m3 m6 r12 r22 m2 m4 m7 r21 m5 r11",
}
_TERMS = {"11": {"m1": 1, "m7": 1, "m5": -1, "m4": 1},
          "12": {"m3": 1, "m5": 1},
          "21": {"m2": 1, "m4": 1},
          "22": {"m1": 1, "m3": 1, "m6": 1, "m2": -1}}


def _stats_pair(x, gates):
    ng = len(gates) if gates else 18
    n = D // 8 // ng
    c = jnp.broadcast_to(x[0:1, :], (8, W2))
    a1 = a2 = None
    for k in range(ng):
        ck = gates[k](c, 2) if gates else c
        v = x[k * n * 8:(k + 1) * n * 8] - cat([ck] * n, axis=0)
        sq = v * v
        if a1 is not None:
            v = cat([a1, v], axis=0)
            sq = cat([a2, sq], axis=0)
        a1 = jnp.sum(v.reshape(-1, 8, W2), axis=0)
        a2 = jnp.sum(sq.reshape(-1, 8, W2), axis=0)
    a1 = jnp.sum(a1, axis=0, keepdims=True) * (1.0 / D)
    a2 = jnp.sum(a2, axis=0, keepdims=True) * (1.0 / D)
    m = c[0:1] + a1
    var = jnp.maximum(a2 - a1 * a1, 0.0)
    r = lax.rsqrt(var + EPS)
    return jnp.broadcast_to(m, (8, W2)), jnp.broadcast_to(r, (8, W2))


def _stats_quad(x, gates):
    h = len(gates) // 2
    ma, ra = _stats_pair(x[:, 0:W2], gates[:h])
    mb, rb = _stats_pair(x[:, W2:], gates[h:])
    return cat([ma, mb], axis=1), cat([ra, rb], axis=1)


def _norm_quad(x, m, r, p_ref, gates):
    def tiles(v, tc):
        return cat([v[:, tc * PW:(tc + 1) * PW],
                    v[:, (tc + 2) * PW:(tc + 3) * PW]], axis=1)

    def wide(v):
        return cat([cat([v, v], axis=1)] * 2, axis=0)

    xt = [tiles(x, 0), tiles(x, 1)]
    mt = [tiles(m, 0), tiles(m, 1)]
    rt = [wide(tiles(r, 0)), wide(tiles(r, 1))]
    r16 = cat([r, r], axis=0)
    it = iter(gates)

    def sub(k, kr, tc):
        g = next(it, None)
        mg = mt[tc] if g is None else g(mt[tc], 2)
        r0 = kr * 128 + k * 16
        xb = cat([xt[tc][r0:r0 + 16], xt[tc][KH + r0:KH + r0 + 16]], axis=1)
        return (xb - wide(mg)) * rt[tc]

    def emit(k, j, v, gate=False):
        q = [v[:, i * PW:(i + 1) * PW] for i in range(4)]
        g = next(it, None) if gate else None
        if g is not None:
            q[0] = g(q[0], 0)
            q[3] = g(q[3], 0)
        ops = _sb(*q)
        for i0 in range(0, 7, 2):
            grp = ops[i0:i0 + 2]
            r0 = _ppos(i0 + 1, j)[0] + k * 8
            p_ref[r0:r0 + 8, 0:len(grp) * PW] = pltpu.bitcast(
                cat(grp, axis=1).astype(bf16), u32)

    for k in range(8):
        b11 = sub(k, 0, 0)
        emit(k, 2, b11)
        b12 = sub(k, 0, 1)
        emit(k, 6, b11 + b12)
        b22 = sub(k, 1, 1)
        emit(k, 3, b12 - b22)
        emit(k, 1, b11 + b22, True)
        emit(k, 5, b22, True)
        b21 = sub(k, 1, 0)
        emit(k, 4, b21 - b11)
        emit(k, 7, b21 + b22, True)
        if k % 2 == 0:
            g = next(it, None)
            mg = m if g is None else g(m, 4)
            r0 = 2 * KH + k * 8
            v = (x[r0:r0 + 16] - cat([mg, mg], axis=0)) * r16
            for c0 in (0, 2):
                r1 = _rpos(c0)[0] + k * 4
                p_ref[r1:r1 + 8, :] = pltpu.bitcast(
                    v[:, c0 * PW:(c0 + 2) * PW].astype(bf16), u32)


def _kernel(x_hbm, g_hbm, b_hbm, w_hbm, o_hbm, xbuf, obuf,
            p0, p1, p2, p3, u0, u1, u2, u3, u4,
            st_ref, g_ref, b_ref, w_ref, a_ref, ar_ref, zs, sin, sout):
    ps = [p0, p1, p2, p3]
    us = [u0, u1, u2, u3, u4]
    for i in range(4):
        zs[i] = 0

    def cin(i):
        return pltpu.make_async_copy(x_hbm.at[i], xbuf.at[i], sin.at[i])

    def cin_quad(n):
        t, c = divmod(n, 2)
        return pltpu.make_async_copy(
            x_hbm.at[t, :, c * W4:(c + 1) * W4],
            xbuf.at[t, :, c * W4:(c + 1) * W4], sin.at[S + 3 + n])

    def cout(sl, r0, r1, ct):
        idx = (sl, slice(r0, r1), slice(ct * PW, (ct + 1) * PW))
        pltpu.make_async_copy(
            obuf.at[idx], o_hbm.at[idx], sout.at[0]).start(priority=ct % 2)

    def cout_quad(t, c):
        for ct in range(4):
            cout(t, 0, D, 4 * c + ct)

    cw = pltpu.make_async_copy(w_hbm, w_ref, sin.at[S])
    cg = pltpu.make_async_copy(g_hbm, g_ref, sin.at[S + 1])
    cb = pltpu.make_async_copy(b_hbm, b_ref, sin.at[S + 2])
    cg.start()
    cb.start()
    cw.start()
    for n in range(NH):
        cin_quad(n).start()
    for i in range(NH // 2, S):
        cin(i).start()

    row16 = lax.broadcasted_iota(jnp.int32, (16, W2), 0)
    ones = pltpu.bitcast(jnp.where(row16 < 3, 1.0, 0.0).astype(bf16), u32)
    for p_ref in ps:
        for c0 in (0, 2):
            r1 = _rpos(c0)[0] + 32
            p_ref[r1:r1 + 8, :] = ones

    cg.wait()
    cb.wait()
    cw.wait()
    g = g_ref[...].astype(f32).reshape(1, D)
    w = w_ref[...]
    b16 = jnp.broadcast_to(b_ref[...].reshape(1, D), (16, D))
    bias = jnp.dot(b16, w, preferred_element_type=f32)[0:8]
    bh = bias.astype(bf16).astype(f32)
    bl = (bias - bh).astype(bf16).astype(f32)
    bl2 = bias - bh - bl
    row8 = lax.broadcasted_iota(jnp.int32, (8, D), 0)
    ext = jnp.where(row8 == 0, bh,
                    jnp.where(row8 == 1, bl, jnp.where(row8 == 2, bl2, 0.0)))
    wf = w.astype(f32)
    wr = cat([wf[2 * KH:], ext, jnp.zeros((56, D), f32)], axis=0)
    wg = wf[:2 * KH].T * g[:, :2 * KH]
    gr = cat([g[:, 2 * KH:], jnp.ones((1, 64), f32)], axis=1)
    a1 = _sa(wg[0:H, 0:KH], wg[0:H, KH:], wg[H:, 0:KH], wg[H:, KH:])
    for i in range(1, 8):
        top, bot = a1[i - 1][0:Q], a1[i - 1][Q:]
        if i in PERM:
            top, bot = bot, top
        a2 = _sa(top[:, 0:128], top[:, 128:], bot[:, 0:128], bot[:, 128:])
        a_ref[:, (i - 1) * PW:i * PW] = pltpu.bitcast(
            cat(a2, axis=0).astype(bf16), u32)
    arv = (wr.T * gr).astype(bf16)
    ar_ref[:, 0:PW] = pltpu.bitcast(arv[0:H], u32)
    ar_ref[:, PW:] = pltpu.bitcast(arv[H:], u32)

    cin_quad(0).wait()
    _norm_quad(xbuf[zs[2], :, 0:W4].astype(f32),
               *_stats_quad(xbuf[zs[0], :, 0:W4].astype(f32), []), ps[0], [])

    def run(s, nq, fresh, waits, tasks, hooks, have_st, save_st, bubble,
            valu=415, vst=112, ratio=4.79, tweak=True):
        k1 = s + zs[0]
        k2 = s + zs[2]
        never = {n: lax.broadcasted_iota(
            jnp.int32, (8, n * PW) if n else (16, PW), 0) < zs[1]
                 for n in (0, 2, 4)}
        zero = pl.multiple_of(zs[3], 8)
        nr = -(-65 * nq // 4)
        free = [max(valu - _VT[r % 65], 0) for r in range(nr)]
        tn = _TWEAK_N if tweak else [1] * 65
        ts = _TWEAK_S if tweak else [1] * 65
        wn = [(min(free[r], max(vst - _ST[r % 65], 0) * ratio) + 0.01)
              * tn[r % 65] for r in range(nr)]
        sc = sum(_NCOST) * nr / 16.25 / sum(wn)
        ws = [(max(free[r] - wn[r] * sc, 0) + 0.01) * ts[r % 65]
              for r in range(nr)]

        def xload(k, q):
            t, c = divmod(q, 2)
            return xbuf[jnp.minimum(k + t, S - 1), :,
                        c * W4:(c + 1) * W4].astype(f32)

        def make_gate(e):
            if e is None:
                return lambda v, n: v

            def gate(v, n):
                z = e[0][e[1]:e[1] + 8]
                z = cat([z] * n, axis=1) if n else cat([z, z], axis=0)
                return lax.select(never[n], z, v)
            return gate

        mr = {}
        if have_st is not None:
            mr[have_st] = (st_ref[0:8, :], st_ref[8:16, :])
        first = {}
        todo = list(tasks)

        def flush(now):
            for task in [t for t in todo if t[3] <= now + 1e-9]:
                todo.remove(task)
                kind, q, t0, t1 = task
                wt = wn if kind == "N" else ws
                cand = []
                a = 0.0
                if t0 == 0 or t0 in waits:
                    cand.append((0.0, None))
                    a += bubble[kind]
                for r in range(int(t0), nr):
                    for e in range(NPER):
                        if t0 - 1e-9 <= r + e / NPER < t1 - 1e-9:
                            cand.append(
                                (a, (first[r], Q * e // NPER // 8 * 8)))
                            a += wt[r] / NPER
                costs = _NCOST if kind == "N" else [1] * (2 * SG)
                done = 0
                gates = []
                for x in costs:
                    tgt = a * done / sum(costs)
                    gates.append(make_gate(
                        [e for (c, e) in cand if c <= tgt + 1e-9][-1]))
                    done += x
                if kind == "N":
                    _norm_quad(xload(k2, q), *mr.pop(q), ps[q % 4], gates)
                else:
                    mr[q] = _stats_quad(xload(k1, q), gates)

        count = [0]

        def mxu(lhs, rhs):
            r, o = divmod(count[0], 4)
            if o == 0 and r in waits:
                flush(r)
                waits[r]()
            v = jnp.dot(lhs(), rhs(), preferred_element_type=f32)
            if o == 0:
                first[r] = v
            count[0] += 1
            return v

        def get(i):
            return us[i][pl.ds(zero, H), :]

        def quad(p):
            sl = s + p // 2
            c0 = (p % 2) * W4
            p_ref = ps[p % 4]
            if p in fresh:
                p_ref = p_ref.at[pl.ds(zero, BROWS), :]

            def hook(name):
                if (p, name) in hooks:
                    hooks[(p, name)]()

            def dot(i, j):
                r1, c1 = _ppos(i, j)
                return mxu(
                    lambda: pltpu.bitcast(
                        a_ref[(j - 1) * 72:j * 72, (i - 1) * PW:i * PW], bf16),
                    lambda: pltpu.bitcast(
                        p_ref[r1:r1 + 64, c1:c1 + PW], bf16))

            def rem(half, cc, hr, hc):
                r1, c1 = _rpos(2 * cc + hc)
                return mxu(
                    lambda: pltpu.bitcast(
                        ar_ref[hr * 72:(hr + 1) * 72,
                               half * PW:(half + 1) * PW], bf16)[:, :KR],
                    lambda: pltpu.bitcast(
                        p_ref[r1:r1 + 40, c1:c1 + PW], bf16))

            def prod(i, o=None):
                sw = 1 if i in PERM else 0

                def blk(c):
                    rows = [cat([c["11"], c["12"]], axis=1),
                            cat([c["21"], c["22"]], axis=1)]
                    return cat(rows[::-1] if sw else rows, axis=0)

                kind = "sep" if i in (4, 5) else "merge" if o else "put"
                acc = {}
                sign = {}
                sep = {}
                for nm in _ORDER[(kind, count[0] % 4)].split():
                    if nm[0] == "m":
                        v = dot(i, int(nm[1]))
                    else:
                        v = rem(o[0], o[1], (int(nm[1]) - 1) ^ sw,
                                int(nm[2]) - 1)
                        sep[nm[1:]] = v
                    for k, terms in _TERMS.items():
                        sg = terms.get(nm)
                        if kind == "merge" and nm == "r" + k:
                            sg = 1
                        if sg is None:
                            continue
                        if k not in acc:
                            acc[k], sign[k] = v, sg
                        elif sign[k] < 0:
                            acc[k], sign[k] = v - acc[k], 1
                        else:
                            acc[k] = acc[k] + v if sg > 0 else acc[k] - v
                return blk(acc), blk(sep) if kind == "sep" else None

            def out(i, o, plus, minus=()):
                val, v = prod(i, o)
                if o == (1, 1):
                    hook("m6")
                v = val if v is None else val + v
                for u in plus:
                    v = v + get(u)
                for u in minus:
                    v = v - get(u)
                obuf[sl, o[0] * H:(o[0] + 1) * H,
                     c0 + o[1] * W2:c0 + (o[1] + 1) * W2] = v.astype(bf16)
                return val

            us[0][...] = prod(3)[0]
            hook("m3")
            us[1][...] = out(5, (0, 1), [0])
            us[2][...] = prod(2)[0]
            hook("m2")
            m4 = out(4, (1, 0), [2])
            us[3][...] = m4 - get(1)
            us[4][...] = prod(1)[0]
            hook("m1")
            out(7, (0, 0), [3, 4])
            out(6, (1, 1), [0, 4], [2])
            hook("end")

        for p in range(nq):
            flush(-(-count[0] // 4))
            quad(p)
        flush(nr)
        if save_st is not None:
            st_ref[0:8, :] = mr[save_st][0]
            st_ref[8:16, :] = mr[save_st][1]

    def wait_quads(ns):
        return lambda: [(cin_quad(n) if n < NH else cin(n // 2)).wait()
                        for n in ns]

    cin_quad(1).wait()
    run(0, FQ, range(1, FQ),
        {r: wait_quads(ns) for r, ns in _FIRST_WAITS.items()}, _FIRST_TASKS,
        {}, None, FQ + 3, {"N": 287, "S": 321}, 478, 96, 6.56, False)

    f = FQ // 2
    j_flush = (DEFER - f) // 2
    bnd = [0, 17, 33, 49, 65]
    no_bubble = {"N": 0.01, "S": 0.01}

    def body(j, carry):
        s = f + 2 * j
        cin(s + 2).wait()
        cin(s + 3).wait()

        def write_prev(p):
            def fn():
                if p == 0:
                    @pl.when(j == j_flush)
                    def _():
                        for ct in range(8):
                            cout(pl.ds(0, DEFER), 0, D, ct)

                @pl.when(j > j_flush if p == 0 else j >= j_flush)
                def _():
                    cout_quad(s + (p - 1) // 2, (p - 1) % 2)
            return fn

        tasks = []
        for p in range(4):
            tasks += [("N", p + 3, bnd[p], bnd[p + 1]),
                      ("S", p + 4, bnd[p], bnd[p + 1])]
        run(s, 4, (3,), {}, tasks,
            {(p, "m3"): write_prev(p) for p in range(4)}, 3, 7, no_bubble)
        return carry

    lax.fori_loop(0, (S - 2 - f) // 2, body, 0)

    s = S - 2

    def write_part(half, cc):
        return lambda: [cout(S - 1, half * H, (half + 1) * H, 4 + 2 * cc + k)
                        for k in range(2)]

    hooks = {(p, "m3"): (lambda p=p: cout_quad(s + (p - 1) // 2, (p - 1) % 2))
             for p in range(4)}
    hooks.update({(3, "m2"): write_part(0, 1), (3, "m1"): write_part(1, 0),
                  (3, "m6"): write_part(0, 0), (3, "end"): write_part(1, 1)})
    run(s, 4, (3,), {}, [("N", 3, 0, 33)], hooks, 3, None, no_bubble)
    pltpu.make_async_copy(obuf, o_hbm, sout.at[0]).wait()


@jax.jit
def pallas_standalone__layernorm_linear__sampling_kernel(
    x: jax.Array,
    g: jax.Array,
    b: jax.Array,
    w: jax.Array,
):
    assert x.shape == (B, S, D) and w.shape == (D, D)
    xt = jnp.transpose(x, (1, 2, 0))
    out = pl.pallas_call(
        _kernel,
        in_specs=[pl.BlockSpec(memory_space=pl.ANY)] * 4,
        out_specs=pl.BlockSpec(memory_space=pl.ANY),
        out_shape=jax.ShapeDtypeStruct((S, D, B), x.dtype),
        scratch_shapes=[
            pltpu.VMEM((S, D, B), bf16),
            pltpu.VMEM((S, D, B), bf16),
        ] + [pltpu.VMEM((BROWS, W2), u32)] * 4
        + [pltpu.VMEM((H, W2), f32)] * 5
        + [
            pltpu.VMEM((16, W4), f32),
            pltpu.VMEM((D,), bf16),
            pltpu.VMEM((D,), bf16),
            pltpu.VMEM((D, D), bf16),
            pltpu.VMEM((7 * 72, 7 * PW), u32),
            pltpu.VMEM((144, W2), u32),
            pltpu.SMEM((4,), jnp.int32),
            pltpu.SemaphoreType.DMA((S + 3 + NH,)),
            pltpu.SemaphoreType.DMA((1,)),
        ],
        compiler_params=pltpu.CompilerParams(
            vmem_limit_bytes=110 * 1024 * 1024,
            disable_bounds_checks=True,
            disable_semaphore_checks=True,
        ),
    )(xt, g, b, w)
    return jnp.transpose(out, (2, 0, 1))
```

```python
import jax
import jax.numpy as jnp
from jax import lax
import jax.experimental.pallas as pl
import jax.experimental.pallas.tpu as pltpu

EPS = 1e-5
D = 576
S = 32
B = 1024
H = D // 2
Q = D // 4
KH = 256
KR = 80
PW = 128
W2 = 2 * PW
W4 = 4 * PW
NH = 10
FQ = 8
DEFER = 14
NPER = 18
SG = 36
f32 = jnp.float32
bf16 = jnp.bfloat16
u32 = jnp.uint32
cat = jnp.concatenate
PERM = (3, 5, 6, 7)
RROW = 28 * 64
BROWS = RROW + 80


def _sa(a11, a12, a21, a22):
    return [a11 + a22, a21 + a22, a11, a22, a11 + a12, a21 - a11, a12 - a22]


def _sb(b11, b12, b21, b22):
    return [b11 + b22, b11, b12 - b22, b21 - b11, b22, b11 + b12, b21 + b22]


def _ppos(i, j):
    return ((j - 1) * 4 + (i - 1) // 2) * 64, ((i - 1) % 2) * PW


def _rpos(ct):
    return RROW + (ct // 2) * 40, (ct % 2) * PW


_VT = [
    69, 74, 88, 142, 97, 108, 86, 159, 180, 74, 74, 71, 177, 165, 54, 224,
    205, 111, 54, 159, 110, 74, 73, 124, 197, 115, 102, 54, 173, 166, 75, 210,
    186, 112, 69, 140, 144, 74, 74, 122, 180, 98, 114, 61, 173, 181, 60, 206,
    202, 79, 73, 90, 160, 108, 108, 71, 196, 128, 74, 90, 53, 190, 169, 207,
    216]
_ST = [
    17, 54, 35, 55, 19, 52, 59, 40, 54, 18, 54, 10, 17, 19, 12, 21, 55, 56,
    23, 55, 39, 40, 41, 73, 53, 44, 56, 2, 16, 18, 12, 17, 19, 53, 56, 40, 54,
    19, 54, 59, 55, 20, 53, 20, 16, 18, 2, 16, 21, 40, 42, 54, 53, 43, 56, 43,
    53, 41, 45, 38, 9, 17, 46, 19, 18]
_TWEAK_N = [
    0.9253, 0.9354, 0.9478, 1.0229, 1.0795, 0.9303, 0.9248, 1.0735, 0.9475,
    1.073, 0.9784, 0.9462, 0.987, 1.0775, 1.0001, 1.0187, 0.9896, 0.9355,
    0.9913, 0.9862, 0.9478, 1.0335, 1.047, 1.0497, 0.9403, 1.0478, 1.0614,
    1.0101, 1.0771, 1.0353, 0.9234, 1.0758, 1.0599, 0.9549, 1.0484, 0.9912,
    1.0628, 0.9387, 0.9296, 1.0257, 0.9332, 1.0155, 1.0038, 0.9285, 0.9317,
    0.9624, 0.9289, 0.9468, 1.0386, 0.9667, 1.006, 1.0746, 0.9698, 1.0238,
    0.943, 0.9348, 1.027, 0.9221, 0.9333, 0.9957, 0.9775, 0.9369, 0.987,
    1.0613, 1.0794]
_TWEAK_S = [
    0.9577, 0.9269, 0.9884, 0.9264, 1.0386, 1.0098, 1.0269, 1.204, 0.9235,
    0.9502, 1.0472, 0.9905, 1.0602, 0.9279, 1.0287, 1.0749, 1.071, 0.9804,
    0.9234, 1.0212, 0.7479, 1.0026, 1.1669, 1.0276, 1.042, 0.9729, 0.9638,
    1.079, 1.0254, 0.9449, 1.0404, 0.9948, 1.0745, 1.063, 0.949, 0.9791,
    0.9723, 0.9943, 0.9771, 1.0036, 1.1351, 1.0379, 1.0337, 1.0467, 0.9334,
    1.0734, 1.003, 0.9499, 0.6706, 0.9401, 0.9814, 1.1228, 1.0367, 1.059,
    0.9422, 0.9378, 1.0647, 1.0284, 1.073, 0.946, 0.9292, 1.0732, 1.0415,
    1.0331, 0.994]
_NCOST = []
for _k in range(8):
    _NCOST += [43, 51, 51, 29, 21, 51, 29] + ([32] if _k % 2 == 0 else [])

_FIRST_WAITS = {17: (2, 3), 41: (4, 5, 6), 80: (7, 8, 9, 10)}
_FIRST_TASKS = [
    ("S", 1, 0, 4.56),
    ("N", 1, 4.56, 14.49),
    ("S", 2, 17, 19.92),
    ("N", 2, 19.92, 29.8276),
    ("S", 3, 19.92, 29.3276),
    ("N", 3, 29.8276, 41),
    ("S", 4, 41, 44.83),
    ("N", 4, 44.83, 56.55333),
    ("S", 5, 44.83, 56.55333),
    ("N", 5, 56.55333, 68.27667),
    ("S", 6, 56.55333, 68.27667),
    ("N", 6, 68.27667, 80),
    ("S", 7, 80, 84.1),
    ("N", 7, 84.1, 95.575),
    ("S", 8, 84.1, 95.575),
    ("N", 8, 95.575, 107.05),
    ("S", 9, 95.575, 107.05),
    ("N", 9, 107.05, 118.525),
    ("S", 10, 107.05, 118.525),
    ("N", 10, 118.525, 130.0),
    ("S", 11, 118.525, 130.0),
]

_ORDER = {
    ("put", 0): "m1 m2 m4 m6 m3 m5 m7",
    ("put", 1): "m1 m2 m4 m3 m5 m6 m7",
    ("put", 2): "m1 m6 m2 m3 m4 m5 m7",
    ("put", 3): "m2 m1 m3 m5 m6 m4 m7",
    ("sep", 0): "m1 m2 m4 m7 m3 m5 r11 r12 m6 r21 r22",
    ("sep", 1): "m1 m2 m4 m3 m6 r21 r22 m5 m7 r11 r12",
    ("sep", 2): "m3 m4 m1 m2 m6 r21 m5 m7 r11 r12 r22",
    ("sep", 3): "m3 m1 m2 m4 m6 m5 m7 r11 r12 r21 r22",
    ("merge", 0): "m3 m6 r12 r22 m1 m2 m4 r21 m5 m7 r11",
    ("merge", 1): "m3 m6 r22 m1 m2 m4 r21 m5 m7 r11 r12",
    ("merge", 2): "m6 r22 m4 m7 r11 r21 m1 m3 m5 r12 m2",
    ("merge", 3): "m1 m3 m6 r12 r22 m2 m4 m7 r21 m5 r11",
}
_TERMS = {"11": {"m1": 1, "m7": 1, "m5": -1, "m4": 1},
          "12": {"m3": 1, "m5": 1},
          "21": {"m2": 1, "m4": 1},
          "22": {"m1": 1, "m3": 1, "m6": 1, "m2": -1}}


def _stats_pair(x, gates):
    ng = len(gates) if gates else 18
    n = D // 8 // ng
    c = jnp.broadcast_to(x[0:1, :], (8, W2))
    a1 = a2 = None
    for k in range(ng):
        ck = gates[k](c, 2) if gates else c
        v = x[k * n * 8:(k + 1) * n * 8] - cat([ck] * n, axis=0)
        sq = v * v
        if a1 is not None:
            v = cat([a1, v], axis=0)
            sq = cat([a2, sq], axis=0)
        a1 = jnp.sum(v.reshape(-1, 8, W2), axis=0)
        a2 = jnp.sum(sq.reshape(-1, 8, W2), axis=0)
    a1 = jnp.sum(a1, axis=0, keepdims=True) * (1.0 / D)
    a2 = jnp.sum(a2, axis=0, keepdims=True) * (1.0 / D)
    m = c[0:1] + a1
    var = jnp.maximum(a2 - a1 * a1, 0.0)
    r = lax.rsqrt(var + EPS)
    return jnp.broadcast_to(m, (8, W2)), jnp.broadcast_to(r, (8, W2))


def _stats_quad(x, gates):
    h = len(gates) // 2
    ma, ra = _stats_pair(x[:, 0:W2], gates[:h])
    mb, rb = _stats_pair(x[:, W2:], gates[h:])
    return cat([ma, mb], axis=1), cat([ra, rb], axis=1)


def _norm_quad(x, m, r, p_ref, gates):
    def tiles(v, tc):
        return cat([v[:, tc * PW:(tc + 1) * PW],
                    v[:, (tc + 2) * PW:(tc + 3) * PW]], axis=1)

    def wide(v):
        return cat([cat([v, v], axis=1)] * 2, axis=0)

    xt = [tiles(x, 0), tiles(x, 1)]
    mt = [tiles(m, 0), tiles(m, 1)]
    rt = [wide(tiles(r, 0)), wide(tiles(r, 1))]
    r16 = cat([r, r], axis=0)
    it = iter(gates)

    def sub(k, kr, tc):
        g = next(it, None)
        mg = mt[tc] if g is None else g(mt[tc], 2)
        r0 = kr * 128 + k * 16
        xb = cat([xt[tc][r0:r0 + 16], xt[tc][KH + r0:KH + r0 + 16]], axis=1)
        return (xb - wide(mg)) * rt[tc]

    def emit(k, j, v, gate=False):
        q = [v[:, i * PW:(i + 1) * PW] for i in range(4)]
        g = next(it, None) if gate else None
        if g is not None:
            q[0] = g(q[0], 0)
            q[3] = g(q[3], 0)
        ops = _sb(*q)
        for i0 in range(0, 7, 2):
            grp = ops[i0:i0 + 2]
            r0 = _ppos(i0 + 1, j)[0] + k * 8
            p_ref[r0:r0 + 8, 0:len(grp) * PW] = pltpu.bitcast(
                cat(grp, axis=1).astype(bf16), u32)

    for k in range(8):
        b11 = sub(k, 0, 0)
        emit(k, 2, b11)
        b12 = sub(k, 0, 1)
        emit(k, 6, b11 + b12)
        b22 = sub(k, 1, 1)
        emit(k, 3, b12 - b22)
        emit(k, 1, b11 + b22, True)
        emit(k, 5, b22, True)
        b21 = sub(k, 1, 0)
        emit(k, 4, b21 - b11)
        emit(k, 7, b21 + b22, True)
        if k % 2 == 0:
            g = next(it, None)
            mg = m if g is None else g(m, 4)
            r0 = 2 * KH + k * 8
            v = (x[r0:r0 + 16] - cat([mg, mg], axis=0)) * r16
            for c0 in (0, 2):
                r1 = _rpos(c0)[0] + k * 4
                p_ref[r1:r1 + 8, :] = pltpu.bitcast(
                    v[:, c0 * PW:(c0 + 2) * PW].astype(bf16), u32)


def _kernel(x_hbm, g_hbm, b_hbm, w_hbm, o_hbm, xbuf, obuf,
            p0, p1, p2, p3, u0, u1, u2, u3, u4,
            st_ref, g_ref, b_ref, w_ref, a_ref, ar_ref, zs, sin, sout):
    ps = [p0, p1, p2, p3]
    us = [u0, u1, u2, u3, u4]
    for i in range(4):
        zs[i] = 0

    def cin(i):
        return pltpu.make_async_copy(x_hbm.at[i], xbuf.at[i], sin.at[i])

    def cin_quad(n):
        t, c = divmod(n, 2)
        return pltpu.make_async_copy(
            x_hbm.at[t, :, c * W4:(c + 1) * W4],
            xbuf.at[t, :, c * W4:(c + 1) * W4], sin.at[S + 3 + n])

    def cout(sl, r0, r1, ct):
        idx = (sl, slice(r0, r1), slice(ct * PW, (ct + 1) * PW))
        pltpu.make_async_copy(
            obuf.at[idx], o_hbm.at[idx], sout.at[0]).start(priority=ct % 2)

    def cout_quad(t, c):
        for ct in range(4):
            cout(t, 0, D, 4 * c + ct)

    cw = pltpu.make_async_copy(w_hbm, w_ref, sin.at[S])
    cg = pltpu.make_async_copy(g_hbm, g_ref, sin.at[S + 1])
    cb = pltpu.make_async_copy(b_hbm, b_ref, sin.at[S + 2])
    cg.start()
    cb.start()
    cw.start()
    for n in range(NH):
        cin_quad(n).start()
    for i in range(NH // 2, S):
        cin(i).start()

    row16 = lax.broadcasted_iota(jnp.int32, (16, W2), 0)
    ones = pltpu.bitcast(jnp.where(row16 < 3, 1.0, 0.0).astype(bf16), u32)
    for p_ref in ps:
        for c0 in (0, 2):
            r1 = _rpos(c0)[0] + 32
            p_ref[r1:r1 + 8, :] = ones

    cg.wait()
    cb.wait()
    cw.wait()
    g = g_ref[...].astype(f32).reshape(1, D)
    w = w_ref[...]
    b16 = jnp.broadcast_to(b_ref[...].reshape(1, D), (16, D))
    bias = jnp.dot(b16, w, preferred_element_type=f32)[0:8]
    bh = bias.astype(bf16).astype(f32)
    bl = (bias - bh).astype(bf16).astype(f32)
    bl2 = bias - bh - bl
    row8 = lax.broadcasted_iota(jnp.int32, (8, D), 0)
    ext = jnp.where(row8 == 0, bh,
                    jnp.where(row8 == 1, bl, jnp.where(row8 == 2, bl2, 0.0)))
    wf = w.astype(f32)
    wr = cat([wf[2 * KH:], ext, jnp.zeros((56, D), f32)], axis=0)
    wg = wf[:2 * KH].T * g[:, :2 * KH]
    gr = cat([g[:, 2 * KH:], jnp.ones((1, 64), f32)], axis=1)
    a1 = _sa(wg[0:H, 0:KH], wg[0:H, KH:], wg[H:, 0:KH], wg[H:, KH:])
    for i in range(1, 8):
        top, bot = a1[i - 1][0:Q], a1[i - 1][Q:]
        if i in PERM:
            top, bot = bot, top
        a2 = _sa(top[:, 0:128], top[:, 128:], bot[:, 0:128], bot[:, 128:])
        a_ref[:, (i - 1) * PW:i * PW] = pltpu.bitcast(
            cat(a2, axis=0).astype(bf16), u32)
    arv = (wr.T * gr).astype(bf16)
    ar_ref[:, 0:PW] = pltpu.bitcast(arv[0:H], u32)
    ar_ref[:, PW:] = pltpu.bitcast(arv[H:], u32)

    cin_quad(0).wait()
    _norm_quad(xbuf[zs[2], :, 0:W4].astype(f32),
               *_stats_quad(xbuf[zs[0], :, 0:W4].astype(f32), []), ps[0], [])

    def run(s, nq, fresh, waits, tasks, hooks, have_st, save_st, bubble,
            valu=446, vst=99, ratio=6.89, tweak=True):
        k1 = s + zs[0]
        k2 = s + zs[2]
        never = {n: lax.broadcasted_iota(
            jnp.int32, (8, n * PW) if n else (16, PW), 0) < zs[1]
                 for n in (0, 2, 4)}
        zero = pl.multiple_of(zs[3], 8)
        nr = -(-65 * nq // 4)
        free = [max(valu - _VT[r % 65], 0) for r in range(nr)]
        tn = _TWEAK_N if tweak else [1] * 65
        ts = _TWEAK_S if tweak else [1] * 65
        wn = [(min(free[r], max(vst - _ST[r % 65], 0) * ratio) + 0.01)
              * tn[r % 65] for r in range(nr)]
        sc = sum(_NCOST) * nr / 16.25 / sum(wn)
        ws = [(max(free[r] - wn[r] * sc, 0) + 0.01) * ts[r % 65]
              for r in range(nr)]

        def xload(k, q):
            t, c = divmod(q, 2)
            return xbuf[jnp.minimum(k + t, S - 1), :,
                        c * W4:(c + 1) * W4].astype(f32)

        def make_gate(e):
            if e is None:
                return lambda v, n: v

            def gate(v, n):
                z = e[0][e[1]:e[1] + 8]
                z = cat([z] * n, axis=1) if n else cat([z, z], axis=0)
                return lax.select(never[n], z, v)
            return gate

        mr = {}
        if have_st is not None:
            mr[have_st] = (st_ref[0:8, :], st_ref[8:16, :])
        first = {}
        todo = list(tasks)

        def flush(now):
            for task in [t for t in todo if t[3] <= now + 1e-9]:
                todo.remove(task)
                kind, q, t0, t1 = task
                wt = wn if kind == "N" else ws
                cand = []
                a = 0.0
                if t0 == 0 or t0 in waits:
                    cand.append((0.0, None))
                    a += bubble[kind]
                for r in range(int(t0), nr):
                    for e in range(NPER):
                        if t0 - 1e-9 <= r + e / NPER < t1 - 1e-9:
                            cand.append(
                                (a, (first[r], Q * e // NPER // 8 * 8)))
                            a += wt[r] / NPER
                costs = _NCOST if kind == "N" else [1] * (2 * SG)
                done = 0
                gates = []
                for x in costs:
                    tgt = a * done / sum(costs)
                    gates.append(make_gate(
                        [e for (c, e) in cand if c <= tgt + 1e-9][-1]))
                    done += x
                if kind == "N":
                    _norm_quad(xload(k2, q), *mr.pop(q), ps[q % 4], gates)
                else:
                    mr[q] = _stats_quad(xload(k1, q), gates)

        count = [0]

        def mxu(lhs, rhs):
            r, o = divmod(count[0], 4)
            if o == 0 and r in waits:
                flush(r)
                waits[r]()
            v = jnp.dot(lhs(), rhs(), preferred_element_type=f32)
            if o == 0:
                first[r] = v
            count[0] += 1
            return v

        def get(i):
            return us[i][pl.ds(zero, H), :]

        def quad(p):
            sl = s + p // 2
            c0 = (p % 2) * W4
            p_ref = ps[p % 4]
            if p in fresh:
                p_ref = p_ref.at[pl.ds(zero, BROWS), :]

            def hook(name):
                if (p, name) in hooks:
                    hooks[(p, name)]()

            def dot(i, j):
                r1, c1 = _ppos(i, j)
                return mxu(
                    lambda: pltpu.bitcast(
                        a_ref[(j - 1) * 72:j * 72, (i - 1) * PW:i * PW], bf16),
                    lambda: pltpu.bitcast(
                        p_ref[r1:r1 + 64, c1:c1 + PW], bf16))

            def rem(half, cc, hr, hc):
                r1, c1 = _rpos(2 * cc + hc)
                return mxu(
                    lambda: pltpu.bitcast(
                        ar_ref[hr * 72:(hr + 1) * 72,
                               half * PW:(half + 1) * PW], bf16)[:, :KR],
                    lambda: pltpu.bitcast(
                        p_ref[r1:r1 + 40, c1:c1 + PW], bf16))

            def prod(i, o=None):
                sw = 1 if i in PERM else 0

                def blk(c):
                    rows = [cat([c["11"], c["12"]], axis=1),
                            cat([c["21"], c["22"]], axis=1)]
                    return cat(rows[::-1] if sw else rows, axis=0)

                kind = "sep" if i in (4, 5) else "merge" if o else "put"
                acc = {}
                sign = {}
                sep = {}
                for nm in _ORDER[(kind, count[0] % 4)].split():
                    if nm[0] == "m":
                        v = dot(i, int(nm[1]))
                    else:
                        v = rem(o[0], o[1], (int(nm[1]) - 1) ^ sw,
                                int(nm[2]) - 1)
                        sep[nm[1:]] = v
                    for k, terms in _TERMS.items():
                        sg = terms.get(nm)
                        if kind == "merge" and nm == "r" + k:
                            sg = 1
                        if sg is None:
                            continue
                        if k not in acc:
                            acc[k], sign[k] = v, sg
                        elif sign[k] < 0:
                            acc[k], sign[k] = v - acc[k], 1
                        else:
                            acc[k] = acc[k] + v if sg > 0 else acc[k] - v
                return blk(acc), blk(sep) if kind == "sep" else None

            def out(i, o, plus, minus=()):
                val, v = prod(i, o)
                if o == (1, 1):
                    hook("m6")
                v = val if v is None else val + v
                for u in plus:
                    v = v + get(u)
                for u in minus:
                    v = v - get(u)
                obuf[sl, o[0] * H:(o[0] + 1) * H,
                     c0 + o[1] * W2:c0 + (o[1] + 1) * W2] = v.astype(bf16)
                return val

            us[0][...] = prod(3)[0]
            hook("m3")
            us[1][...] = out(5, (0, 1), [0])
            us[2][...] = prod(2)[0]
            hook("m2")
            m4 = out(4, (1, 0), [2])
            us[3][...] = m4 - get(1)
            us[4][...] = prod(1)[0]
            hook("m1")
            out(7, (0, 0), [3, 4])
            out(6, (1, 1), [0, 4], [2])

        for p in range(nq):
            flush(-(-count[0] // 4))
            quad(p)
        flush(nr)
        st_ref[0:8, :] = mr[save_st][0]
        st_ref[8:16, :] = mr[save_st][1]

    def wait_quads(ns):
        return lambda: [(cin_quad(n) if n < NH else cin(n // 2)).wait()
                        for n in ns]

    cin_quad(1).wait()
    run(0, FQ, range(1, FQ),
        {r: wait_quads(ns) for r, ns in _FIRST_WAITS.items()}, _FIRST_TASKS,
        {}, None, FQ + 3, {"N": 287, "S": 321}, 478, 96, 6.56, False)

    f = FQ // 2
    n_iter = (S - f) // 2
    j_flush = (DEFER - f) // 2
    bnd = [0, 17, 33, 49, 65]

    def write_part(half, cc):
        for k in range(2):
            cout(S - 1, half * H, (half + 1) * H, 4 + 2 * cc + k)

    def body(j, carry):
        s = f + 2 * j
        for t in (2, 3):
            @pl.when(s + t < S)
            def _():
                cin(jnp.minimum(s + t, S - 1)).wait()

        def write_prev(p):
            def fn():
                if p == 0:
                    @pl.when(j == j_flush)
                    def _():
                        for ct in range(8):
                            cout(pl.ds(0, DEFER), 0, D, ct)

                @pl.when(j > j_flush if p == 0 else j >= j_flush)
                def _():
                    cout_quad(s + (p - 1) // 2, (p - 1) % 2)
            return fn

        def write_last(half, cc):
            return lambda: pl.when(j == n_iter - 1)(
                lambda: write_part(half, cc))

        hooks = {(p, "m3"): write_prev(p) for p in range(4)}
        hooks.update({(3, "m2"): write_last(0, 1), (3, "m1"): write_last(1, 0),
                      (3, "m6"): write_last(0, 0)})
        tasks = []
        for p in range(4):
            tasks += [("N", p + 3, bnd[p], bnd[p + 1]),
                      ("S", p + 4, bnd[p], bnd[p + 1])]
        run(s, 4, (3,), {}, tasks, hooks, 3, 7, {"N": 0.01, "S": 0.01})
        return carry

    lax.fori_loop(0, n_iter, body, 0)
    write_part(1, 1)
    pltpu.make_async_copy(obuf, o_hbm, sout.at[0]).wait()


@jax.jit
def pallas_standalone__layernorm_linear__sampling_kernel(
    x: jax.Array,
    g: jax.Array,
    b: jax.Array,
    w: jax.Array,
):
    assert x.shape == (B, S, D) and w.shape == (D, D)
    xt = jnp.transpose(x, (1, 2, 0))
    out = pl.pallas_call(
        _kernel,
        in_specs=[pl.BlockSpec(memory_space=pl.ANY)] * 4,
        out_specs=pl.BlockSpec(memory_space=pl.ANY),
        out_shape=jax.ShapeDtypeStruct((S, D, B), x.dtype),
        scratch_shapes=[
            pltpu.VMEM((S, D, B), bf16),
            pltpu.VMEM((S, D, B), bf16),
        ] + [pltpu.VMEM((BROWS, W2), u32)] * 4
        + [pltpu.VMEM((H, W2), f32)] * 5
        + [
            pltpu.VMEM((16, W4), f32),
            pltpu.VMEM((D,), bf16),
            pltpu.VMEM((D,), bf16),
            pltpu.VMEM((D, D), bf16),
            pltpu.VMEM((7 * 72, 7 * PW), u32),
            pltpu.VMEM((144, W2), u32),
            pltpu.SMEM((4,), jnp.int32),
            pltpu.SemaphoreType.DMA((S + 3 + NH,)),
            pltpu.SemaphoreType.DMA((1,)),
        ],
        compiler_params=pltpu.CompilerParams(
            vmem_limit_bytes=110 * 1024 * 1024,
            disable_bounds_checks=True,
            disable_semaphore_checks=True,
        ),
    )(xt, g, b, w)
    return jnp.transpose(out, (2, 0, 1))
```

```python
import jax
import jax.numpy as jnp
from jax import lax
import jax.experimental.pallas as pl
import jax.experimental.pallas.tpu as pltpu

EPS = 1e-5
D = 576
S = 32
B = 1024
H = D // 2
Q = D // 4
KH = 256
KR = 80
PW = 128
W2 = 2 * PW
W4 = 4 * PW
NH = 10
FQ = 8
NI = 14
DEFER = 14
NPER = 18
SG = 36
f32 = jnp.float32
bf16 = jnp.bfloat16
u32 = jnp.uint32
cat = jnp.concatenate
PERM = (3, 5, 6, 7)
RROW = 28 * 64
BROWS = RROW + 80


def _sa(a11, a12, a21, a22):
    return [a11 + a22, a21 + a22, a11, a22, a11 + a12, a21 - a11, a12 - a22]


def _sb(b11, b12, b21, b22):
    return [b11 + b22, b11, b12 - b22, b21 - b11, b22, b11 + b12, b21 + b22]


def _ppos(i, j):
    return ((j - 1) * 4 + (i - 1) // 2) * 64, ((i - 1) % 2) * PW


def _rpos(ct):
    return RROW + (ct // 2) * 40, (ct % 2) * PW


_VT = [
    69, 74, 88, 142, 97, 108, 86, 159, 180, 74, 74, 71, 177, 165, 54, 224,
    205, 111, 54, 159, 110, 74, 73, 124, 197, 115, 102, 54, 173, 166, 75, 210,
    186, 112, 69, 140, 144, 74, 74, 122, 180, 98, 114, 61, 173, 181, 60, 206,
    202, 79, 73, 90, 160, 108, 108, 71, 196, 128, 74, 90, 53, 190, 169, 207,
    216]
_ST = [
    17, 54, 35, 55, 19, 52, 59, 40, 54, 18, 54, 10, 17, 19, 12, 21, 55, 56,
    23, 55, 39, 40, 41, 73, 53, 44, 56, 2, 16, 18, 12, 17, 19, 53, 56, 40, 54,
    19, 54, 59, 55, 20, 53, 20, 16, 18, 2, 16, 21, 40, 42, 54, 53, 43, 56, 43,
    53, 41, 45, 38, 9, 17, 46, 19, 18]
_TWEAK_N = [
    0.9253, 0.9354, 0.9478, 1.0229, 1.0795, 0.9303, 0.9248, 1.0735, 0.9475,
    1.073, 0.9784, 0.9462, 0.987, 1.0775, 1.0001, 1.0187, 0.9896, 0.9355,
    0.9913, 0.9862, 0.9478, 1.0335, 1.047, 1.0497, 0.9403, 1.0478, 1.0614,
    1.0101, 1.0771, 1.0353, 0.9234, 1.0758, 1.0599, 0.9549, 1.0484, 0.9912,
    1.0628, 0.9387, 0.9296, 1.0257, 0.9332, 1.0155, 1.0038, 0.9285, 0.9317,
    0.9624, 0.9289, 0.9468, 1.0386, 0.9667, 1.006, 1.0746, 0.9698, 1.0238,
    0.943, 0.9348, 1.027, 0.9221, 0.9333, 0.9957, 0.9775, 0.9369, 0.987,
    1.0613, 1.0794]
_TWEAK_S = [
    0.9577, 0.9269, 0.9884, 0.9264, 1.0386, 1.0098, 1.0269, 1.204, 0.9235,
    0.9502, 1.0472, 0.9905, 1.0602, 0.9279, 1.0287, 1.0749, 1.071, 0.9804,
    0.9234, 1.0212, 0.7479, 1.0026, 1.1669, 1.0276, 1.042, 0.9729, 0.9638,
    1.079, 1.0254, 0.9449, 1.0404, 0.9948, 1.0745, 1.063, 0.949, 0.9791,
    0.9723, 0.9943, 0.9771, 1.0036, 1.1351, 1.0379, 1.0337, 1.0467, 0.9334,
    1.0734, 1.003, 0.9499, 0.6706, 0.9401, 0.9814, 1.1228, 1.0367, 1.059,
    0.9422, 0.9378, 1.0647, 1.0284, 1.073, 0.946, 0.9292, 1.0732, 1.0415,
    1.0331, 0.994]
_NCOST = []
for _k in range(8):
    _NCOST += [43, 51, 51, 29, 21, 51, 29] + ([32] if _k % 2 == 0 else [])

_FIRST_WAITS = {17: (2, 3), 41: (4, 5, 6), 80: (7, 8, 9, 10)}
_FIRST_TASKS = [
    ("S", 1, 0, 4.56),
    ("N", 1, 4.56, 14.49),
    ("S", 2, 17, 19.92),
    ("N", 2, 19.92, 29.8276),
    ("S", 3, 19.92, 29.3276),
    ("N", 3, 29.8276, 41),
    ("S", 4, 41, 44.83),
    ("N", 4, 44.83, 56.55333),
    ("S", 5, 44.83, 56.55333),
    ("N", 5, 56.55333, 68.27667),
    ("S", 6, 56.55333, 68.27667),
    ("N", 6, 68.27667, 80),
    ("S", 7, 80, 84.1),
    ("N", 7, 84.1, 95.575),
    ("S", 8, 84.1, 95.575),
    ("N", 8, 95.575, 107.05),
    ("S", 9, 95.575, 107.05),
    ("N", 9, 107.05, 118.525),
    ("S", 10, 107.05, 118.525),
    ("N", 10, 118.525, 130.0),
    ("S", 11, 118.525, 130.0),
]

_ORDER = {
    ("put", 0): "m1 m2 m4 m6 m3 m5 m7",
    ("put", 1): "m1 m2 m4 m3 m5 m6 m7",
    ("put", 2): "m1 m6 m2 m3 m4 m5 m7",
    ("put", 3): "m2 m1 m3 m5 m6 m4 m7",
    ("sep", 0): "m1 m2 m4 m7 m3 m5 r11 r12 m6 r21 r22",
    ("sep", 1): "m1 m2 m4 m3 m6 r21 r22 m5 m7 r11 r12",
    ("sep", 2): "m3 m4 m1 m2 m6 r21 m5 m7 r11 r12 r22",
    ("sep", 3): "m3 m1 m2 m4 m6 m5 m7 r11 r12 r21 r22",
    ("merge", 0): "m3 m6 r12 r22 m1 m2 m4 r21 m5 m7 r11",
    ("merge", 1): "m3 m6 r22 m1 m2 m4 r21 m5 m7 r11 r12",
    ("merge", 2): "m6 r22 m4 m7 r11 r21 m1 m3 m5 r12 m2",
    ("merge", 3): "m1 m3 m6 r12 r22 m2 m4 m7 r21 m5 r11",
}
_TERMS = {"11": {"m1": 1, "m7": 1, "m5": -1, "m4": 1},
          "12": {"m3": 1, "m5": 1},
          "21": {"m2": 1, "m4": 1},
          "22": {"m1": 1, "m3": 1, "m6": 1, "m2": -1}}


def _stats_pair(x, gates):
    ng = len(gates) if gates else 18
    n = D // 8 // ng
    c = jnp.broadcast_to(x[0:1, :], (8, W2))
    a1 = a2 = None
    for k in range(ng):
        ck = gates[k](c, 2) if gates else c
        v = x[k * n * 8:(k + 1) * n * 8] - cat([ck] * n, axis=0)
        sq = v * v
        if a1 is not None:
            v = cat([a1, v], axis=0)
            sq = cat([a2, sq], axis=0)
        a1 = jnp.sum(v.reshape(-1, 8, W2), axis=0)
        a2 = jnp.sum(sq.reshape(-1, 8, W2), axis=0)
    a1 = jnp.sum(a1, axis=0, keepdims=True) * (1.0 / D)
    a2 = jnp.sum(a2, axis=0, keepdims=True) * (1.0 / D)
    m = c[0:1] + a1
    var = jnp.maximum(a2 - a1 * a1, 0.0)
    r = lax.rsqrt(var + EPS)
    return jnp.broadcast_to(m, (8, W2)), jnp.broadcast_to(r, (8, W2))


def _stats_quad(x, gates):
    h = len(gates) // 2
    ma, ra = _stats_pair(x[:, 0:W2], gates[:h])
    mb, rb = _stats_pair(x[:, W2:], gates[h:])
    return cat([ma, mb], axis=1), cat([ra, rb], axis=1)


def _norm_quad(x, m, r, p_ref, gates):
    def tiles(v, tc):
        return cat([v[:, tc * PW:(tc + 1) * PW],
                    v[:, (tc + 2) * PW:(tc + 3) * PW]], axis=1)

    def wide(v):
        return cat([cat([v, v], axis=1)] * 2, axis=0)

    xt = [tiles(x, 0), tiles(x, 1)]
    mt = [tiles(m, 0), tiles(m, 1)]
    rt = [wide(tiles(r, 0)), wide(tiles(r, 1))]
    r16 = cat([r, r], axis=0)
    it = iter(gates)

    def sub(k, kr, tc):
        g = next(it, None)
        mg = mt[tc] if g is None else g(mt[tc], 2)
        r0 = kr * 128 + k * 16
        xb = cat([xt[tc][r0:r0 + 16], xt[tc][KH + r0:KH + r0 + 16]], axis=1)
        return (xb - wide(mg)) * rt[tc]

    def emit(k, j, v, gate=False):
        q = [v[:, i * PW:(i + 1) * PW] for i in range(4)]
        g = next(it, None) if gate else None
        if g is not None:
            q[0] = g(q[0], 0)
            q[3] = g(q[3], 0)
        ops = _sb(*q)
        for i0 in range(0, 7, 2):
            grp = ops[i0:i0 + 2]
            r0 = _ppos(i0 + 1, j)[0] + k * 8
            p_ref[r0:r0 + 8, 0:len(grp) * PW] = pltpu.bitcast(
                cat(grp, axis=1).astype(bf16), u32)

    for k in range(8):
        b11 = sub(k, 0, 0)
        emit(k, 2, b11)
        b12 = sub(k, 0, 1)
        emit(k, 6, b11 + b12)
        b22 = sub(k, 1, 1)
        emit(k, 3, b12 - b22)
        emit(k, 1, b11 + b22, True)
        emit(k, 5, b22, True)
        b21 = sub(k, 1, 0)
        emit(k, 4, b21 - b11)
        emit(k, 7, b21 + b22, True)
        if k % 2 == 0:
            g = next(it, None)
            mg = m if g is None else g(m, 4)
            r0 = 2 * KH + k * 8
            v = (x[r0:r0 + 16] - cat([mg, mg], axis=0)) * r16
            for c0 in (0, 2):
                r1 = _rpos(c0)[0] + k * 4
                p_ref[r1:r1 + 8, :] = pltpu.bitcast(
                    v[:, c0 * PW:(c0 + 2) * PW].astype(bf16), u32)


def _kernel(x_hbm, g_hbm, b_hbm, w_hbm, o_hbm, xbuf, obuf,
            p0, p1, p2, p3, u0, u1, u2, u3, u4,
            st_ref, g_ref, b_ref, w_ref, a_ref, ar_ref, zs, sin, sout):
    ps = [p0, p1, p2, p3]
    us = [u0, u1, u2, u3, u4]
    for i in range(4):
        zs[i] = 0

    def cin_slab5():
        return pltpu.make_async_copy(x_hbm.at[5], xbuf.at[5], sin.at[NI])

    def cin_pair(j):
        rows = pl.ds(6 + 2 * j, 2)
        return pltpu.make_async_copy(x_hbm.at[rows], xbuf.at[rows], sin.at[j])

    def cin_quad(n):
        t, c = divmod(n, 2)
        return pltpu.make_async_copy(
            x_hbm.at[t, :, c * W4:(c + 1) * W4],
            xbuf.at[t, :, c * W4:(c + 1) * W4], sin.at[NI + 4 + n])

    def cout(sl, r0, r1, ct):
        idx = (sl, slice(r0, r1), slice(ct * PW, (ct + 1) * PW))
        pltpu.make_async_copy(
            obuf.at[idx], o_hbm.at[idx], sout.at[0]).start(priority=ct % 2)

    def cout_quad(t, c):
        for ct in range(4):
            cout(t, 0, D, 4 * c + ct)

    cw = pltpu.make_async_copy(w_hbm, w_ref, sin.at[NI + 1])
    cg = pltpu.make_async_copy(g_hbm, g_ref, sin.at[NI + 2])
    cb = pltpu.make_async_copy(b_hbm, b_ref, sin.at[NI + 3])
    cg.start()
    cb.start()
    cw.start()
    for n in range(NH):
        cin_quad(n).start()
    cin_slab5().start()
    for j in range(NI - 1):
        cin_pair(j).start()

    row16 = lax.broadcasted_iota(jnp.int32, (16, W2), 0)
    ones = pltpu.bitcast(jnp.where(row16 < 3, 1.0, 0.0).astype(bf16), u32)
    for p_ref in ps:
        for c0 in (0, 2):
            r1 = _rpos(c0)[0] + 32
            p_ref[r1:r1 + 8, :] = ones

    cg.wait()
    cb.wait()
    cw.wait()
    g = g_ref[...].astype(f32).reshape(1, D)
    w = w_ref[...]
    b16 = jnp.broadcast_to(b_ref[...].reshape(1, D), (16, D))
    bias = jnp.dot(b16, w, preferred_element_type=f32)[0:8]
    bh = bias.astype(bf16).astype(f32)
    bl = (bias - bh).astype(bf16).astype(f32)
    bl2 = bias - bh - bl
    row8 = lax.broadcasted_iota(jnp.int32, (8, D), 0)
    ext = jnp.where(row8 == 0, bh,
                    jnp.where(row8 == 1, bl, jnp.where(row8 == 2, bl2, 0.0)))
    wf = w.astype(f32)
    wr = cat([wf[2 * KH:], ext, jnp.zeros((56, D), f32)], axis=0)
    wg = wf[:2 * KH].T * g[:, :2 * KH]
    gr = cat([g[:, 2 * KH:], jnp.ones((1, 64), f32)], axis=1)
    a1 = _sa(wg[0:H, 0:KH], wg[0:H, KH:], wg[H:, 0:KH], wg[H:, KH:])
    for i in range(1, 8):
        top, bot = a1[i - 1][0:Q], a1[i - 1][Q:]
        if i in PERM:
            top, bot = bot, top
        a2 = _sa(top[:, 0:128], top[:, 128:], bot[:, 0:128], bot[:, 128:])
        a_ref[:, (i - 1) * PW:i * PW] = pltpu.bitcast(
            cat(a2, axis=0).astype(bf16), u32)
    arv = (wr.T * gr).astype(bf16)
    ar_ref[:, 0:PW] = pltpu.bitcast(arv[0:H], u32)
    ar_ref[:, PW:] = pltpu.bitcast(arv[H:], u32)

    cin_quad(0).wait()
    _norm_quad(xbuf[zs[2], :, 0:W4].astype(f32),
               *_stats_quad(xbuf[zs[0], :, 0:W4].astype(f32), []), ps[0], [])

    def run(s, nq, fresh, waits, tasks, hooks, have_st, save_st, bubble,
            valu=446, vst=99, ratio=6.89, tweak=True):
        k1 = s + zs[0]
        k2 = s + zs[2]
        never = {n: lax.broadcasted_iota(
            jnp.int32, (8, n * PW) if n else (16, PW), 0) < zs[1]
                 for n in (0, 2, 4)}
        zero = pl.multiple_of(zs[3], 8)
        nr = -(-65 * nq // 4)
        free = [max(valu - _VT[r % 65], 0) for r in range(nr)]
        tn = _TWEAK_N if tweak else [1] * 65
        ts = _TWEAK_S if tweak else [1] * 65
        wn = [(min(free[r], max(vst - _ST[r % 65], 0) * ratio) + 0.01)
              * tn[r % 65] for r in range(nr)]
        sc = sum(_NCOST) * nr / 16.25 / sum(wn)
        ws = [(max(free[r] - wn[r] * sc, 0) + 0.01) * ts[r % 65]
              for r in range(nr)]

        def xload(k, q):
            t, c = divmod(q, 2)
            return xbuf[jnp.minimum(k + t, S - 1), :,
                        c * W4:(c + 1) * W4].astype(f32)

        def make_gate(e):
            if e is None:
                return lambda v, n: v

            def gate(v, n):
                z = e[0][e[1]:e[1] + 8]
                z = cat([z] * n, axis=1) if n else cat([z, z], axis=0)
                return lax.select(never[n], z, v)
            return gate

        mr = {}
        if have_st is not None:
            mr[have_st] = (st_ref[0:8, :], st_ref[8:16, :])
        first = {}
        todo = list(tasks)

        def flush(now):
            for task in [t for t in todo if t[3] <= now + 1e-9]:
                todo.remove(task)
                kind, q, t0, t1 = task
                wt = wn if kind == "N" else ws
                cand = []
                a = 0.0
                if t0 == 0 or t0 in waits:
                    cand.append((0.0, None))
                    a += bubble[kind]
                for r in range(int(t0), nr):
                    for e in range(NPER):
                        if t0 - 1e-9 <= r + e / NPER < t1 - 1e-9:
                            cand.append(
                                (a, (first[r], Q * e // NPER // 8 * 8)))
                            a += wt[r] / NPER
                costs = _NCOST if kind == "N" else [1] * (2 * SG)
                done = 0
                gates = []
                for x in costs:
                    tgt = a * done / sum(costs)
                    gates.append(make_gate(
                        [e for (c, e) in cand if c <= tgt + 1e-9][-1]))
                    done += x
                if kind == "N":
                    _norm_quad(xload(k2, q), *mr.pop(q), ps[q % 4], gates)
                else:
                    mr[q] = _stats_quad(xload(k1, q), gates)

        count = [0]

        def mxu(lhs, rhs):
            r, o = divmod(count[0], 4)
            if o == 0 and r in waits:
                flush(r)
                waits[r]()
            v = jnp.dot(lhs(), rhs(), preferred_element_type=f32)
            if o == 0:
                first[r] = v
            count[0] += 1
            return v

        def get(i):
            return us[i][pl.ds(zero, H), :]

        def quad(p):
            sl = s + p // 2
            c0 = (p % 2) * W4
            p_ref = ps[p % 4]
            if p in fresh:
                p_ref = p_ref.at[pl.ds(zero, BROWS), :]

            def hook(name):
                if (p, name) in hooks:
                    hooks[(p, name)]()

            def dot(i, j):
                r1, c1 = _ppos(i, j)
                return mxu(
                    lambda: pltpu.bitcast(
                        a_ref[(j - 1) * 72:j * 72, (i - 1) * PW:i * PW], bf16),
                    lambda: pltpu.bitcast(
                        p_ref[r1:r1 + 64, c1:c1 + PW], bf16))

            def rem(half, cc, hr, hc):
                r1, c1 = _rpos(2 * cc + hc)
                return mxu(
                    lambda: pltpu.bitcast(
                        ar_ref[hr * 72:(hr + 1) * 72,
                               half * PW:(half + 1) * PW], bf16)[:, :KR],
                    lambda: pltpu.bitcast(
                        p_ref[r1:r1 + 40, c1:c1 + PW], bf16))

            def prod(i, o=None):
                sw = 1 if i in PERM else 0

                def blk(c):
                    rows = [cat([c["11"], c["12"]], axis=1),
                            cat([c["21"], c["22"]], axis=1)]
                    return cat(rows[::-1] if sw else rows, axis=0)

                kind = "sep" if i in (4, 5) else "merge" if o else "put"
                acc = {}
                sign = {}
                sep = {}
                for nm in _ORDER[(kind, count[0] % 4)].split():
                    if nm[0] == "m":
                        v = dot(i, int(nm[1]))
                    else:
                        v = rem(o[0], o[1], (int(nm[1]) - 1) ^ sw,
                                int(nm[2]) - 1)
                        sep[nm[1:]] = v
                    for k, terms in _TERMS.items():
                        sg = terms.get(nm)
                        if kind == "merge" and nm == "r" + k:
                            sg = 1
                        if sg is None:
                            continue
                        if k not in acc:
                            acc[k], sign[k] = v, sg
                        elif sign[k] < 0:
                            acc[k], sign[k] = v - acc[k], 1
                        else:
                            acc[k] = acc[k] + v if sg > 0 else acc[k] - v
                return blk(acc), blk(sep) if kind == "sep" else None

            def out(i, o, plus, minus=()):
                val, v = prod(i, o)
                if o == (1, 1):
                    hook("m6")
                v = val if v is None else val + v
                for u in plus:
                    v = v + get(u)
                for u in minus:
                    v = v - get(u)
                obuf[sl, o[0] * H:(o[0] + 1) * H,
                     c0 + o[1] * W2:c0 + (o[1] + 1) * W2] = v.astype(bf16)
                return val

            us[0][...] = prod(3)[0]
            hook("m3")
            us[1][...] = out(5, (0, 1), [0])
            us[2][...] = prod(2)[0]
            hook("m2")
            m4 = out(4, (1, 0), [2])
            us[3][...] = m4 - get(1)
            us[4][...] = prod(1)[0]
            hook("m1")
            out(7, (0, 0), [3, 4])
            out(6, (1, 1), [0, 4], [2])

        for p in range(nq):
            flush(-(-count[0] // 4))
            quad(p)
        flush(nr)
        st_ref[0:8, :] = mr[save_st][0]
        st_ref[8:16, :] = mr[save_st][1]

    def wait_quads(ns):
        return lambda: [(cin_quad(n) if n < NH else cin_slab5()).wait()
                        for n in ns]

    cin_quad(1).wait()
    run(0, FQ, range(1, FQ),
        {r: wait_quads(ns) for r, ns in _FIRST_WAITS.items()}, _FIRST_TASKS,
        {}, None, FQ + 3, {"N": 287, "S": 321}, 478, 96, 6.56, False)

    f = FQ // 2
    j_flush = (DEFER - f) // 2
    bnd = [0, 17, 33, 49, 65]

    def write_part(half, cc):
        for k in range(2):
            cout(S - 1, half * H, (half + 1) * H, 4 + 2 * cc + k)

    def body(j, carry):
        s = f + 2 * j

        @pl.when(j < NI - 1)
        def _():
            cin_pair(j).wait()

        def write_prev(p):
            def fn():
                if p == 0:
                    @pl.when(j == j_flush)
                    def _():
                        for ct in range(8):
                            cout(pl.ds(0, DEFER), 0, D, ct)

                @pl.when(j > j_flush if p == 0 else j >= j_flush)
                def _():
                    cout_quad(s + (p - 1) // 2, (p - 1) % 2)
            return fn

        def write_last(half, cc):
            return lambda: pl.when(j == NI - 1)(
                lambda: write_part(half, cc))

        hooks = {(p, "m3"): write_prev(p) for p in range(4)}
        hooks.update({(3, "m2"): write_last(0, 1), (3, "m1"): write_last(1, 0),
                      (3, "m6"): write_last(0, 0)})
        tasks = []
        for p in range(4):
            tasks += [("N", p + 3, bnd[p], bnd[p + 1]),
                      ("S", p + 4, bnd[p], bnd[p + 1])]
        run(s, 4, (3,), {}, tasks, hooks, 3, 7, {"N": 0.01, "S": 0.01})
        return carry

    lax.fori_loop(0, NI, body, 0)
    write_part(1, 1)
    pltpu.make_async_copy(obuf, o_hbm, sout.at[0]).wait()


@jax.jit
def pallas_standalone__layernorm_linear__sampling_kernel(
    x: jax.Array,
    g: jax.Array,
    b: jax.Array,
    w: jax.Array,
):
    assert x.shape == (B, S, D) and w.shape == (D, D)
    xt = jnp.transpose(x, (1, 2, 0))
    out = pl.pallas_call(
        _kernel,
        in_specs=[pl.BlockSpec(memory_space=pl.ANY)] * 4,
        out_specs=pl.BlockSpec(memory_space=pl.ANY),
        out_shape=jax.ShapeDtypeStruct((S, D, B), x.dtype),
        scratch_shapes=[
            pltpu.VMEM((S, D, B), bf16),
            pltpu.VMEM((S, D, B), bf16),
        ] + [pltpu.VMEM((BROWS, W2), u32)] * 4
        + [pltpu.VMEM((H, W2), f32)] * 5
        + [
            pltpu.VMEM((16, W4), f32),
            pltpu.VMEM((D,), bf16),
            pltpu.VMEM((D,), bf16),
            pltpu.VMEM((D, D), bf16),
            pltpu.VMEM((7 * 72, 7 * PW), u32),
            pltpu.VMEM((144, W2), u32),
            pltpu.SMEM((4,), jnp.int32),
            pltpu.SemaphoreType.DMA((NI + 4 + NH,)),
            pltpu.SemaphoreType.DMA((1,)),
        ],
        compiler_params=pltpu.CompilerParams(
            vmem_limit_bytes=110 * 1024 * 1024,
            disable_bounds_checks=True,
            disable_semaphore_checks=True,
        ),
    )(xt, g, b, w)
    return jnp.transpose(out, (2, 0, 1))
```

```python
import jax
import jax.numpy as jnp
from jax import lax
import jax.experimental.pallas as pl
import jax.experimental.pallas.tpu as pltpu

EPS = 1e-5
D = 576
S = 32
B = 1024
H = D // 2
Q = D // 4
KH = 256
KR = 80
PW = 128
W2 = 2 * PW
W4 = 4 * PW
NH = 10
FQ = 8
NI = 14
DEFER = 14
NPER = 18
SG = 36
f32 = jnp.float32
bf16 = jnp.bfloat16
u32 = jnp.uint32
cat = jnp.concatenate
PERM = (3, 5, 6, 7)
RROW = 28 * 64
BROWS = RROW + 80


def _sa(a11, a12, a21, a22):
    return [a11 + a22, a21 + a22, a11, a22, a11 + a12, a21 - a11, a12 - a22]


def _sb(b11, b12, b21, b22):
    return [b11 + b22, b11, b12 - b22, b21 - b11, b22, b11 + b12, b21 + b22]


def _ppos(i, j):
    return ((j - 1) * 4 + (i - 1) // 2) * 64, ((i - 1) % 2) * PW


def _rpos(ct):
    return RROW + (ct // 2) * 40, (ct % 2) * PW


_VT = [
    69, 74, 88, 142, 97, 108, 86, 159, 180, 74, 74, 71, 177, 165, 54, 224,
    205, 111, 54, 159, 110, 74, 73, 124, 197, 115, 102, 54, 173, 166, 75, 210,
    186, 112, 69, 140, 144, 74, 74, 122, 180, 98, 114, 61, 173, 181, 60, 206,
    202, 79, 73, 90, 160, 108, 108, 71, 196, 128, 74, 90, 53, 190, 169, 207,
    216]
_ST = [
    17, 54, 35, 55, 19, 52, 59, 40, 54, 18, 54, 10, 17, 19, 12, 21, 55, 56,
    23, 55, 39, 40, 41, 73, 53, 44, 56, 2, 16, 18, 12, 17, 19, 53, 56, 40, 54,
    19, 54, 59, 55, 20, 53, 20, 16, 18, 2, 16, 21, 40, 42, 54, 53, 43, 56, 43,
    53, 41, 45, 38, 9, 17, 46, 19, 18]
_TWEAK_N = [
    0.9253, 0.9354, 0.9478, 0.941, 1.0795, 0.9303, 0.9248, 1.0735, 0.9475,
    1.073, 0.9784, 0.9462, 0.987, 1.0775, 1.0001, 1.0187, 0.9896, 0.9355,
    0.9913, 0.9862, 0.9478, 1.0335, 1.047, 1.0497, 0.9403, 1.0478, 1.0614,
    1.0101, 1.0771, 1.0353, 0.9234, 1.0758, 1.0599, 0.9549, 1.0484, 0.9912,
    1.0628, 0.9387, 0.9296, 1.0257, 0.9332, 1.0155, 1.0038, 0.9285, 0.9317,
    0.9624, 0.9289, 0.8593, 1.0386, 0.9667, 1.006, 1.0746, 0.9698, 1.0238,
    0.943, 0.9348, 1.027, 0.9221, 0.9333, 0.9957, 0.9775, 0.9395, 0.987,
    1.0613, 1.0794]
_TWEAK_S = [
    0.9577, 0.9269, 0.9884, 0.9399, 1.0151, 1.0098, 1.0697, 1.204, 1.0286,
    0.9502, 1.0472, 0.9905, 1.0602, 0.9279, 1.0266, 1.0749, 1.071, 0.9804,
    0.9234, 1.0212, 0.7479, 1.0026, 1.1669, 1.0276, 1.042, 1.0388, 0.9646,
    1.079, 1.0254, 0.9449, 1.0404, 0.9948, 1.0745, 1.063, 0.9523, 0.9791,
    0.9723, 0.9943, 0.9771, 1.0036, 1.1351, 1.0379, 1.0337, 1.0467, 0.9334,
    1.0734, 1.003, 0.9499, 0.6706, 0.9401, 0.9814, 1.1229, 1.0297, 1.059,
    0.9422, 0.8877, 1.0647, 1.0284, 1.073, 0.946, 0.9292, 1.0732, 1.0415,
    1.0331, 0.994]
_NCOST = []
for _k in range(8):
    _NCOST += [43, 51, 51, 29, 21, 51, 29] + ([32] if _k % 2 == 0 else [])

_FIRST_WAITS = {17: (2, 3), 41: (4, 5, 6), 80: (7, 8, 9, 10)}
_FIRST_TASKS = [
    ("S", 1, 0, 4.56),
    ("N", 1, 4.56, 14.49),
    ("S", 2, 17, 19.92),
    ("N", 2, 19.92, 29.8276),
    ("S", 3, 19.92, 29.3276),
    ("N", 3, 29.8276, 41),
    ("S", 4, 41, 44.83),
    ("N", 4, 44.83, 56.55333),
    ("S", 5, 44.83, 56.55333),
    ("N", 5, 56.55333, 68.27667),
    ("S", 6, 56.55333, 68.27667),
    ("N", 6, 68.27667, 80),
    ("S", 7, 80, 84.1),
    ("N", 7, 84.1, 95.575),
    ("S", 8, 84.1, 95.575),
    ("N", 8, 95.575, 107.05),
    ("S", 9, 95.575, 107.05),
    ("N", 9, 107.05, 118.525),
    ("S", 10, 107.05, 118.525),
    ("N", 10, 118.525, 130.0),
    ("S", 11, 118.525, 130.0),
]

_ORDER = {
    ("put", 0): "m1 m2 m4 m6 m3 m5 m7",
    ("put", 1): "m1 m2 m4 m3 m5 m6 m7",
    ("put", 2): "m1 m6 m2 m3 m4 m5 m7",
    ("put", 3): "m2 m1 m3 m5 m6 m4 m7",
    ("sep", 0): "m1 m2 m4 m7 m3 m5 r11 r12 m6 r21 r22",
    ("sep", 1): "m1 m2 m4 m3 m6 r21 r22 m5 m7 r11 r12",
    ("sep", 2): "m3 m4 m1 m2 m6 r21 m5 m7 r11 r12 r22",
    ("sep", 3): "m3 m1 m2 m4 m6 m5 m7 r11 r12 r21 r22",
    ("merge", 0): "m3 m6 r12 r22 m1 m2 m4 r21 m5 m7 r11",
    ("merge", 1): "m3 m6 r22 m1 m2 m4 r21 m5 m7 r11 r12",
    ("merge", 2): "m6 r22 m4 m7 r11 r21 m1 m3 m5 r12 m2",
    ("merge", 3): "m1 m3 m6 r12 r22 m2 m4 m7 r21 m5 r11",
    ("early", 3): "m3 m1 m2 m4 m6 m5 m7",
}
_TERMS = {"11": {"m1": 1, "m7": 1, "m5": -1, "m4": 1},
          "12": {"m3": 1, "m5": 1},
          "21": {"m2": 1, "m4": 1},
          "22": {"m1": 1, "m3": 1, "m6": 1, "m2": -1}}


def _stats_pair(x, gates):
    ng = len(gates) if gates else 18
    n = D // 8 // ng
    c = jnp.broadcast_to(x[0:1, :], (8, W2))
    a1 = a2 = None
    for k in range(ng):
        ck = gates[k](c, 2) if gates else c
        v = x[k * n * 8:(k + 1) * n * 8] - cat([ck] * n, axis=0)
        sq = v * v
        if a1 is not None:
            v = cat([a1, v], axis=0)
            sq = cat([a2, sq], axis=0)
        a1 = jnp.sum(v.reshape(-1, 8, W2), axis=0)
        a2 = jnp.sum(sq.reshape(-1, 8, W2), axis=0)
    a1 = jnp.sum(a1, axis=0, keepdims=True) * (1.0 / D)
    a2 = jnp.sum(a2, axis=0, keepdims=True) * (1.0 / D)
    m = c[0:1] + a1
    var = jnp.maximum(a2 - a1 * a1, 0.0)
    r = lax.rsqrt(var + EPS)
    return jnp.broadcast_to(m, (8, W2)), jnp.broadcast_to(r, (8, W2))


def _stats_quad(x, gates):
    h = len(gates) // 2
    ma, ra = _stats_pair(x[:, 0:W2], gates[:h])
    mb, rb = _stats_pair(x[:, W2:], gates[h:])
    return cat([ma, mb], axis=1), cat([ra, rb], axis=1)


def _norm_quad(x, m, r, p_ref, gates):
    def tiles(v, tc):
        return cat([v[:, tc * PW:(tc + 1) * PW],
                    v[:, (tc + 2) * PW:(tc + 3) * PW]], axis=1)

    def wide(v):
        return cat([cat([v, v], axis=1)] * 2, axis=0)

    xt = [tiles(x, 0), tiles(x, 1)]
    mt = [tiles(m, 0), tiles(m, 1)]
    rt = [wide(tiles(r, 0)), wide(tiles(r, 1))]
    r16 = cat([r, r], axis=0)
    it = iter(gates)

    def sub(k, kr, tc):
        g = next(it, None)
        mg = mt[tc] if g is None else g(mt[tc], 2)
        r0 = kr * 128 + k * 16
        xb = cat([xt[tc][r0:r0 + 16], xt[tc][KH + r0:KH + r0 + 16]], axis=1)
        return (xb - wide(mg)) * rt[tc]

    def emit(k, j, v, gate=False):
        q = [v[:, i * PW:(i + 1) * PW] for i in range(4)]
        g = next(it, None) if gate else None
        if g is not None:
            q[0] = g(q[0], 0)
            q[3] = g(q[3], 0)
        ops = _sb(*q)
        for i0 in range(0, 7, 2):
            grp = ops[i0:i0 + 2]
            r0 = _ppos(i0 + 1, j)[0] + k * 8
            p_ref[r0:r0 + 8, 0:len(grp) * PW] = pltpu.bitcast(
                cat(grp, axis=1).astype(bf16), u32)

    for k in range(8):
        b11 = sub(k, 0, 0)
        emit(k, 2, b11)
        b12 = sub(k, 0, 1)
        emit(k, 6, b11 + b12)
        b22 = sub(k, 1, 1)
        emit(k, 3, b12 - b22)
        emit(k, 1, b11 + b22, True)
        emit(k, 5, b22, True)
        b21 = sub(k, 1, 0)
        emit(k, 4, b21 - b11)
        emit(k, 7, b21 + b22, True)
        if k % 2 == 0:
            g = next(it, None)
            mg = m if g is None else g(m, 4)
            r0 = 2 * KH + k * 8
            v = (x[r0:r0 + 16] - cat([mg, mg], axis=0)) * r16
            for c0 in (0, 2):
                r1 = _rpos(c0)[0] + k * 4
                p_ref[r1:r1 + 8, :] = pltpu.bitcast(
                    v[:, c0 * PW:(c0 + 2) * PW].astype(bf16), u32)


def _kernel(x_hbm, g_hbm, b_hbm, w_hbm, o_hbm, xbuf, obuf,
            p0, p1, p2, p3, u0, u1, u2, u3, u4,
            st_ref, g_ref, b_ref, w_ref, a_ref, ar_ref, zs, sin, sout):
    ps = [p0, p1, p2, p3]
    us = [u0, u1, u2, u3, u4]
    for i in range(4):
        zs[i] = 0

    def cin_slab5():
        return pltpu.make_async_copy(x_hbm.at[5], xbuf.at[5], sin.at[NI])

    def cin_pair(j):
        rows = pl.ds(6 + 2 * j, 2)
        return pltpu.make_async_copy(x_hbm.at[rows], xbuf.at[rows], sin.at[j])

    def cin_quad(n):
        t, c = divmod(n, 2)
        return pltpu.make_async_copy(
            x_hbm.at[t, :, c * W4:(c + 1) * W4],
            xbuf.at[t, :, c * W4:(c + 1) * W4], sin.at[NI + 4 + n])

    def cout(sl, r0, r1, ct):
        idx = (sl, slice(r0, r1), slice(ct * PW, (ct + 1) * PW))
        pltpu.make_async_copy(
            obuf.at[idx], o_hbm.at[idx], sout.at[0]).start(priority=ct % 2)

    def cout_quad(t, c):
        for ct in range(4):
            cout(t, 0, D, 4 * c + ct)

    cw = pltpu.make_async_copy(w_hbm, w_ref, sin.at[NI + 1])
    cg = pltpu.make_async_copy(g_hbm, g_ref, sin.at[NI + 2])
    cb = pltpu.make_async_copy(b_hbm, b_ref, sin.at[NI + 3])
    cg.start()
    cb.start()
    cw.start()
    for n in range(NH):
        cin_quad(n).start()
    cin_slab5().start()
    for j in range(NI - 1):
        cin_pair(j).start()

    row16 = lax.broadcasted_iota(jnp.int32, (16, W2), 0)
    ones = pltpu.bitcast(jnp.where(row16 < 3, 1.0, 0.0).astype(bf16), u32)
    for p_ref in ps:
        for c0 in (0, 2):
            r1 = _rpos(c0)[0] + 32
            p_ref[r1:r1 + 8, :] = ones

    cg.wait()
    cb.wait()
    cw.wait()
    g = g_ref[...].astype(f32).reshape(1, D)
    w = w_ref[...]
    b16 = jnp.broadcast_to(b_ref[...].reshape(1, D), (16, D))
    bias = jnp.dot(b16, w, preferred_element_type=f32)[0:8]
    bh = bias.astype(bf16).astype(f32)
    bl = (bias - bh).astype(bf16).astype(f32)
    bl2 = bias - bh - bl
    row8 = lax.broadcasted_iota(jnp.int32, (8, D), 0)
    ext = jnp.where(row8 == 0, bh,
                    jnp.where(row8 == 1, bl, jnp.where(row8 == 2, bl2, 0.0)))
    wf = w.astype(f32)
    wr = cat([wf[2 * KH:], ext, jnp.zeros((56, D), f32)], axis=0)
    wg = wf[:2 * KH].T * g[:, :2 * KH]
    gr = cat([g[:, 2 * KH:], jnp.ones((1, 64), f32)], axis=1)
    a1 = _sa(wg[0:H, 0:KH], wg[0:H, KH:], wg[H:, 0:KH], wg[H:, KH:])
    for i in range(1, 8):
        top, bot = a1[i - 1][0:Q], a1[i - 1][Q:]
        if i in PERM:
            top, bot = bot, top
        a2 = _sa(top[:, 0:128], top[:, 128:], bot[:, 0:128], bot[:, 128:])
        a_ref[:, (i - 1) * PW:i * PW] = pltpu.bitcast(
            cat(a2, axis=0).astype(bf16), u32)
    arv = (wr.T * gr).astype(bf16)
    ar_ref[:, 0:PW] = pltpu.bitcast(arv[0:H], u32)
    ar_ref[:, PW:] = pltpu.bitcast(arv[H:], u32)

    cin_quad(0).wait()
    _norm_quad(xbuf[zs[2], :, 0:W4].astype(f32),
               *_stats_quad(xbuf[zs[0], :, 0:W4].astype(f32), []), ps[0], [])

    def run(s, nq, fresh, waits, tasks, hooks, have_st, save_st, bubble,
            valu=446, vst=99, ratio=6.89, tweak=True):
        k1 = s + zs[0]
        k2 = s + zs[2]
        never = {n: lax.broadcasted_iota(
            jnp.int32, (8, n * PW) if n else (16, PW), 0) < zs[1]
                 for n in (0, 2, 4)}
        zero = pl.multiple_of(zs[3], 8)
        nr = -(-65 * nq // 4)
        free = [max(valu - _VT[r % 65], 0) for r in range(nr)]
        tn = _TWEAK_N if tweak else [1] * 65
        ts = _TWEAK_S if tweak else [1] * 65
        wn = [(min(free[r], max(vst - _ST[r % 65], 0) * ratio) + 0.01)
              * tn[r % 65] for r in range(nr)]
        sc = sum(_NCOST) * nr / 16.25 / sum(wn)
        ws = [(max(free[r] - wn[r] * sc, 0) + 0.01) * ts[r % 65]
              for r in range(nr)]

        def xload(k, q):
            t, c = divmod(q, 2)
            return xbuf[jnp.minimum(k + t, S - 1), :,
                        c * W4:(c + 1) * W4].astype(f32)

        def make_gate(e):
            if e is None:
                return lambda v, n: v

            def gate(v, n):
                z = e[0][e[1]:e[1] + 8]
                z = cat([z] * n, axis=1) if n else cat([z, z], axis=0)
                return lax.select(never[n], z, v)
            return gate

        mr = {}
        if have_st is not None:
            mr[have_st] = (st_ref[0:8, :], st_ref[8:16, :])
        first = {}
        todo = list(tasks)

        def flush(now):
            for task in [t for t in todo if t[3] <= now + 1e-9]:
                todo.remove(task)
                kind, q, t0, t1 = task
                wt = wn if kind == "N" else ws
                cand = []
                a = 0.0
                if t0 == 0 or t0 in waits:
                    cand.append((0.0, None))
                    a += bubble[kind]
                for r in range(int(t0), nr):
                    for e in range(NPER):
                        if t0 - 1e-9 <= r + e / NPER < t1 - 1e-9:
                            cand.append(
                                (a, (first[r], Q * e // NPER // 8 * 8)))
                            a += wt[r] / NPER
                costs = _NCOST if kind == "N" else [1] * (2 * SG)
                done = 0
                gates = []
                for x in costs:
                    tgt = a * done / sum(costs)
                    gates.append(make_gate(
                        [e for (c, e) in cand if c <= tgt + 1e-9][-1]))
                    done += x
                if kind == "N":
                    _norm_quad(xload(k2, q), *mr.pop(q), ps[q % 4], gates)
                else:
                    mr[q] = _stats_quad(xload(k1, q), gates)

        count = [0]

        def mxu(lhs, rhs):
            r, o = divmod(count[0], 4)
            if o == 0 and r in waits:
                flush(r)
                waits[r]()
            v = jnp.dot(lhs(), rhs(), preferred_element_type=f32)
            if o == 0:
                first[r] = v
            count[0] += 1
            return v

        def get(i):
            return us[i][pl.ds(zero, H), :]

        def get_sub(i, hr, hc):
            return us[i][pl.ds(pl.multiple_of(zero + hr * Q, 8), Q),
                         hc * PW:(hc + 1) * PW]

        def quad(p):
            sl = s + p // 2
            c0 = (p % 2) * W4
            p_ref = ps[p % 4]
            if p in fresh:
                p_ref = p_ref.at[pl.ds(zero, BROWS), :]

            def hook(name):
                if (p, name) in hooks:
                    hooks[(p, name)]()

            def dot(i, j):
                r1, c1 = _ppos(i, j)
                return mxu(
                    lambda: pltpu.bitcast(
                        a_ref[(j - 1) * 72:j * 72, (i - 1) * PW:i * PW], bf16),
                    lambda: pltpu.bitcast(
                        p_ref[r1:r1 + 64, c1:c1 + PW], bf16))

            def rem(half, cc, hr, hc):
                r1, c1 = _rpos(2 * cc + hc)
                return mxu(
                    lambda: pltpu.bitcast(
                        ar_ref[hr * 72:(hr + 1) * 72,
                               half * PW:(half + 1) * PW], bf16)[:, :KR],
                    lambda: pltpu.bitcast(
                        p_ref[r1:r1 + 40, c1:c1 + PW], bf16))

            def prod(i, o=None, sep=None, plus=(), minus=()):
                sw = 1 if i in PERM else 0

                def blk(c):
                    rows = [cat([c["11"], c["12"]], axis=1),
                            cat([c["21"], c["22"]], axis=1)]
                    return cat(rows[::-1] if sw else rows, axis=0)

                kind = "sep" if i in (4, 5) else "merge" if o else "put"
                seq = _ORDER[("early" if sep else kind, count[0] % 4)].split()
                acc = {}
                sign = {}
                sep = dict(sep or {})
                for n, nm in enumerate(seq):
                    if nm[0] == "m":
                        v = dot(i, int(nm[1]))
                    else:
                        v = rem(o[0], o[1], (int(nm[1]) - 1) ^ sw,
                                int(nm[2]) - 1)
                        sep[nm[1:]] = v
                    for k, terms in _TERMS.items():
                        sg = terms.get(nm)
                        if kind == "merge" and nm == "r" + k:
                            sg = 1
                        if sg is None:
                            continue
                        if k not in acc:
                            acc[k], sign[k] = v, sg
                        elif sign[k] < 0:
                            acc[k], sign[k] = v - acc[k], 1
                        else:
                            acc[k] = acc[k] + v if sg > 0 else acc[k] - v
                    if plus and n == len(seq) - 5:
                        for k in _TERMS:
                            hr, hc = (int(k[0]) - 1) ^ sw, int(k[1]) - 1
                            for u in plus:
                                acc[k] = acc[k] + get_sub(u, hr, hc)
                            for u in minus:
                                acc[k] = acc[k] - get_sub(u, hr, hc)
                return blk(acc), blk(sep) if kind == "sep" else None

            def out(i, o, plus, minus=(), sep=None):
                if i == 6 and p == nq - 1:
                    val, v = prod(i, o, None, plus, minus)
                    plus = minus = ()
                else:
                    val, v = prod(i, o, sep)
                if o == (1, 1):
                    hook("m6")
                v = val if v is None else val + v
                for u in plus:
                    v = v + get(u)
                for u in minus:
                    v = v - get(u)
                obuf[sl, o[0] * H:(o[0] + 1) * H,
                     c0 + o[1] * W2:c0 + (o[1] + 1) * W2] = v.astype(bf16)
                return val

            early = None
            if p == 0:
                early = {k: rem(0, 1, (int(k[0]) - 1) ^ 1, int(k[1]) - 1)
                         for k in _TERMS}
            us[0][...] = prod(3)[0]
            hook("m3")
            us[1][...] = out(5, (0, 1), [0], sep=early)
            us[2][...] = prod(2)[0]
            hook("m2")
            m4 = out(4, (1, 0), [2])
            us[3][...] = m4 - get(1)
            us[4][...] = prod(1)[0]
            hook("m1")
            out(7, (0, 0), [3, 4])
            out(6, (1, 1), [0, 4], [2])

        for p in range(nq):
            flush(-(-count[0] // 4))
            quad(p)
        flush(nr)
        st_ref[0:8, :] = mr[save_st][0]
        st_ref[8:16, :] = mr[save_st][1]

    def wait_quads(ns):
        return lambda: [(cin_quad(n) if n < NH else cin_slab5()).wait()
                        for n in ns]

    cin_quad(1).wait()
    run(0, FQ, range(1, FQ),
        {r: wait_quads(ns) for r, ns in _FIRST_WAITS.items()}, _FIRST_TASKS,
        {}, None, FQ + 3, {"N": 287, "S": 321}, 478, 96, 6.56, False)

    f = FQ // 2
    j_flush = (DEFER - f) // 2
    bnd = [0, 17, 33, 49, 65]

    def write_part(half, cc):
        for k in range(2):
            cout(S - 1, half * H, (half + 1) * H, 4 + 2 * cc + k)

    def body(j, carry):
        s = f + 2 * j

        @pl.when(j < NI - 1)
        def _():
            cin_pair(j).wait()

        def write_prev(p):
            def fn():
                if p == 0:
                    @pl.when(j == j_flush)
                    def _():
                        for ct in range(8):
                            cout(pl.ds(0, DEFER), 0, D, ct)

                @pl.when(j > j_flush if p == 0 else j >= j_flush)
                def _():
                    cout_quad(s + (p - 1) // 2, (p - 1) % 2)
            return fn

        def write_last(half, cc):
            return lambda: pl.when(j == NI - 1)(
                lambda: write_part(half, cc))

        hooks = {(p, "m3"): write_prev(p) for p in range(4)}
        hooks.update({(3, "m2"): write_last(0, 1), (3, "m1"): write_last(1, 0),
                      (3, "m6"): write_last(0, 0)})
        tasks = []
        for p in range(4):
            tasks += [("N", p + 3, bnd[p], bnd[p + 1]),
                      ("S", p + 4, bnd[p], bnd[p + 1])]
        run(s, 4, (3,), {}, tasks, hooks, 3, 7, {"N": 0.01, "S": 0.01})
        return carry

    lax.fori_loop(0, NI, body, 0)
    write_part(1, 1)
    pltpu.make_async_copy(obuf, o_hbm, sout.at[0]).wait()


@jax.jit
def pallas_standalone__layernorm_linear__sampling_kernel(
    x: jax.Array,
    g: jax.Array,
    b: jax.Array,
    w: jax.Array,
):
    assert x.shape == (B, S, D) and w.shape == (D, D)
    xt = jnp.transpose(x, (1, 2, 0))
    out = pl.pallas_call(
        _kernel,
        in_specs=[pl.BlockSpec(memory_space=pl.ANY)] * 4,
        out_specs=pl.BlockSpec(memory_space=pl.ANY),
        out_shape=jax.ShapeDtypeStruct((S, D, B), x.dtype),
        scratch_shapes=[
            pltpu.VMEM((S, D, B), bf16),
            pltpu.VMEM((S, D, B), bf16),
        ] + [pltpu.VMEM((BROWS, W2), u32)] * 4
        + [pltpu.VMEM((H, W2), f32)] * 5
        + [
            pltpu.VMEM((16, W4), f32),
            pltpu.VMEM((D,), bf16),
            pltpu.VMEM((D,), bf16),
            pltpu.VMEM((D, D), bf16),
            pltpu.VMEM((7 * 72, 7 * PW), u32),
            pltpu.VMEM((144, W2), u32),
            pltpu.SMEM((4,), jnp.int32),
            pltpu.SemaphoreType.DMA((NI + 4 + NH,)),
            pltpu.SemaphoreType.DMA((1,)),
        ],
        compiler_params=pltpu.CompilerParams(
            vmem_limit_bytes=110 * 1024 * 1024,
            disable_bounds_checks=True,
            disable_semaphore_checks=True,
        ),
    )(xt, g, b, w)
    return jnp.transpose(out, (2, 0, 1))
```

```python
import jax
import jax.numpy as jnp
from jax import lax
import jax.experimental.pallas as pl
import jax.experimental.pallas.tpu as pltpu

EPS = 1e-5
D = 576
S = 32
B = 1024
H = D // 2
Q = D // 4
KH = 256
KR = 80
PW = 128
W2 = 2 * PW
W4 = 4 * PW
NH = 10
FQ = 8
NI = 14
DEFER = 14
NPER = 18
SG = 36
f32 = jnp.float32
bf16 = jnp.bfloat16
u32 = jnp.uint32
cat = jnp.concatenate
PERM = (3, 5, 6, 7)
RROW = 28 * 64
BROWS = RROW + 80


def _sa(a11, a12, a21, a22):
    return [a11 + a22, a21 + a22, a11, a22, a11 + a12, a21 - a11, a12 - a22]


def _sb(b11, b12, b21, b22):
    return [b11 + b22, b11, b12 - b22, b21 - b11, b22, b11 + b12, b21 + b22]


def _ppos(i, j):
    return ((j - 1) * 4 + (i - 1) // 2) * 64, ((i - 1) % 2) * PW


def _rpos(ct):
    return RROW + (ct // 2) * 40, (ct % 2) * PW


_VT = [
    69, 74, 88, 142, 97, 108, 86, 159, 180, 74, 74, 71, 177, 165, 54, 224,
    205, 111, 54, 159, 110, 74, 73, 124, 197, 115, 102, 54, 173, 166, 75, 210,
    186, 112, 69, 140, 144, 74, 74, 122, 180, 98, 114, 61, 173, 181, 60, 206,
    202, 79, 73, 90, 160, 108, 108, 71, 196, 128, 74, 90, 53, 190, 169, 207,
    216]
_ST = [
    17, 54, 35, 55, 19, 52, 59, 40, 54, 18, 54, 10, 17, 19, 12, 21, 55, 56,
    23, 55, 39, 40, 41, 73, 53, 44, 56, 2, 16, 18, 12, 17, 19, 53, 56, 40, 54,
    19, 54, 59, 55, 20, 53, 20, 16, 18, 2, 16, 21, 40, 42, 54, 53, 43, 56, 43,
    53, 41, 45, 38, 9, 17, 46, 19, 18]
_TWEAK_N = [
    0.9828, 0.9839, 1.01398, 0.98541, 1.00728, 0.99425, 1.00389, 1.01152,
    0.99502, 0.98379, 1.01123, 1.01835, 0.98509, 1.0029, 0.99551, 1.01405,
    0.99855, 0.98243, 0.98056, 1.00118, 0.99897, 1.01689, 1.00727, 1.01595,
    0.98844, 1.01765, 0.8735, 0.98703, 1.1143, 0.986, 0.98997, 0.98439,
    0.98695, 0.99158, 1.01374, 0.98589, 0.98108, 1.01386, 0.98936, 0.99016,
    0.9814, 1.00424, 1.01849, 1.01495, 1.00793, 1.00902, 0.98653, 0.98687,
    1.01838, 0.98093, 1.00808, 1.01421, 1.072, 0.9419, 1.01009, 0.99972,
    0.99743, 1.01128, 1.0018, 1.01947, 0.98541, 1.01755, 0.98403, 0.99922,
    0.99382]
_TWEAK_S = [
    1.0053, 1.01411, 1.01355, 1.01331, 1.01532, 0.98415, 0.99508, 0.98366,
    1.01019, 1.00921, 1.01064, 1.01369, 0.98088, 0.98484, 0.98206, 1.01342,
    0.99292, 1.00066, 1.00765, 1.0284, 1.00497, 0.9715, 1.01995, 1.131,
    0.9811, 0.901, 0.99564, 1.00568, 0.9122, 1.0664, 0.99055, 1.0011, 1.00992,
    0.99784, 0.99829, 1.01798, 1.0003, 1.01299, 0.99382, 1.00796, 0.98314,
    1.00115, 0.99082, 1.00391, 1.00266, 0.99323, 1.00732, 0.99376, 1.0182,
    1.00364, 0.98682, 1.00752, 0.98366, 0.98479, 0.99891, 1.0002, 0.8172,
    1.01446, 1.1488, 1.0194, 1.1624, 0.8247, 0.7226, 0.99523, 1.2142]
_NCOST = []
for _k in range(8):
    _NCOST += [43, 51, 51, 29, 21, 51, 29] + ([32] if _k % 2 == 0 else [])

_FIRST_WAITS = {17: (2, 3), 41: (4, 5, 6), 80: (7, 8, 9, 10)}
_FIRST_TASKS = [
    ("S", 1, 0, 4.56),
    ("N", 1, 4.56, 14.49),
    ("S", 2, 17, 19.92),
    ("N", 2, 19.92, 29.8276),
    ("S", 3, 19.92, 29.3276),
    ("N", 3, 29.8276, 41),
    ("S", 4, 41, 44.83),
    ("N", 4, 44.83, 56.55333),
    ("S", 5, 44.83, 56.55333),
    ("N", 5, 56.55333, 68.27667),
    ("S", 6, 56.55333, 68.27667),
    ("N", 6, 68.27667, 80),
    ("S", 7, 80, 84.1),
    ("N", 7, 84.1, 95.575),
    ("S", 8, 84.1, 95.575),
    ("N", 8, 95.575, 107.05),
    ("S", 9, 95.575, 107.05),
    ("N", 9, 107.05, 118.525),
    ("S", 10, 107.05, 118.525),
    ("N", 10, 118.525, 130.0),
    ("S", 11, 118.525, 130.0),
]

_ORDER = {
    ("put", 0): "m1 m2 m4 m6 m3 m5 m7",
    ("put", 1): "m1 m2 m4 m3 m5 m6 m7",
    ("put", 2): "m1 m6 m2 m3 m4 m5 m7",
    ("put", 3): "m2 m1 m3 m5 m6 m4 m7",
    ("sep", 0): "m1 m2 m4 m7 m3 m5 r11 r12 m6 r21 r22",
    ("sep", 1): "m1 m2 m4 m3 m6 r21 r22 m5 m7 r11 r12",
    ("sep", 2): "m3 m4 m1 m2 m6 r21 m5 m7 r11 r12 r22",
    ("sep", 3): "m3 m1 m2 m4 m6 m5 m7 r11 r12 r21 r22",
    ("merge", 0): "m3 m6 r12 r22 m1 m2 m4 r21 m5 m7 r11",
    ("merge", 1): "m3 m6 r22 m1 m2 m4 r21 m5 m7 r11 r12",
    ("merge", 2): "m6 r22 m4 m7 r11 r21 m1 m3 m5 r12 m2",
    ("merge", 3): "m1 m3 m6 r12 r22 m2 m4 m7 r21 m5 r11",
    ("early", 3): "m3 m1 m2 m4 m6 m5 m7",
}
_TERMS = {"11": {"m1": 1, "m7": 1, "m5": -1, "m4": 1},
          "12": {"m3": 1, "m5": 1},
          "21": {"m2": 1, "m4": 1},
          "22": {"m1": 1, "m3": 1, "m6": 1, "m2": -1}}


def _stats_pair(x, gates):
    ng = len(gates) if gates else 18
    n = D // 8 // ng
    c = jnp.broadcast_to(x[0:1, :], (8, W2))
    a1 = a2 = None
    for k in range(ng):
        ck = gates[k](c, 2) if gates else c
        v = x[k * n * 8:(k + 1) * n * 8] - cat([ck] * n, axis=0)
        sq = v * v
        if a1 is not None:
            v = cat([a1, v], axis=0)
            sq = cat([a2, sq], axis=0)
        a1 = jnp.sum(v.reshape(-1, 8, W2), axis=0)
        a2 = jnp.sum(sq.reshape(-1, 8, W2), axis=0)
    a1 = jnp.sum(a1, axis=0, keepdims=True) * (1.0 / D)
    a2 = jnp.sum(a2, axis=0, keepdims=True) * (1.0 / D)
    m = c[0:1] + a1
    var = jnp.maximum(a2 - a1 * a1, 0.0)
    r = lax.rsqrt(var + EPS)
    return jnp.broadcast_to(m, (8, W2)), jnp.broadcast_to(r, (8, W2))


def _stats_quad(x, gates):
    h = len(gates) // 2
    ma, ra = _stats_pair(x[:, 0:W2], gates[:h])
    mb, rb = _stats_pair(x[:, W2:], gates[h:])
    return cat([ma, mb], axis=1), cat([ra, rb], axis=1)


def _norm_quad(x, m, r, p_ref, gates):
    def tiles(v, tc):
        return cat([v[:, tc * PW:(tc + 1) * PW],
                    v[:, (tc + 2) * PW:(tc + 3) * PW]], axis=1)

    def wide(v):
        return cat([cat([v, v], axis=1)] * 2, axis=0)

    xt = [tiles(x, 0), tiles(x, 1)]
    mt = [tiles(m, 0), tiles(m, 1)]
    rt = [wide(tiles(r, 0)), wide(tiles(r, 1))]
    r16 = cat([r, r], axis=0)
    it = iter(gates)

    def sub(k, kr, tc):
        g = next(it, None)
        mg = mt[tc] if g is None else g(mt[tc], 2)
        r0 = kr * 128 + k * 16
        xb = cat([xt[tc][r0:r0 + 16], xt[tc][KH + r0:KH + r0 + 16]], axis=1)
        return (xb - wide(mg)) * rt[tc]

    def emit(k, j, v, gate=False):
        q = [v[:, i * PW:(i + 1) * PW] for i in range(4)]
        g = next(it, None) if gate else None
        if g is not None:
            q[0] = g(q[0], 0)
            q[3] = g(q[3], 0)
        ops = _sb(*q)
        for i0 in range(0, 7, 2):
            grp = ops[i0:i0 + 2]
            r0 = _ppos(i0 + 1, j)[0] + k * 8
            p_ref[r0:r0 + 8, 0:len(grp) * PW] = pltpu.bitcast(
                cat(grp, axis=1).astype(bf16), u32)

    for k in range(8):
        b11 = sub(k, 0, 0)
        emit(k, 2, b11)
        b12 = sub(k, 0, 1)
        emit(k, 6, b11 + b12)
        b22 = sub(k, 1, 1)
        emit(k, 3, b12 - b22)
        emit(k, 1, b11 + b22, True)
        emit(k, 5, b22, True)
        b21 = sub(k, 1, 0)
        emit(k, 4, b21 - b11)
        emit(k, 7, b21 + b22, True)
        if k % 2 == 0:
            g = next(it, None)
            mg = m if g is None else g(m, 4)
            r0 = 2 * KH + k * 8
            v = (x[r0:r0 + 16] - cat([mg, mg], axis=0)) * r16
            for c0 in (0, 2):
                r1 = _rpos(c0)[0] + k * 4
                p_ref[r1:r1 + 8, :] = pltpu.bitcast(
                    v[:, c0 * PW:(c0 + 2) * PW].astype(bf16), u32)


def _kernel(x_hbm, g_hbm, b_hbm, w_hbm, o_hbm, xbuf, obuf,
            p0, p1, p2, p3, u0, u1, u2, u3, u4,
            st_ref, g_ref, b_ref, w_ref, a_ref, ar_ref, zs, sin, sout):
    ps = [p0, p1, p2, p3]
    us = [u0, u1, u2, u3, u4]
    for i in range(4):
        zs[i] = 0

    def cin_slab5():
        return pltpu.make_async_copy(x_hbm.at[5], xbuf.at[5], sin.at[NI])

    def cin_pair(j):
        rows = pl.ds(6 + 2 * j, 2)
        return pltpu.make_async_copy(x_hbm.at[rows], xbuf.at[rows], sin.at[j])

    def cin_quad(n):
        t, c = divmod(n, 2)
        return pltpu.make_async_copy(
            x_hbm.at[t, :, c * W4:(c + 1) * W4],
            xbuf.at[t, :, c * W4:(c + 1) * W4], sin.at[NI + 4 + n])

    def cout(sl, r0, r1, ct):
        idx = (sl, slice(r0, r1), slice(ct * PW, (ct + 1) * PW))
        pltpu.make_async_copy(
            obuf.at[idx], o_hbm.at[idx], sout.at[0]).start(priority=ct % 2)

    def cout_quad(t, c):
        for ct in range(4):
            cout(t, 0, D, 4 * c + ct)

    cw = pltpu.make_async_copy(w_hbm, w_ref, sin.at[NI + 1])
    cg = pltpu.make_async_copy(g_hbm, g_ref, sin.at[NI + 2])
    cb = pltpu.make_async_copy(b_hbm, b_ref, sin.at[NI + 3])
    cg.start()
    cb.start()
    cw.start()
    for n in range(NH):
        cin_quad(n).start()
    cin_slab5().start()
    for j in range(NI - 1):
        cin_pair(j).start()

    row16 = lax.broadcasted_iota(jnp.int32, (16, W2), 0)
    ones = pltpu.bitcast(jnp.where(row16 < 3, 1.0, 0.0).astype(bf16), u32)
    for p_ref in ps:
        for c0 in (0, 2):
            r1 = _rpos(c0)[0] + 32
            p_ref[r1:r1 + 8, :] = ones

    cg.wait()
    cb.wait()
    cw.wait()
    g = g_ref[...].astype(f32).reshape(1, D)
    w = w_ref[...]
    b16 = jnp.broadcast_to(b_ref[...].reshape(1, D), (16, D))
    bias = jnp.dot(b16, w, preferred_element_type=f32)[0:8]
    bh = bias.astype(bf16).astype(f32)
    bl = (bias - bh).astype(bf16).astype(f32)
    bl2 = bias - bh - bl
    row8 = lax.broadcasted_iota(jnp.int32, (8, D), 0)
    ext = jnp.where(row8 == 0, bh,
                    jnp.where(row8 == 1, bl, jnp.where(row8 == 2, bl2, 0.0)))
    wf = w.astype(f32)
    wr = cat([wf[2 * KH:], ext, jnp.zeros((56, D), f32)], axis=0)
    wg = wf[:2 * KH].T * g[:, :2 * KH]
    gr = cat([g[:, 2 * KH:], jnp.ones((1, 64), f32)], axis=1)
    a1 = _sa(wg[0:H, 0:KH], wg[0:H, KH:], wg[H:, 0:KH], wg[H:, KH:])
    for i in range(1, 8):
        top, bot = a1[i - 1][0:Q], a1[i - 1][Q:]
        if i in PERM:
            top, bot = bot, top
        a2 = _sa(top[:, 0:128], top[:, 128:], bot[:, 0:128], bot[:, 128:])
        a_ref[:, (i - 1) * PW:i * PW] = pltpu.bitcast(
            cat(a2, axis=0).astype(bf16), u32)
    arv = (wr.T * gr).astype(bf16)
    ar_ref[:, 0:PW] = pltpu.bitcast(arv[0:H], u32)
    ar_ref[:, PW:] = pltpu.bitcast(arv[H:], u32)

    cin_quad(0).wait()
    _norm_quad(xbuf[zs[2], :, 0:W4].astype(f32),
               *_stats_quad(xbuf[zs[0], :, 0:W4].astype(f32), []), ps[0], [])

    def run(s, nq, fresh, waits, tasks, hooks, have_st, save_st, bubble,
            valu=461, vst=87, ratio=5.74, tweak=True):
        k1 = s + zs[0]
        k2 = s + zs[2]
        never = {n: lax.broadcasted_iota(
            jnp.int32, (8, n * PW) if n else (16, PW), 0) < zs[1]
                 for n in (0, 2, 4)}
        zero = pl.multiple_of(zs[3], 8)
        nr = -(-65 * nq // 4)
        free = [max(valu - _VT[r % 65], 0) for r in range(nr)]
        tn = _TWEAK_N if tweak else [1] * 65
        ts = _TWEAK_S if tweak else [1] * 65
        wn = [(min(free[r], max(vst - _ST[r % 65], 0) * ratio) + 0.01)
              * tn[r % 65] for r in range(nr)]
        sc = sum(_NCOST) * nr / 16.25 / sum(wn)
        ws = [(max(free[r] - wn[r] * sc, 0) + 0.01) * ts[r % 65]
              for r in range(nr)]

        def xload(k, q):
            t, c = divmod(q, 2)
            return xbuf[jnp.minimum(k + t, S - 1), :,
                        c * W4:(c + 1) * W4].astype(f32)

        def make_gate(e):
            if e is None:
                return lambda v, n: v

            def gate(v, n):
                z = e[0][e[1]:e[1] + 8]
                z = cat([z] * n, axis=1) if n else cat([z, z], axis=0)
                return lax.select(never[n], z, v)
            return gate

        mr = {}
        if have_st is not None:
            mr[have_st] = (st_ref[0:8, :], st_ref[8:16, :])
        first = {}
        todo = list(tasks)

        def flush(now):
            for task in [t for t in todo if t[3] <= now + 1e-9]:
                todo.remove(task)
                kind, q, t0, t1 = task
                wt = wn if kind == "N" else ws
                cand = []
                a = 0.0
                if t0 == 0 or t0 in waits:
                    cand.append((0.0, None))
                    a += bubble[kind]
                for r in range(int(t0), nr):
                    for e in range(NPER):
                        if t0 - 1e-9 <= r + e / NPER < t1 - 1e-9:
                            cand.append(
                                (a, (first[r], Q * e // NPER // 8 * 8)))
                            a += wt[r] / NPER
                costs = _NCOST if kind == "N" else [1] * (2 * SG)
                done = 0
                gates = []
                for x in costs:
                    tgt = a * done / sum(costs)
                    gates.append(make_gate(
                        [e for (c, e) in cand if c <= tgt + 1e-9][-1]))
                    done += x
                if kind == "N":
                    _norm_quad(xload(k2, q), *mr.pop(q), ps[q % 4], gates)
                else:
                    mr[q] = _stats_quad(xload(k1, q), gates)

        count = [0]

        def mxu(lhs, rhs):
            r, o = divmod(count[0], 4)
            if o == 0 and r in waits:
                flush(r)
                waits[r]()
            v = jnp.dot(lhs(), rhs(), preferred_element_type=f32)
            if o == 0:
                first[r] = v
            count[0] += 1
            return v

        def get(i):
            return us[i][pl.ds(zero, H), :]

        def get_sub(i, hr, hc):
            return us[i][pl.ds(pl.multiple_of(zero + hr * Q, 8), Q),
                         hc * PW:(hc + 1) * PW]

        def quad(p):
            sl = s + p // 2
            c0 = (p % 2) * W4
            p_ref = ps[p % 4]
            if p in fresh:
                p_ref = p_ref.at[pl.ds(zero, BROWS), :]

            def hook(name):
                if (p, name) in hooks:
                    hooks[(p, name)]()

            def dot(i, j):
                r1, c1 = _ppos(i, j)
                return mxu(
                    lambda: pltpu.bitcast(
                        a_ref[(j - 1) * 72:j * 72, (i - 1) * PW:i * PW], bf16),
                    lambda: pltpu.bitcast(
                        p_ref[r1:r1 + 64, c1:c1 + PW], bf16))

            def rem(half, cc, hr, hc):
                r1, c1 = _rpos(2 * cc + hc)
                return mxu(
                    lambda: pltpu.bitcast(
                        ar_ref[hr * 72:(hr + 1) * 72,
                               half * PW:(half + 1) * PW], bf16)[:, :KR],
                    lambda: pltpu.bitcast(
                        p_ref[r1:r1 + 40, c1:c1 + PW], bf16))

            def prod(i, o=None, sep=None, plus=(), minus=()):
                sw = 1 if i in PERM else 0

                def blk(c):
                    rows = [cat([c["11"], c["12"]], axis=1),
                            cat([c["21"], c["22"]], axis=1)]
                    return cat(rows[::-1] if sw else rows, axis=0)

                kind = "sep" if i in (4, 5) else "merge" if o else "put"
                seq = _ORDER[("early" if sep else kind, count[0] % 4)].split()
                acc = {}
                sign = {}
                sep = dict(sep or {})
                for n, nm in enumerate(seq):
                    if nm[0] == "m":
                        v = dot(i, int(nm[1]))
                    else:
                        v = rem(o[0], o[1], (int(nm[1]) - 1) ^ sw,
                                int(nm[2]) - 1)
                        sep[nm[1:]] = v
                    for k, terms in _TERMS.items():
                        sg = terms.get(nm)
                        if kind == "merge" and nm == "r" + k:
                            sg = 1
                        if sg is None:
                            continue
                        if k not in acc:
                            acc[k], sign[k] = v, sg
                        elif sign[k] < 0:
                            acc[k], sign[k] = v - acc[k], 1
                        else:
                            acc[k] = acc[k] + v if sg > 0 else acc[k] - v
                    if plus and n == len(seq) - 5:
                        for k in _TERMS:
                            hr, hc = (int(k[0]) - 1) ^ sw, int(k[1]) - 1
                            for u in plus:
                                acc[k] = acc[k] + get_sub(u, hr, hc)
                            for u in minus:
                                acc[k] = acc[k] - get_sub(u, hr, hc)
                return blk(acc), blk(sep) if kind == "sep" else None

            def out(i, o, plus, minus=(), sep=None):
                if i == 6 and p == nq - 1:
                    val, v = prod(i, o, None, plus, minus)
                    plus = minus = ()
                else:
                    val, v = prod(i, o, sep)
                if o == (1, 1):
                    hook("m6")
                v = val if v is None else val + v
                for u in plus:
                    v = v + get(u)
                for u in minus:
                    v = v - get(u)
                obuf[sl, o[0] * H:(o[0] + 1) * H,
                     c0 + o[1] * W2:c0 + (o[1] + 1) * W2] = v.astype(bf16)
                return val

            early = None
            if p == 0:
                early = {k: rem(0, 1, (int(k[0]) - 1) ^ 1, int(k[1]) - 1)
                         for k in _TERMS}
            us[0][...] = prod(3)[0]
            hook("m3")
            us[1][...] = out(5, (0, 1), [0], sep=early)
            us[2][...] = prod(2)[0]
            hook("m2")
            m4 = out(4, (1, 0), [2])
            us[3][...] = m4 - get(1)
            us[4][...] = prod(1)[0]
            hook("m1")
            out(7, (0, 0), [3, 4])
            out(6, (1, 1), [0, 4], [2])

        for p in range(nq):
            flush(-(-count[0] // 4))
            quad(p)
        flush(nr)
        st_ref[0:8, :] = mr[save_st][0]
        st_ref[8:16, :] = mr[save_st][1]

    def wait_quads(ns):
        return lambda: [(cin_quad(n) if n < NH else cin_slab5()).wait()
                        for n in ns]

    cin_quad(1).wait()
    run(0, FQ, range(1, FQ),
        {r: wait_quads(ns) for r, ns in _FIRST_WAITS.items()}, _FIRST_TASKS,
        {}, None, FQ + 3, {"N": 287, "S": 321}, 478, 96, 6.56, False)

    f = FQ // 2
    j_flush = (DEFER - f) // 2
    bnd = [0, 17, 33, 49, 65]

    def write_part(half, cc):
        for k in range(2):
            cout(S - 1, half * H, (half + 1) * H, 4 + 2 * cc + k)

    def body(j, carry):
        s = f + 2 * j

        @pl.when(j < NI - 1)
        def _():
            cin_pair(j).wait()

        def write_prev(p):
            def fn():
                if p == 0:
                    @pl.when(j == j_flush)
                    def _():
                        for ct in range(8):
                            cout(pl.ds(0, DEFER), 0, D, ct)

                @pl.when(j > j_flush if p == 0 else j >= j_flush)
                def _():
                    cout_quad(s + (p - 1) // 2, (p - 1) % 2)
            return fn

        def write_last(half, cc):
            return lambda: pl.when(j == NI - 1)(
                lambda: write_part(half, cc))

        hooks = {(p, "m3"): write_prev(p) for p in range(4)}
        hooks.update({(3, "m2"): write_last(0, 1), (3, "m1"): write_last(1, 0),
                      (3, "m6"): write_last(0, 0)})
        tasks = []
        for p in range(4):
            tasks += [("S", p + 4, max(bnd[p] - 3, 0), bnd[p + 1] - 3),
                      ("N", p + 3, bnd[p], bnd[p + 1])]
        run(s, 4, (3,), {}, tasks, hooks, 3, 7, {"N": 0.01, "S": 0.01})
        return carry

    lax.fori_loop(0, NI, body, 0)
    write_part(1, 1)
    pltpu.make_async_copy(obuf, o_hbm, sout.at[0]).wait()


@jax.jit
def pallas_standalone__layernorm_linear__sampling_kernel(
    x: jax.Array,
    g: jax.Array,
    b: jax.Array,
    w: jax.Array,
):
    assert x.shape == (B, S, D) and w.shape == (D, D)
    xt = jnp.transpose(x, (1, 2, 0))
    out = pl.pallas_call(
        _kernel,
        in_specs=[pl.BlockSpec(memory_space=pl.ANY)] * 4,
        out_specs=pl.BlockSpec(memory_space=pl.ANY),
        out_shape=jax.ShapeDtypeStruct((S, D, B), x.dtype),
        scratch_shapes=[
            pltpu.VMEM((S, D, B), bf16),
            pltpu.VMEM((S, D, B), bf16),
        ] + [pltpu.VMEM((BROWS, W2), u32)] * 4
        + [pltpu.VMEM((H, W2), f32)] * 5
        + [
            pltpu.VMEM((16, W4), f32),
            pltpu.VMEM((D,), bf16),
            pltpu.VMEM((D,), bf16),
            pltpu.VMEM((D, D), bf16),
            pltpu.VMEM((7 * 72, 7 * PW), u32),
            pltpu.VMEM((144, W2), u32),
            pltpu.SMEM((4,), jnp.int32),
            pltpu.SemaphoreType.DMA((NI + 4 + NH,)),
            pltpu.SemaphoreType.DMA((1,)),
        ],
        compiler_params=pltpu.CompilerParams(
            vmem_limit_bytes=110 * 1024 * 1024,
            disable_bounds_checks=True,
            disable_semaphore_checks=True,
        ),
    )(xt, g, b, w)
    return jnp.transpose(out, (2, 0, 1))
```

```python
import jax
import jax.numpy as jnp
from jax import lax
import jax.experimental.pallas as pl
import jax.experimental.pallas.tpu as pltpu

EPS = 1e-5
D = 576
S = 32
B = 1024
H = D // 2
Q = D // 4
KH = 256
KR = 80
PW = 128
W2 = 2 * PW
W4 = 4 * PW
NH = 10
FQ = 8
NI = 14
DEFER = 14
NPER = 18
f32 = jnp.float32
bf16 = jnp.bfloat16
u32 = jnp.uint32
cat = jnp.concatenate
PERM = (3, 5, 6, 7)
RROW = 28 * 64
BROWS = RROW + 80


def _sa(a11, a12, a21, a22):
    return [a11 + a22, a21 + a22, a11, a22, a11 + a12, a21 - a11, a12 - a22]


def _sb(b11, b12, b21, b22):
    return [b11 + b22, b11, b12 - b22, b21 - b11, b22, b11 + b12, b21 + b22]


def _ppos(i, j):
    return ((j - 1) * 4 + (i - 1) // 2) * 64, ((i - 1) % 2) * PW


def _rpos(ct):
    return RROW + (ct // 2) * 40, (ct % 2) * PW


_VT = [
    69, 74, 88, 142, 97, 108, 86, 159, 180, 74, 74, 71, 177, 165, 54, 224,
    205, 111, 54, 159, 110, 74, 73, 124, 197, 115, 102, 54, 173, 166, 75, 210,
    186, 112, 69, 140, 144, 74, 74, 122, 180, 98, 114, 61, 173, 181, 60, 206,
    202, 79, 73, 90, 160, 108, 108, 71, 196, 128, 74, 90, 53, 190, 169, 207,
    216]
_ST = [
    17, 54, 35, 55, 19, 52, 59, 40, 54, 18, 54, 10, 17, 19, 12, 21, 55, 56,
    23, 55, 39, 40, 41, 73, 53, 44, 56, 2, 16, 18, 12, 17, 19, 53, 56, 40, 54,
    19, 54, 59, 55, 20, 53, 20, 16, 18, 2, 16, 21, 40, 42, 54, 53, 43, 56, 43,
    53, 41, 45, 38, 9, 17, 46, 19, 18]
_TWEAK_N = [
    1.0, 1.0517, 0.9483, 1.0, 1.0, 1.0, 1.0, 1.0, 1.0, 1.0, 1.0, 1.0, 1.0,
    1.0, 1.0, 1.0, 1.0, 1.0, 1.0, 1.0, 1.0, 1.0, 1.0, 1.0, 1.0, 1.0, 1.0, 1.0,
    0.8555, 1.1445, 1.0, 1.0, 1.0, 1.0, 1.0, 1.0, 1.0, 1.0, 1.0, 1.0, 1.0,
    1.0, 1.0, 1.0, 1.0, 1.0, 1.0, 1.0, 1.0, 1.0, 1.0, 1.0, 1.0, 1.0, 1.0, 1.0,
    1.0, 1.0, 0.797, 1.203, 1.0, 1.0, 1.0, 1.0, 1.0]
_TWEAK_S = [
    1.0, 1.0, 1.0, 0.7852, 1.2148, 1.0, 1.0, 1.0, 1.0, 1.0, 1.0, 1.0, 1.0,
    1.0, 1.0, 1.0, 1.0, 0.8003, 1.0, 1.0, 1.0, 1.0, 1.0, 1.0, 1.0, 1.0, 1.0,
    1.0, 1.0, 1.0, 1.0, 1.0, 1.0, 1.0, 1.0, 1.0, 1.0, 1.0, 1.0, 1.0, 1.0, 1.0,
    1.0, 1.0, 1.0, 1.0843, 1.0, 0.9157, 1.0, 1.0, 1.0, 1.0, 1.0, 1.0, 1.0,
    1.0, 1.0, 1.0, 1.0, 1.0, 1.0, 0.9167, 1.0, 1.0833, 1.0]
_NCOST = []
for _k in range(8):
    _NCOST += [13, 13, 9, 12, 17, 17, 9, 12, 17, 17, 9, 12, 17, 12, 9, 12, 17,
               17, 9, 12, 17, 12] + ([16, 16] if _k % 2 == 0 else [])

_FIRST_WAITS = {17: (2, 3), 42: (4, 5, 6), 82: (7, 8, 9, 10)}
_FIRST_TASKS = [
    ("S", 1, 0, 4.46),
    ("N", 1, 4.46, 14.59),
    ("S", 2, 17, 20.23),
    ("N", 2, 20.23, 30.2442),
    ("S", 3, 20.23, 29.7442),
    ("N", 3, 30.2442, 42),
    ("S", 4, 42, 46.49),
    ("N", 4, 46.49, 58.326667),
    ("S", 5, 46.49, 58.326667),
    ("N", 5, 58.326667, 70.163333),
    ("S", 6, 58.326667, 70.163333),
    ("N", 6, 70.163333, 82),
    ("S", 7, 82, 87.39),
    ("N", 7, 87.39, 98.0425),
    ("S", 8, 87.39, 98.0425),
    ("N", 8, 98.0425, 108.695),
    ("S", 9, 98.0425, 108.695),
    ("N", 9, 108.695, 119.3475),
    ("S", 10, 108.695, 119.3475),
    ("N", 10, 119.3475, 130.0),
    ("S", 11, 119.3475, 130.0),
]

_ORDER = {
    ("put", 0): "m1 m2 m4 m6 m3 m5 m7",
    ("put", 1): "m1 m2 m4 m3 m5 m6 m7",
    ("put", 2): "m1 m6 m2 m3 m4 m5 m7",
    ("put", 3): "m2 m1 m3 m5 m6 m4 m7",
    ("sep", 0): "m1 m2 m4 m7 m3 m5 r11 r12 m6 r21 r22",
    ("sep", 1): "m1 m2 m4 m3 m6 r21 r22 m5 m7 r11 r12",
    ("sep", 2): "m3 m4 m1 m2 m6 r21 m5 m7 r11 r12 r22",
    ("sep", 3): "m3 m1 m2 m4 m6 m5 m7 r11 r12 r21 r22",
    ("merge", 0): "m3 m6 r12 r22 m1 m2 m4 r21 m5 m7 r11",
    ("merge", 1): "m3 m6 r22 m1 m2 m4 r21 m5 m7 r11 r12",
    ("merge", 2): "m6 r22 m4 m7 r11 r21 m1 m3 m5 r12 m2",
    ("merge", 3): "m1 m3 m6 r12 r22 m2 m4 m7 r21 m5 r11",
    ("early", 3): "m3 m1 m2 m4 m6 m5 m7",
}
_TERMS = {"11": {"m1": 1, "m7": 1, "m5": -1, "m4": 1},
          "12": {"m3": 1, "m5": 1},
          "21": {"m2": 1, "m4": 1},
          "22": {"m1": 1, "m3": 1, "m6": 1, "m2": -1}}


def _stats_pair(x, gates):
    c = jnp.broadcast_to(x[0:1, :], (8, W2))
    a1 = a2 = None
    if gates:
        for k in range(D // 8):
            v = x[k * 8:(k + 1) * 8] - gates[k](c, 2)
            a1 = v if a1 is None else a1 + v
            a2 = v * v if a2 is None else a2 + v * v
    else:
        c4 = cat([c] * 4, axis=0)
        for k in range(D // 32):
            v = x[k * 32:(k + 1) * 32] - c4
            sq = v * v
            if a1 is not None:
                v = cat([a1, v], axis=0)
                sq = cat([a2, sq], axis=0)
            a1 = jnp.sum(v.reshape(-1, 8, W2), axis=0)
            a2 = jnp.sum(sq.reshape(-1, 8, W2), axis=0)
    a1 = jnp.sum(a1, axis=0, keepdims=True) * (1.0 / D)
    a2 = jnp.sum(a2, axis=0, keepdims=True) * (1.0 / D)
    m = c[0:1] + a1
    var = jnp.maximum(a2 - a1 * a1, 0.0)
    r = lax.rsqrt(var + EPS)
    return jnp.broadcast_to(m, (8, W2)), jnp.broadcast_to(r, (8, W2))


def _stats_quad(x, gates):
    h = len(gates) // 2
    ma, ra = _stats_pair(x[:, 0:W2], gates[:h])
    mb, rb = _stats_pair(x[:, W2:], gates[h:])
    return cat([ma, mb], axis=1), cat([ra, rb], axis=1)


def _norm_quad(x, m, r, p_ref, gates):
    def tiles(v, tc):
        return cat([v[:, tc * PW:(tc + 1) * PW],
                    v[:, (tc + 2) * PW:(tc + 3) * PW]], axis=1)

    def wide(v):
        return cat([cat([v, v], axis=1)] * 2, axis=0)

    xt = [tiles(x, 0), tiles(x, 1)]
    mt = [tiles(m, 0), tiles(m, 1)]
    rt = [wide(tiles(r, 0)), wide(tiles(r, 1))]
    ms = [m[:, c * PW:(c + 1) * PW] for c in range(4)]
    r16 = cat([r, r], axis=0)
    it = iter(gates)

    def sub(k, kr, tc):
        mg = mt[tc]
        if gates:
            mg = cat([next(it)(ms[tc], 1), next(it)(ms[tc + 2], 1)], axis=1)
        r0 = kr * 128 + k * 16
        xb = cat([xt[tc][r0:r0 + 16], xt[tc][KH + r0:KH + r0 + 16]], axis=1)
        return (xb - wide(mg)) * rt[tc]

    def emit(k, j, v):
        q = [v[:, i * PW:(i + 1) * PW] for i in range(4)]
        if gates:
            q[0] = next(it)(q[0], 0)
            q[3] = next(it)(q[3], 0)
        ops = _sb(*q)
        for i0 in range(0, 7, 2):
            grp = ops[i0:i0 + 2]
            r0 = _ppos(i0 + 1, j)[0] + k * 8
            p_ref[r0:r0 + 8, 0:len(grp) * PW] = pltpu.bitcast(
                cat(grp, axis=1).astype(bf16), u32)

    for k in range(8):
        b11 = sub(k, 0, 0)
        emit(k, 2, b11)
        b12 = sub(k, 0, 1)
        emit(k, 6, b11 + b12)
        b22 = sub(k, 1, 1)
        emit(k, 3, b12 - b22)
        emit(k, 1, b11 + b22)
        emit(k, 5, b22)
        b21 = sub(k, 1, 0)
        emit(k, 4, b21 - b11)
        emit(k, 7, b21 + b22)
        if k % 2 == 0:
            mg = m
            if gates:
                mg = cat([next(it)(m[:, 0:W2], 2), next(it)(m[:, W2:], 2)],
                         axis=1)
            r0 = 2 * KH + k * 8
            v = (x[r0:r0 + 16] - cat([mg, mg], axis=0)) * r16
            for c0 in (0, 2):
                r1 = _rpos(c0)[0] + k * 4
                p_ref[r1:r1 + 8, :] = pltpu.bitcast(
                    v[:, c0 * PW:(c0 + 2) * PW].astype(bf16), u32)


def _kernel(x_hbm, g_hbm, b_hbm, w_hbm, o_hbm, xbuf, obuf,
            p0, p1, p2, p3, u0, u1, u2, u3, u4,
            st_ref, g_ref, b_ref, w_ref, a_ref, ar_ref, zs, sin, sout):
    ps = [p0, p1, p2, p3]
    us = [u0, u1, u2, u3, u4]
    for i in range(4):
        zs[i] = 0

    def cin_slab5():
        return pltpu.make_async_copy(x_hbm.at[5], xbuf.at[5], sin.at[NI])

    def cin_pair(j):
        rows = pl.ds(6 + 2 * j, 2)
        return pltpu.make_async_copy(x_hbm.at[rows], xbuf.at[rows], sin.at[j])

    def cin_quad(n):
        t, c = divmod(n, 2)
        return pltpu.make_async_copy(
            x_hbm.at[t, :, c * W4:(c + 1) * W4],
            xbuf.at[t, :, c * W4:(c + 1) * W4], sin.at[NI + 4 + n])

    def cout(sl, r0, r1, ct):
        idx = (sl, slice(r0, r1), slice(ct * PW, (ct + 1) * PW))
        pltpu.make_async_copy(
            obuf.at[idx], o_hbm.at[idx], sout.at[0]).start(priority=ct % 2)

    def cout_quad(t, c):
        for ct in range(4):
            cout(t, 0, D, 4 * c + ct)

    cw = pltpu.make_async_copy(w_hbm, w_ref, sin.at[NI + 1])
    cg = pltpu.make_async_copy(g_hbm, g_ref, sin.at[NI + 2])
    cb = pltpu.make_async_copy(b_hbm, b_ref, sin.at[NI + 3])
    cg.start()
    cb.start()
    cw.start()
    for n in range(NH):
        cin_quad(n).start()
    cin_slab5().start()
    for j in range(NI - 1):
        cin_pair(j).start()

    row16 = lax.broadcasted_iota(jnp.int32, (16, W2), 0)
    ones = pltpu.bitcast(jnp.where(row16 < 3, 1.0, 0.0).astype(bf16), u32)
    for p_ref in ps:
        for c0 in (0, 2):
            r1 = _rpos(c0)[0] + 32
            p_ref[r1:r1 + 8, :] = ones

    cg.wait()
    cb.wait()
    cw.wait()
    g = g_ref[...].astype(f32).reshape(1, D)
    w = w_ref[...]
    b16 = jnp.broadcast_to(b_ref[...].reshape(1, D), (16, D))
    bias = jnp.dot(b16, w, preferred_element_type=f32)[0:8]
    bh = bias.astype(bf16).astype(f32)
    bl = (bias - bh).astype(bf16).astype(f32)
    bl2 = bias - bh - bl
    row8 = lax.broadcasted_iota(jnp.int32, (8, D), 0)
    ext = jnp.where(row8 == 0, bh,
                    jnp.where(row8 == 1, bl, jnp.where(row8 == 2, bl2, 0.0)))
    wf = w.astype(f32)
    wr = cat([wf[2 * KH:], ext, jnp.zeros((56, D), f32)], axis=0)
    wg = wf[:2 * KH].T * g[:, :2 * KH]
    gr = cat([g[:, 2 * KH:], jnp.ones((1, 64), f32)], axis=1)
    a1 = _sa(wg[0:H, 0:KH], wg[0:H, KH:], wg[H:, 0:KH], wg[H:, KH:])
    for i in range(1, 8):
        top, bot = a1[i - 1][0:Q], a1[i - 1][Q:]
        if i in PERM:
            top, bot = bot, top
        a2 = _sa(top[:, 0:128], top[:, 128:], bot[:, 0:128], bot[:, 128:])
        a_ref[:, (i - 1) * PW:i * PW] = pltpu.bitcast(
            cat(a2, axis=0).astype(bf16), u32)
    arv = (wr.T * gr).astype(bf16)
    ar_ref[:, 0:PW] = pltpu.bitcast(arv[0:H], u32)
    ar_ref[:, PW:] = pltpu.bitcast(arv[H:], u32)

    cin_quad(0).wait()
    _norm_quad(xbuf[zs[2], :, 0:W4].astype(f32),
               *_stats_quad(xbuf[zs[0], :, 0:W4].astype(f32), []), ps[0], [])

    def run(s, nq, fresh, waits, tasks, hooks, have_st, save_st, bubble,
            valu=427, vst=114, ratio=5.7, tweak=True):
        k1 = s + zs[0]
        k2 = s + zs[2]
        never = {n: lax.broadcasted_iota(
            jnp.int32, (8, n * PW) if n else (16, PW), 0) < zs[1]
                 for n in (0, 1, 2)}
        zero = pl.multiple_of(zs[3], 8)
        nr = -(-65 * nq // 4)
        free = [max(valu - _VT[r % 65], 0) for r in range(nr)]
        tn = _TWEAK_N if tweak else [1] * 65
        ts = _TWEAK_S if tweak else [1] * 65
        wn = [(min(free[r], max(vst - _ST[r % 65], 0) * ratio) + 0.01)
              * tn[r % 65] for r in range(nr)]
        sc = sum(_NCOST) * nr / 16.25 / sum(wn)
        ws = [(max(free[r] - wn[r] * sc, 0) + 0.01) * ts[r % 65]
              for r in range(nr)]

        def xload(k, q):
            t, c = divmod(q, 2)
            return xbuf[jnp.minimum(k + t, S - 1), :,
                        c * W4:(c + 1) * W4].astype(f32)

        def make_gate(e):
            if e is None:
                return lambda v, n: v

            def gate(v, n):
                z = e[0][e[1]:e[1] + 8]
                if n != 1:
                    z = cat([z, z], axis=1 if n else 0)
                return lax.select(never[n], z, v)
            return gate

        mr = {}
        if have_st is not None:
            mr[have_st] = (st_ref[0:8, :], st_ref[8:16, :])
        first = {}
        todo = list(tasks)

        def flush(now):
            for task in [t for t in todo if t[3] <= now + 1e-9]:
                todo.remove(task)
                kind, q, t0, t1 = task
                wt = wn if kind == "N" else ws
                cand = []
                a = 0.0
                if t0 == 0 or t0 in waits:
                    cand.append((0.0, None))
                    a += bubble[kind]
                for r in range(int(t0), nr):
                    for e in range(NPER):
                        if t0 - 1e-9 <= r + e / NPER < t1 - 1e-9:
                            cand.append(
                                (a, (first[r], Q * e // NPER // 8 * 8)))
                            a += wt[r] / NPER
                costs = _NCOST if kind == "N" else [1] * (D // 4)
                done = 0
                gates = []
                for x in costs:
                    tgt = a * done / sum(costs)
                    gates.append(make_gate(
                        [e for (c, e) in cand if c <= tgt + 1e-9][-1]))
                    done += x
                if kind == "N":
                    _norm_quad(xload(k2, q), *mr.pop(q), ps[q % 4], gates)
                else:
                    mr[q] = _stats_quad(xload(k1, q), gates)

        count = [0]

        def mxu(lhs, rhs):
            r, o = divmod(count[0], 4)
            if o == 0 and r in waits:
                flush(r)
                waits[r]()
            v = jnp.dot(lhs(), rhs(), preferred_element_type=f32)
            if o == 0:
                first[r] = v
            count[0] += 1
            return v

        def get(i):
            return us[i][pl.ds(zero, H), :]

        def get_sub(i, hr, hc):
            return us[i][pl.ds(pl.multiple_of(zero + hr * Q, 8), Q),
                         hc * PW:(hc + 1) * PW]

        def quad(p):
            sl = s + p // 2
            c0 = (p % 2) * W4
            p_ref = ps[p % 4]
            if p in fresh:
                p_ref = p_ref.at[pl.ds(zero, BROWS), :]

            def hook(name):
                if (p, name) in hooks:
                    hooks[(p, name)]()

            def dot(i, j):
                r1, c1 = _ppos(i, j)
                return mxu(
                    lambda: pltpu.bitcast(
                        a_ref[(j - 1) * 72:j * 72, (i - 1) * PW:i * PW], bf16),
                    lambda: pltpu.bitcast(
                        p_ref[r1:r1 + 64, c1:c1 + PW], bf16))

            def rem(half, cc, hr, hc):
                r1, c1 = _rpos(2 * cc + hc)
                return mxu(
                    lambda: pltpu.bitcast(
                        ar_ref[hr * 72:(hr + 1) * 72,
                               half * PW:(half + 1) * PW], bf16)[:, :KR],
                    lambda: pltpu.bitcast(
                        p_ref[r1:r1 + 40, c1:c1 + PW], bf16))

            def prod(i, o=None, sep=None, plus=(), minus=()):
                sw = 1 if i in PERM else 0

                def blk(c):
                    rows = [cat([c["11"], c["12"]], axis=1),
                            cat([c["21"], c["22"]], axis=1)]
                    return cat(rows[::-1] if sw else rows, axis=0)

                kind = "sep" if i in (4, 5) else "merge" if o else "put"
                seq = _ORDER[("early" if sep else kind, count[0] % 4)].split()
                acc = {}
                sign = {}
                sep = dict(sep or {})
                for n, nm in enumerate(seq):
                    if nm[0] == "m":
                        v = dot(i, int(nm[1]))
                    else:
                        v = rem(o[0], o[1], (int(nm[1]) - 1) ^ sw,
                                int(nm[2]) - 1)
                        sep[nm[1:]] = v
                    for k, terms in _TERMS.items():
                        sg = terms.get(nm)
                        if kind == "merge" and nm == "r" + k:
                            sg = 1
                        if sg is None:
                            continue
                        if k not in acc:
                            acc[k], sign[k] = v, sg
                        elif sign[k] < 0:
                            acc[k], sign[k] = v - acc[k], 1
                        else:
                            acc[k] = acc[k] + v if sg > 0 else acc[k] - v
                    if plus and n == len(seq) - 5:
                        for k in _TERMS:
                            hr, hc = (int(k[0]) - 1) ^ sw, int(k[1]) - 1
                            for u in plus:
                                acc[k] = acc[k] + get_sub(u, hr, hc)
                            for u in minus:
                                acc[k] = acc[k] - get_sub(u, hr, hc)
                return blk(acc), blk(sep) if kind == "sep" else None

            def out(i, o, plus, minus=(), sep=None):
                if i == 6 and p == nq - 1:
                    val, v = prod(i, o, None, plus, minus)
                    plus = minus = ()
                else:
                    val, v = prod(i, o, sep)
                if o == (1, 1):
                    hook("m6")
                v = val if v is None else val + v
                for u in plus:
                    v = v + get(u)
                for u in minus:
                    v = v - get(u)
                obuf[sl, o[0] * H:(o[0] + 1) * H,
                     c0 + o[1] * W2:c0 + (o[1] + 1) * W2] = v.astype(bf16)
                return val

            early = None
            if p == 0:
                early = {k: rem(0, 1, (int(k[0]) - 1) ^ 1, int(k[1]) - 1)
                         for k in _TERMS}
            us[0][...] = prod(3)[0]
            hook("m3")
            us[1][...] = out(5, (0, 1), [0], sep=early)
            us[2][...] = prod(2)[0]
            hook("m2")
            m4 = out(4, (1, 0), [2])
            us[3][...] = m4 - get(1)
            us[4][...] = prod(1)[0]
            hook("m1")
            out(7, (0, 0), [3, 4])
            out(6, (1, 1), [0, 4], [2])

        for p in range(nq):
            flush(-(-count[0] // 4))
            quad(p)
        flush(nr)
        st_ref[0:8, :] = mr[save_st][0]
        st_ref[8:16, :] = mr[save_st][1]

    def wait_quads(ns):
        return lambda: [(cin_quad(n) if n < NH else cin_slab5()).wait()
                        for n in ns]

    cin_quad(1).wait()
    run(0, FQ, range(1, FQ),
        {r: wait_quads(ns) for r, ns in _FIRST_WAITS.items()}, _FIRST_TASKS,
        {}, None, FQ + 3, {"N": 279, "S": 218}, 509, 109, 5.63, False)

    f = FQ // 2
    j_flush = (DEFER - f) // 2
    bnd = [0, 17, 33, 49, 65]

    def write_part(half, cc):
        for k in range(2):
            cout(S - 1, half * H, (half + 1) * H, 4 + 2 * cc + k)

    def body(j, carry):
        s = f + 2 * j

        @pl.when(j < NI - 1)
        def _():
            cin_pair(j).wait()

        def write_prev(p):
            def fn():
                if p == 0:
                    @pl.when(j == j_flush)
                    def _():
                        for ct in range(8):
                            cout(pl.ds(0, DEFER), 0, D, ct)

                @pl.when(j > j_flush if p == 0 else j >= j_flush)
                def _():
                    cout_quad(s + (p - 1) // 2, (p - 1) % 2)
            return fn

        def write_last(half, cc):
            return lambda: pl.when(j == NI - 1)(
                lambda: write_part(half, cc))

        hooks = {(p, "m3"): write_prev(p) for p in range(4)}
        hooks.update({(3, "m2"): write_last(0, 1), (3, "m1"): write_last(1, 0),
                      (3, "m6"): write_last(0, 0)})
        tasks = []
        for p in range(4):
            tasks += [("S", p + 4, max(bnd[p] - 5, 0), bnd[p + 1] - 5),
                      ("N", p + 3, bnd[p], bnd[p + 1])]
        run(s, 4, (3,), {}, tasks, hooks, 3, 7, {"N": 0.01, "S": 0.01})
        return carry

    lax.fori_loop(0, NI, body, 0)
    write_part(1, 1)
    pltpu.make_async_copy(obuf, o_hbm, sout.at[0]).wait()


@jax.jit
def pallas_standalone__layernorm_linear__sampling_kernel(
    x: jax.Array,
    g: jax.Array,
    b: jax.Array,
    w: jax.Array,
):
    assert x.shape == (B, S, D) and w.shape == (D, D)
    xt = jnp.transpose(x, (1, 2, 0))
    out = pl.pallas_call(
        _kernel,
        in_specs=[pl.BlockSpec(memory_space=pl.ANY)] * 4,
        out_specs=pl.BlockSpec(memory_space=pl.ANY),
        out_shape=jax.ShapeDtypeStruct((S, D, B), x.dtype),
        scratch_shapes=[
            pltpu.VMEM((S, D, B), bf16),
            pltpu.VMEM((S, D, B), bf16),
        ] + [pltpu.VMEM((BROWS, W2), u32)] * 4
        + [pltpu.VMEM((H, W2), f32)] * 5
        + [
            pltpu.VMEM((16, W4), f32),
            pltpu.VMEM((D,), bf16),
            pltpu.VMEM((D,), bf16),
            pltpu.VMEM((D, D), bf16),
            pltpu.VMEM((7 * 72, 7 * PW), u32),
            pltpu.VMEM((144, W2), u32),
            pltpu.SMEM((4,), jnp.int32),
            pltpu.SemaphoreType.DMA((NI + 4 + NH,)),
            pltpu.SemaphoreType.DMA((1,)),
        ],
        compiler_params=pltpu.CompilerParams(
            vmem_limit_bytes=110 * 1024 * 1024,
            disable_bounds_checks=True,
            disable_semaphore_checks=True,
        ),
    )(xt, g, b, w)
    return jnp.transpose(out, (2, 0, 1))
```

```python
import jax
import jax.numpy as jnp
from jax import lax
import jax.experimental.pallas as pl
import jax.experimental.pallas.tpu as pltpu

EPS = 1e-5
D = 576
S = 32
B = 1024
H = D // 2
Q = D // 4
KH = 256
KR = 80
PW = 128
W2 = 2 * PW
W4 = 4 * PW
NH = 6
NI = 15
DEFER = 14
NPER = 18
f32 = jnp.float32
bf16 = jnp.bfloat16
u32 = jnp.uint32
cat = jnp.concatenate
PERM = (3, 5, 6, 7)
RROW = 28 * 64
BROWS = RROW + 80


def _sa(a11, a12, a21, a22):
    return [a11 + a22, a21 + a22, a11, a22, a11 + a12, a21 - a11, a12 - a22]


def _sb(b11, b12, b21, b22):
    return [b11 + b22, b11, b12 - b22, b21 - b11, b22, b11 + b12, b21 + b22]


def _ppos(i, j):
    return ((j - 1) * 4 + (i - 1) // 2) * 64, ((i - 1) % 2) * PW


def _rpos(ct):
    return RROW + (ct // 2) * 40, (ct % 2) * PW


_VT = [
    69, 74, 88, 142, 97, 108, 86, 159, 180, 74, 74, 71, 177, 165, 54, 224,
    205, 111, 54, 159, 110, 74, 73, 124, 197, 115, 102, 54, 173, 166, 75, 210,
    186, 112, 69, 140, 144, 74, 74, 122, 180, 98, 114, 61, 173, 181, 60, 206,
    202, 79, 73, 90, 160, 108, 108, 71, 196, 128, 74, 90, 53, 190, 169, 207,
    216]
_ST = [
    17, 54, 35, 55, 19, 52, 59, 40, 54, 18, 54, 10, 17, 19, 12, 21, 55, 56,
    23, 55, 39, 40, 41, 73, 53, 44, 56, 2, 16, 18, 12, 17, 19, 53, 56, 40, 54,
    19, 54, 59, 55, 20, 53, 20, 16, 18, 2, 16, 21, 40, 42, 54, 53, 43, 56, 43,
    53, 41, 45, 38, 9, 17, 46, 19, 18]
_TWEAK_N = [
    1.0, 1.0, 1.0, 1.0, 1.0, 1.0, 1.0, 1.0, 1.0, 1.0, 0.7387, 1.0, 1.2613,
    1.0, 1.0, 1.0, 1.0, 1.0, 1.0, 1.0, 1.0, 1.0, 1.0, 1.0, 1.0, 1.0, 1.0, 1.0,
    1.0, 1.0, 1.0, 1.0, 1.0, 1.0, 1.0, 1.0, 1.0, 1.0, 0.8802, 1.1198, 1.0,
    1.0, 1.0, 1.0, 1.0, 1.0, 1.0, 1.0, 1.0, 1.0, 1.0, 0.8967, 1.1033, 1.0,
    0.7503, 1.0, 1.2497, 0.9599, 1.0401, 1.0, 1.0, 1.0, 1.0, 1.0, 1.0]
_TWEAK_S = [
    1.0, 1.0, 1.0, 1.0, 1.0, 1.0, 1.0, 1.0671, 1.0, 0.9329, 1.0, 1.0, 1.0,
    1.0, 1.0, 1.0, 1.0, 1.0, 1.0, 1.0, 1.0, 1.0, 1.0, 1.0, 1.0, 1.0, 1.0, 1.0,
    1.0, 1.0, 1.0, 1.0, 1.0, 1.0, 1.0, 1.0, 1.0, 1.0, 0.8505, 1.0, 1.0, 1.0,
    1.1489, 0.8511, 1.0, 1.0, 1.0, 1.0, 1.0, 1.0, 1.0, 1.0, 1.0, 0.5428, 1.0,
    1.2631, 1.0, 1.2321, 1.0, 0.7679, 1.0, 1.0, 0.9074, 1.0, 1.0]
_NCOST = []
for _k in range(8):
    _NCOST += [13, 13, 9, 12, 17, 17, 9, 12, 17, 17, 9, 12, 17, 12, 9, 12, 17,
               17, 9, 12, 17, 12] + ([16, 16] if _k % 2 == 0 else [])

_FIRST_WAITS = {17: (2, 3), 39: (4, 5)}
_FIRST_TASKS = [
    ("S", 1, 0, 5.21),
    ("N", 1, 5.21, 14.69),
    ("S", 2, 17, 19.63),
    ("N", 2, 19.63, 30.2835),
    ("S", 3, 19.63, 29.7835),
    ("N", 3, 30.2835, 39),
    ("S", 4, 39, 42.84),
    ("S", 5, 42.84, 53.1984),
    ("N", 4, 42.84, 53.6984),
    ("N", 5, 53.6984, 65),
]
_LOOP_TASKS = [
    ("S", 2, 0, 4.8),
    ("S", 3, 4.8, 14.64),
    ("N", 2, 4.8, 19.85),
    ("S", 4, 14.64, 29.69),
    ("N", 3, 19.85, 34.9),
    ("S", 5, 29.69, 44.74),
    ("N", 4, 34.9, 49.95),
    ("N", 5, 49.95, 65.0),
]

_ORDER = {
    ("put", 0): "m1 m2 m4 m6 m3 m5 m7",
    ("put", 1): "m1 m2 m4 m3 m5 m6 m7",
    ("put", 2): "m1 m6 m2 m3 m4 m5 m7",
    ("put", 3): "m2 m1 m3 m5 m6 m4 m7",
    ("sep", 0): "m1 m2 m4 m7 m3 m5 r11 r12 m6 r21 r22",
    ("sep", 1): "m1 m2 m4 m3 m6 r21 r22 m5 m7 r11 r12",
    ("sep", 2): "m3 m4 m1 m2 m6 r21 m5 m7 r11 r12 r22",
    ("sep", 3): "m3 m1 m2 m4 m6 m5 m7 r11 r12 r21 r22",
    ("merge", 0): "m3 m6 r12 r22 m1 m2 m4 r21 m5 m7 r11",
    ("merge", 1): "m3 m6 r22 m1 m2 m4 r21 m5 m7 r11 r12",
    ("merge", 2): "m6 r22 m4 m7 r11 r21 m1 m3 m5 r12 m2",
    ("merge", 3): "m1 m3 m6 r12 r22 m2 m4 m7 r21 m5 r11",
    ("early", 3): "m3 m1 m2 m4 m6 m5 m7",
}
_TERMS = {"11": {"m1": 1, "m7": 1, "m5": -1, "m4": 1},
          "12": {"m3": 1, "m5": 1},
          "21": {"m2": 1, "m4": 1},
          "22": {"m1": 1, "m3": 1, "m6": 1, "m2": -1}}


def _stats_pair(x, gates):
    c = jnp.broadcast_to(x[0:1, :], (8, W2))
    a1 = a2 = None
    if gates:
        for k in range(D // 8):
            v = x[k * 8:(k + 1) * 8] - gates[k](c, 2)
            a1 = v if a1 is None else a1 + v
            a2 = v * v if a2 is None else a2 + v * v
    else:
        c4 = cat([c] * 4, axis=0)
        for k in range(D // 32):
            v = x[k * 32:(k + 1) * 32] - c4
            sq = v * v
            if a1 is not None:
                v = cat([a1, v], axis=0)
                sq = cat([a2, sq], axis=0)
            a1 = jnp.sum(v.reshape(-1, 8, W2), axis=0)
            a2 = jnp.sum(sq.reshape(-1, 8, W2), axis=0)
    a1 = jnp.sum(a1, axis=0, keepdims=True) * (1.0 / D)
    a2 = jnp.sum(a2, axis=0, keepdims=True) * (1.0 / D)
    m = c[0:1] + a1
    var = jnp.maximum(a2 - a1 * a1, 0.0)
    r = lax.rsqrt(var + EPS)
    return jnp.broadcast_to(m, (8, W2)), jnp.broadcast_to(r, (8, W2))


def _stats_quad(x, gates):
    h = len(gates) // 2
    ma, ra = _stats_pair(x[:, 0:W2], gates[:h])
    mb, rb = _stats_pair(x[:, W2:], gates[h:])
    return cat([ma, mb], axis=1), cat([ra, rb], axis=1)


def _norm_quad(x, m, r, p_ref, gates):
    def tiles(v, tc):
        return cat([v[:, tc * PW:(tc + 1) * PW],
                    v[:, (tc + 2) * PW:(tc + 3) * PW]], axis=1)

    def wide(v):
        return cat([cat([v, v], axis=1)] * 2, axis=0)

    xt = [tiles(x, 0), tiles(x, 1)]
    mt = [tiles(m, 0), tiles(m, 1)]
    rt = [wide(tiles(r, 0)), wide(tiles(r, 1))]
    ms = [m[:, c * PW:(c + 1) * PW] for c in range(4)]
    r16 = cat([r, r], axis=0)
    it = iter(gates)

    def sub(k, kr, tc):
        mg = mt[tc]
        if gates:
            mg = cat([next(it)(ms[tc], 1), next(it)(ms[tc + 2], 1)], axis=1)
        r0 = kr * 128 + k * 16
        xb = cat([xt[tc][r0:r0 + 16], xt[tc][KH + r0:KH + r0 + 16]], axis=1)
        return (xb - wide(mg)) * rt[tc]

    def emit(k, j, v):
        q = [v[:, i * PW:(i + 1) * PW] for i in range(4)]
        if gates:
            q[0] = next(it)(q[0], 0)
            q[3] = next(it)(q[3], 0)
        ops = _sb(*q)
        for i0 in range(0, 7, 2):
            grp = ops[i0:i0 + 2]
            r0 = _ppos(i0 + 1, j)[0] + k * 8
            p_ref[r0:r0 + 8, 0:len(grp) * PW] = pltpu.bitcast(
                cat(grp, axis=1).astype(bf16), u32)

    for k in range(8):
        b11 = sub(k, 0, 0)
        emit(k, 2, b11)
        b12 = sub(k, 0, 1)
        emit(k, 6, b11 + b12)
        b22 = sub(k, 1, 1)
        emit(k, 3, b12 - b22)
        emit(k, 1, b11 + b22)
        emit(k, 5, b22)
        b21 = sub(k, 1, 0)
        emit(k, 4, b21 - b11)
        emit(k, 7, b21 + b22)
        if k % 2 == 0:
            mg = m
            if gates:
                mg = cat([next(it)(m[:, 0:W2], 2), next(it)(m[:, W2:], 2)],
                         axis=1)
            r0 = 2 * KH + k * 8
            v = (x[r0:r0 + 16] - cat([mg, mg], axis=0)) * r16
            for c0 in (0, 2):
                r1 = _rpos(c0)[0] + k * 4
                p_ref[r1:r1 + 8, :] = pltpu.bitcast(
                    v[:, c0 * PW:(c0 + 2) * PW].astype(bf16), u32)


def _kernel(x_hbm, g_hbm, b_hbm, w_hbm, o_hbm, xbuf, obuf,
            p0, p1, p2, p3, u0, u1, u2, u3, u4,
            g_ref, b_ref, w_ref, a_ref, ar_ref, zs, sin, sout):
    ps = [p0, p1, p2, p3]
    us = [u0, u1, u2, u3, u4]
    for i in range(4):
        zs[i] = 0

    def cin_last():
        return pltpu.make_async_copy(
            x_hbm.at[S - 1], xbuf.at[S - 1], sin.at[NI - 1])

    def cin_pair(j):
        rows = pl.ds(3 + 2 * j, 2)
        return pltpu.make_async_copy(x_hbm.at[rows], xbuf.at[rows], sin.at[j])

    def cin_quad(n):
        t, c = divmod(n, 2)
        return pltpu.make_async_copy(
            x_hbm.at[t, :, c * W4:(c + 1) * W4],
            xbuf.at[t, :, c * W4:(c + 1) * W4], sin.at[NI + 3 + n])

    def cout(sl, r0, r1, ct):
        idx = (sl, slice(r0, r1), slice(ct * PW, (ct + 1) * PW))
        pltpu.make_async_copy(
            obuf.at[idx], o_hbm.at[idx], sout.at[0]).start(priority=ct % 2)

    def cout_quad(t, c):
        for ct in range(4):
            cout(t, 0, D, 4 * c + ct)

    cw = pltpu.make_async_copy(w_hbm, w_ref, sin.at[NI])
    cg = pltpu.make_async_copy(g_hbm, g_ref, sin.at[NI + 1])
    cb = pltpu.make_async_copy(b_hbm, b_ref, sin.at[NI + 2])
    cg.start()
    cb.start()
    cw.start()
    for n in range(NH):
        cin_quad(n).start()
    for j in range(NI - 1):
        cin_pair(j).start()
    cin_last().start()

    row16 = lax.broadcasted_iota(jnp.int32, (16, W2), 0)
    ones = pltpu.bitcast(jnp.where(row16 < 3, 1.0, 0.0).astype(bf16), u32)
    for p_ref in ps:
        for c0 in (0, 2):
            r1 = _rpos(c0)[0] + 32
            p_ref[r1:r1 + 8, :] = ones

    cg.wait()
    cb.wait()
    cw.wait()
    g = g_ref[...].astype(f32).reshape(1, D)
    w = w_ref[...]
    b16 = jnp.broadcast_to(b_ref[...].reshape(1, D), (16, D))
    bias = jnp.dot(b16, w, preferred_element_type=f32)[0:8]
    bh = bias.astype(bf16).astype(f32)
    bl = (bias - bh).astype(bf16).astype(f32)
    bl2 = bias - bh - bl
    row8 = lax.broadcasted_iota(jnp.int32, (8, D), 0)
    ext = jnp.where(row8 == 0, bh,
                    jnp.where(row8 == 1, bl, jnp.where(row8 == 2, bl2, 0.0)))
    wf = w.astype(f32)
    wr = cat([wf[2 * KH:], ext, jnp.zeros((56, D), f32)], axis=0)
    wg = wf[:2 * KH].T * g[:, :2 * KH]
    gr = cat([g[:, 2 * KH:], jnp.ones((1, 64), f32)], axis=1)
    a1 = _sa(wg[0:H, 0:KH], wg[0:H, KH:], wg[H:, 0:KH], wg[H:, KH:])
    for i in range(1, 8):
        top, bot = a1[i - 1][0:Q], a1[i - 1][Q:]
        if i in PERM:
            top, bot = bot, top
        a2 = _sa(top[:, 0:128], top[:, 128:], bot[:, 0:128], bot[:, 128:])
        a_ref[:, (i - 1) * PW:i * PW] = pltpu.bitcast(
            cat(a2, axis=0).astype(bf16), u32)
    arv = (wr.T * gr).astype(bf16)
    ar_ref[:, 0:PW] = pltpu.bitcast(arv[0:H], u32)
    ar_ref[:, PW:] = pltpu.bitcast(arv[H:], u32)

    cin_quad(0).wait()
    _norm_quad(xbuf[zs[2], :, 0:W4].astype(f32),
               *_stats_quad(xbuf[zs[0], :, 0:W4].astype(f32), []), ps[0], [])

    def run(s, fresh, waits, tasks, hooks, bubble, valu, vst, ratio, tweak):
        k1 = s + zs[0]
        k2 = s + zs[2]
        never = {n: lax.broadcasted_iota(
            jnp.int32, (8, n * PW) if n else (16, PW), 0) < zs[1]
                 for n in (0, 1, 2)}
        zero = pl.multiple_of(zs[3], 8)
        nq = 4
        nr = 65
        free = [max(valu - _VT[r], 0) for r in range(nr)]
        tn = _TWEAK_N if tweak else [1] * 65
        ts = _TWEAK_S if tweak else [1] * 65
        wn = [(min(free[r], max(vst - _ST[r], 0) * ratio) + 0.01)
              * tn[r] for r in range(nr)]
        sc = sum(_NCOST) * nq / sum(wn)
        ws = [(max(free[r] - wn[r] * sc, 0) + 0.01) * ts[r]
              for r in range(nr)]

        def xload(k, q):
            t, c = divmod(q, 2)
            return xbuf[jnp.minimum(k + t, S - 1), :,
                        c * W4:(c + 1) * W4].astype(f32)

        def make_gate(e):
            if e is None:
                return lambda v, n: v

            def gate(v, n):
                z = e[0][e[1]:e[1] + 8]
                if n != 1:
                    z = cat([z, z], axis=1 if n else 0)
                return lax.select(never[n], z, v)
            return gate

        mr = {}
        first = {}
        todo = list(tasks)

        def flush(now):
            for task in [t for t in todo if t[3] <= now + 1e-9]:
                todo.remove(task)
                kind, q, t0, t1 = task
                wt = wn if kind == "N" else ws
                cand = []
                a = 0.0
                if t0 == 0 or t0 in waits:
                    cand.append((0.0, None))
                    a += bubble[kind]
                for r in range(int(t0), nr):
                    for e in range(NPER):
                        if t0 - 1e-9 <= r + e / NPER < t1 - 1e-9:
                            cand.append(
                                (a, (first[r], Q * e // NPER // 8 * 8)))
                            a += wt[r] / NPER
                costs = _NCOST if kind == "N" else [1] * (D // 4)
                done = 0
                gates = []
                for x in costs:
                    tgt = a * done / sum(costs)
                    gates.append(make_gate(
                        [e for (c, e) in cand if c <= tgt + 1e-9][-1]))
                    done += x
                if kind == "N":
                    _norm_quad(xload(k2, q), *mr.pop(q), ps[q % 4], gates)
                else:
                    mr[q] = _stats_quad(xload(k1, q), gates)

        count = [0]

        def mxu(lhs, rhs):
            r, o = divmod(count[0], 4)
            if o == 0 and r in waits:
                flush(r)
                waits[r]()
            v = jnp.dot(lhs(), rhs(), preferred_element_type=f32)
            if o == 0:
                first[r] = v
            count[0] += 1
            return v

        def get(i):
            return us[i][pl.ds(zero, H), :]

        def get_sub(i, hr, hc):
            return us[i][pl.ds(pl.multiple_of(zero + hr * Q, 8), Q),
                         hc * PW:(hc + 1) * PW]

        def quad(p):
            sl = s + p // 2
            c0 = (p % 2) * W4
            p_ref = ps[p % 4]
            if p in fresh:
                p_ref = p_ref.at[pl.ds(zero, BROWS), :]

            def hook(name):
                if (p, name) in hooks:
                    hooks[(p, name)]()

            def dot(i, j):
                r1, c1 = _ppos(i, j)
                return mxu(
                    lambda: pltpu.bitcast(
                        a_ref[(j - 1) * 72:j * 72, (i - 1) * PW:i * PW], bf16),
                    lambda: pltpu.bitcast(
                        p_ref[r1:r1 + 64, c1:c1 + PW], bf16))

            def rem(half, cc, hr, hc):
                r1, c1 = _rpos(2 * cc + hc)
                return mxu(
                    lambda: pltpu.bitcast(
                        ar_ref[hr * 72:(hr + 1) * 72,
                               half * PW:(half + 1) * PW], bf16)[:, :KR],
                    lambda: pltpu.bitcast(
                        p_ref[r1:r1 + 40, c1:c1 + PW], bf16))

            def prod(i, o=None, sep=None, plus=(), minus=()):
                sw = 1 if i in PERM else 0

                def blk(c):
                    rows = [cat([c["11"], c["12"]], axis=1),
                            cat([c["21"], c["22"]], axis=1)]
                    return cat(rows[::-1] if sw else rows, axis=0)

                kind = "sep" if i in (4, 5) else "merge" if o else "put"
                seq = _ORDER[("early" if sep else kind, count[0] % 4)].split()
                acc = {}
                sign = {}
                sep = dict(sep or {})
                for n, nm in enumerate(seq):
                    if nm[0] == "m":
                        v = dot(i, int(nm[1]))
                    else:
                        v = rem(o[0], o[1], (int(nm[1]) - 1) ^ sw,
                                int(nm[2]) - 1)
                        sep[nm[1:]] = v
                    for k, terms in _TERMS.items():
                        sg = terms.get(nm)
                        if kind == "merge" and nm == "r" + k:
                            sg = 1
                        if sg is None:
                            continue
                        if k not in acc:
                            acc[k], sign[k] = v, sg
                        elif sign[k] < 0:
                            acc[k], sign[k] = v - acc[k], 1
                        else:
                            acc[k] = acc[k] + v if sg > 0 else acc[k] - v
                    if plus and n == len(seq) - 5:
                        for k in _TERMS:
                            hr, hc = (int(k[0]) - 1) ^ sw, int(k[1]) - 1
                            for u in plus:
                                acc[k] = acc[k] + get_sub(u, hr, hc)
                            for u in minus:
                                acc[k] = acc[k] - get_sub(u, hr, hc)
                return blk(acc), blk(sep) if kind == "sep" else None

            def out(i, o, plus, minus=(), sep=None):
                if i == 6 and p == nq - 1:
                    val, v = prod(i, o, None, plus, minus)
                    plus = minus = ()
                else:
                    val, v = prod(i, o, sep)
                if o == (1, 1):
                    hook("m6")
                v = val if v is None else val + v
                for u in plus:
                    v = v + get(u)
                for u in minus:
                    v = v - get(u)
                obuf[sl, o[0] * H:(o[0] + 1) * H,
                     c0 + o[1] * W2:c0 + (o[1] + 1) * W2] = v.astype(bf16)
                return val

            early = None
            if p == 0:
                early = {k: rem(0, 1, (int(k[0]) - 1) ^ 1, int(k[1]) - 1)
                         for k in _TERMS}
            us[0][...] = prod(3)[0]
            hook("m3")
            us[1][...] = out(5, (0, 1), [0], sep=early)
            us[2][...] = prod(2)[0]
            hook("m2")
            m4 = out(4, (1, 0), [2])
            us[3][...] = m4 - get(1)
            us[4][...] = prod(1)[0]
            hook("m1")
            out(7, (0, 0), [3, 4])
            out(6, (1, 1), [0, 4], [2])

        for p in range(nq):
            flush(-(-count[0] // 4))
            quad(p)
        flush(nr)

    def wait_quads(ns):
        return lambda: [cin_quad(n).wait() for n in ns]

    cin_quad(1).wait()
    run(0, (1, 2, 3), {r: wait_quads(ns) for r, ns in _FIRST_WAITS.items()},
        _FIRST_TASKS, {}, {"N": 125, "S": 176}, 467, 125, 4.61, False)

    j_flush = (DEFER - 2) // 2

    def write_part(half, cc):
        for k in range(2):
            cout(S - 1, half * H, (half + 1) * H, 4 + 2 * cc + k)

    def body(j, carry):
        s = 2 + 2 * j

        @pl.when(j < NI - 1)
        def _():
            cin_pair(j).wait()

        @pl.when(j == NI - 1)
        def _():
            cin_last().wait()

        def write_prev(p):
            def fn():
                if p == 0:
                    @pl.when(j == j_flush)
                    def _():
                        for ct in range(8):
                            cout(pl.ds(0, DEFER), 0, D, ct)

                @pl.when(j > j_flush if p == 0 else j >= j_flush)
                def _():
                    cout_quad(s + (p - 1) // 2, (p - 1) % 2)
            return fn

        def write_last(half, cc):
            return lambda: pl.when(j == NI - 1)(
                lambda: write_part(half, cc))

        hooks = {(p, "m3"): write_prev(p) for p in range(4)}
        hooks.update({(3, "m2"): write_last(0, 1), (3, "m1"): write_last(1, 0),
                      (3, "m6"): write_last(0, 0)})
        run(s, (2, 3), {}, _LOOP_TASKS, hooks, {"N": 0.01, "S": 400},
            424, 111, 4.32, True)
        return carry

    lax.fori_loop(0, NI, body, 0)
    write_part(1, 1)
    pltpu.make_async_copy(obuf, o_hbm, sout.at[0]).wait()


@jax.jit
def pallas_standalone__layernorm_linear__sampling_kernel(
    x: jax.Array,
    g: jax.Array,
    b: jax.Array,
    w: jax.Array,
):
    assert x.shape == (B, S, D) and w.shape == (D, D)
    xt = jnp.transpose(x, (1, 2, 0))
    out = pl.pallas_call(
        _kernel,
        in_specs=[pl.BlockSpec(memory_space=pl.ANY)] * 4,
        out_specs=pl.BlockSpec(memory_space=pl.ANY),
        out_shape=jax.ShapeDtypeStruct((S, D, B), x.dtype),
        scratch_shapes=[
            pltpu.VMEM((S, D, B), bf16),
            pltpu.VMEM((S, D, B), bf16),
        ] + [pltpu.VMEM((BROWS, W2), u32)] * 4
        + [pltpu.VMEM((H, W2), f32)] * 5
        + [
            pltpu.VMEM((D,), bf16),
            pltpu.VMEM((D,), bf16),
            pltpu.VMEM((D, D), bf16),
            pltpu.VMEM((7 * 72, 7 * PW), u32),
            pltpu.VMEM((144, W2), u32),
            pltpu.SMEM((4,), jnp.int32),
            pltpu.SemaphoreType.DMA((NI + 3 + NH,)),
            pltpu.SemaphoreType.DMA((1,)),
        ],
        compiler_params=pltpu.CompilerParams(
            vmem_limit_bytes=110 * 1024 * 1024,
            disable_bounds_checks=True,
            disable_semaphore_checks=True,
        ),
    )(xt, g, b, w)
    return jnp.transpose(out, (2, 0, 1))
```

```python
import jax
import jax.numpy as jnp
from jax import lax
import jax.experimental.pallas as pl
import jax.experimental.pallas.tpu as pltpu

EPS = 1e-5
D = 576
S = 32
B = 1024
H = D // 2
Q = D // 4
KH = 256
KR = 80
PW = 128
W2 = 2 * PW
W4 = 4 * PW
NH = 6
NI = 15
DEFER = 14
NPER = 18
f32 = jnp.float32
bf16 = jnp.bfloat16
u32 = jnp.uint32
cat = jnp.concatenate
PERM = (3, 5, 6, 7)
RROW = 28 * 64
BROWS = RROW + 80


def _sa(a11, a12, a21, a22):
    return [a11 + a22, a21 + a22, a11, a22, a11 + a12, a21 - a11, a12 - a22]


def _sb(b11, b12, b21, b22):
    return [b11 + b22, b11, b12 - b22, b21 - b11, b22, b11 + b12, b21 + b22]


def _ppos(i, j):
    return ((j - 1) * 4 + (i - 1) // 2) * 64, ((i - 1) % 2) * PW


def _rpos(ct):
    return RROW + (ct // 2) * 40, (ct % 2) * PW


_VT = [
    69, 74, 88, 142, 97, 108, 86, 159, 180, 74, 74, 71, 177, 165, 54, 224,
    205, 111, 54, 159, 110, 74, 73, 124, 197, 115, 102, 54, 173, 166, 75, 210,
    186, 112, 69, 140, 144, 74, 74, 122, 180, 98, 114, 61, 173, 181, 60, 206,
    202, 79, 73, 90, 160, 108, 108, 71, 196, 128, 74, 90, 53, 190, 169, 207,
    216]
_ST = [
    17, 54, 35, 55, 19, 52, 59, 40, 54, 18, 54, 10, 17, 19, 12, 21, 55, 56,
    23, 55, 39, 40, 41, 73, 53, 44, 56, 2, 16, 18, 12, 17, 19, 53, 56, 40, 54,
    19, 54, 59, 55, 20, 53, 20, 16, 18, 2, 16, 21, 40, 42, 54, 53, 43, 56, 43,
    53, 41, 45, 38, 9, 17, 46, 19, 18]
_TWEAK_N = [
    1.0, 1.0, 1.0, 1.0, 1.0, 1.0, 1.0, 1.0, 1.0, 1.0, 1.0, 1.0, 1.0, 1.0, 1.0,
    1.0, 1.0, 1.0, 1.0, 1.0, 1.0, 1.0, 1.0, 1.0, 1.0, 1.0, 1.0, 1.0, 1.0, 1.0,
    1.0, 1.0, 1.0, 1.0, 1.0, 1.0, 1.0, 1.0, 1.0, 1.0, 1.0, 1.0, 1.0, 1.0, 1.0,
    1.0, 1.0, 1.0, 0.8928, 1.0, 1.1072, 1.0, 1.0, 1.0, 1.0, 1.0, 1.0, 1.0,
    0.7203, 1.2478, 1.0424, 1.0, 1.2017, 0.7983, 1.0]
_TWEAK_S = [
    1.0, 1.0, 1.0, 1.0, 1.0, 1.0, 1.0, 1.0, 1.0, 1.0, 1.0, 1.0, 1.0, 1.0, 1.0,
    1.0, 0.7353, 0.7965, 1.0, 1.0, 1.0, 1.0, 1.0, 1.0, 1.0, 1.0, 1.0, 1.0,
    1.0, 1.0, 1.0, 1.0, 1.0, 1.0, 1.0, 1.0, 1.0, 1.0, 1.0, 1.1102, 0.9512,
    0.9332, 1.0, 1.0, 1.0, 1.0445, 0.7247, 1.1393, 1.0824, 1.0, 1.0, 1.0,
    1.0425, 1.0, 0.9575, 1.0, 1.0, 1.0, 1.0, 1.0, 1.1749, 0.8251, 1.0, 1.0,
    1.0]
_NCOST = []
for _k in range(8):
    _NCOST += [13, 13, 9, 12, 17, 17, 9, 12, 17, 17, 9, 12, 17, 12, 9, 12, 17,
               17, 9, 12, 17, 12] + ([16, 16] if _k % 2 == 0 else [])

_FIRST_WAITS = {17: (2, 3), 39: (4, 5)}
_FIRST_TASKS = [
    ("S", 1, 0, 5.21),
    ("N", 1, 5.21, 14.69),
    ("S", 2, 17, 19.63),
    ("N", 2, 19.63, 30.2835),
    ("S", 3, 19.63, 29.7835),
    ("N", 3, 30.2835, 39),
    ("S", 4, 39, 42.84),
    ("S", 5, 42.84, 53.1984),
    ("N", 4, 42.84, 53.6984),
    ("N", 5, 53.6984, 65),
]
_LOOP_TASKS = [
    ("S", 2, 0, 4.97),
    ("S", 3, 4.97, 14.0775),
    ("N", 2, 4.97, 19.9775),
    ("S", 4, 14.0775, 29.085),
    ("N", 3, 19.9775, 34.985),
    ("S", 5, 29.085, 44.0925),
    ("N", 4, 34.985, 49.9925),
    ("N", 5, 49.9925, 65.0),
]

_ORDER = {
    ("put", 0): "m1 m2 m4 m6 m3 m5 m7",
    ("put", 1): "m1 m2 m4 m3 m5 m6 m7",
    ("put", 2): "m1 m6 m2 m3 m4 m5 m7",
    ("put", 3): "m2 m1 m3 m5 m6 m4 m7",
    ("sep", 0): "m1 m2 m4 m7 m3 m5 r11 r12 m6 r21 r22",
    ("sep", 1): "m1 m2 m4 m3 m6 r21 r22 m5 m7 r11 r12",
    ("sep", 2): "m3 m4 m1 m2 m6 r21 m5 m7 r11 r12 r22",
    ("sep", 3): "m3 m1 m2 m4 m6 m5 m7 r11 r12 r21 r22",
    ("merge", 0): "m3 m6 r12 r22 m1 m2 m4 r21 m5 m7 r11",
    ("merge", 1): "m3 m6 r22 m1 m2 m4 r21 m5 m7 r11 r12",
    ("merge", 2): "m6 r22 m4 m7 r11 r21 m1 m3 m5 r12 m2",
    ("merge", 3): "m1 m3 m6 r12 r22 m2 m4 m7 r21 m5 r11",
    ("early", 3): "m3 m1 m2 m4 m6 m5 m7",
}
_TERMS = {"11": {"m1": 1, "m7": 1, "m5": -1, "m4": 1},
          "12": {"m3": 1, "m5": 1},
          "21": {"m2": 1, "m4": 1},
          "22": {"m1": 1, "m3": 1, "m6": 1, "m2": -1}}


def _stats_pair(x, gates):
    c = jnp.broadcast_to(x[0:1, :], (8, W2))
    a1 = a2 = None
    if gates:
        for k in range(D // 8):
            v = x[k * 8:(k + 1) * 8] - gates[k](c, 2)
            a1 = v if a1 is None else a1 + v
            a2 = v * v if a2 is None else a2 + v * v
    else:
        c4 = cat([c] * 4, axis=0)
        for k in range(D // 32):
            v = x[k * 32:(k + 1) * 32] - c4
            sq = v * v
            if a1 is not None:
                v = cat([a1, v], axis=0)
                sq = cat([a2, sq], axis=0)
            a1 = jnp.sum(v.reshape(-1, 8, W2), axis=0)
            a2 = jnp.sum(sq.reshape(-1, 8, W2), axis=0)
    a1 = jnp.sum(a1, axis=0, keepdims=True) * (1.0 / D)
    a2 = jnp.sum(a2, axis=0, keepdims=True) * (1.0 / D)
    m = c[0:1] + a1
    var = jnp.maximum(a2 - a1 * a1, 0.0)
    r = lax.rsqrt(var + EPS)
    return jnp.broadcast_to(m, (8, W2)), jnp.broadcast_to(r, (8, W2))


def _stats_quad(x, gates):
    h = len(gates) // 2
    ma, ra = _stats_pair(x[:, 0:W2], gates[:h])
    mb, rb = _stats_pair(x[:, W2:], gates[h:])
    return cat([ma, mb], axis=1), cat([ra, rb], axis=1)


def _norm_quad(x, m, r, p_ref, gates):
    def tiles(v, tc):
        return cat([v[:, tc * PW:(tc + 1) * PW],
                    v[:, (tc + 2) * PW:(tc + 3) * PW]], axis=1)

    def wide(v):
        return cat([cat([v, v], axis=1)] * 2, axis=0)

    xt = [tiles(x, 0), tiles(x, 1)]
    mt = [tiles(m, 0), tiles(m, 1)]
    rt = [wide(tiles(r, 0)), wide(tiles(r, 1))]
    ms = [m[:, c * PW:(c + 1) * PW] for c in range(4)]
    r16 = cat([r, r], axis=0)
    it = iter(gates)

    def sub(k, kr, tc):
        mg = mt[tc]
        if gates:
            mg = cat([next(it)(ms[tc], 1), next(it)(ms[tc + 2], 1)], axis=1)
        r0 = kr * 128 + k * 16
        xb = cat([xt[tc][r0:r0 + 16], xt[tc][KH + r0:KH + r0 + 16]], axis=1)
        return (xb - wide(mg)) * rt[tc]

    def emit(k, j, v):
        q = [v[:, i * PW:(i + 1) * PW] for i in range(4)]
        if gates:
            q[0] = next(it)(q[0], 0)
            q[3] = next(it)(q[3], 0)
        ops = _sb(*q)
        for i0 in range(0, 7, 2):
            grp = ops[i0:i0 + 2]
            r0 = _ppos(i0 + 1, j)[0] + k * 8
            p_ref[r0:r0 + 8, 0:len(grp) * PW] = pltpu.bitcast(
                cat(grp, axis=1).astype(bf16), u32)

    for k in range(8):
        b11 = sub(k, 0, 0)
        emit(k, 2, b11)
        b12 = sub(k, 0, 1)
        emit(k, 6, b11 + b12)
        b22 = sub(k, 1, 1)
        emit(k, 3, b12 - b22)
        emit(k, 1, b11 + b22)
        emit(k, 5, b22)
        b21 = sub(k, 1, 0)
        emit(k, 4, b21 - b11)
        emit(k, 7, b21 + b22)
        if k % 2 == 0:
            mg = m
            if gates:
                mg = cat([next(it)(m[:, 0:W2], 2), next(it)(m[:, W2:], 2)],
                         axis=1)
            r0 = 2 * KH + k * 8
            v = (x[r0:r0 + 16] - cat([mg, mg], axis=0)) * r16
            for c0 in (0, 2):
                r1 = _rpos(c0)[0] + k * 4
                p_ref[r1:r1 + 8, :] = pltpu.bitcast(
                    v[:, c0 * PW:(c0 + 2) * PW].astype(bf16), u32)


def _kernel(x_hbm, g_hbm, b_hbm, w_hbm, o_hbm, xbuf, obuf,
            p0, p1, p2, p3, u0, u1, u2, u3, u4,
            g_ref, b_ref, w_ref, a_ref, ar_ref, zs, sin, sout):
    ps = [p0, p1, p2, p3]
    us = [u0, u1, u2, u3, u4]
    for i in range(4):
        zs[i] = 0

    def cin_last():
        return pltpu.make_async_copy(
            x_hbm.at[S - 1], xbuf.at[S - 1], sin.at[NI - 1])

    def cin_pair(j):
        rows = pl.ds(3 + 2 * j, 2)
        return pltpu.make_async_copy(x_hbm.at[rows], xbuf.at[rows], sin.at[j])

    def cin_quad(n):
        t, c = divmod(n, 2)
        return pltpu.make_async_copy(
            x_hbm.at[t, :, c * W4:(c + 1) * W4],
            xbuf.at[t, :, c * W4:(c + 1) * W4], sin.at[NI + 3 + n])

    def cout(sl, r0, r1, ct):
        idx = (sl, slice(r0, r1), slice(ct * PW, (ct + 1) * PW))
        pltpu.make_async_copy(
            obuf.at[idx], o_hbm.at[idx], sout.at[0]).start(priority=ct % 2)

    def cout_quad(t, c):
        for ct in range(4):
            cout(t, 0, D, 4 * c + ct)

    cw = pltpu.make_async_copy(w_hbm, w_ref, sin.at[NI])
    cg = pltpu.make_async_copy(g_hbm, g_ref, sin.at[NI + 1])
    cb = pltpu.make_async_copy(b_hbm, b_ref, sin.at[NI + 2])
    cg.start()
    cb.start()
    cw.start()
    for n in range(NH):
        cin_quad(n).start()
    for j in range(NI - 1):
        cin_pair(j).start()
    cin_last().start()

    row16 = lax.broadcasted_iota(jnp.int32, (16, W2), 0)
    ones = pltpu.bitcast(jnp.where(row16 < 3, 1.0, 0.0).astype(bf16), u32)
    for p_ref in ps:
        for c0 in (0, 2):
            r1 = _rpos(c0)[0] + 32
            p_ref[r1:r1 + 8, :] = ones

    cg.wait()
    cb.wait()
    cw.wait()
    g = g_ref[...].astype(f32).reshape(1, D)
    w = w_ref[...]
    b16 = jnp.broadcast_to(b_ref[...].reshape(1, D), (16, D))
    bias = jnp.dot(b16, w, preferred_element_type=f32)[0:8]
    bh = bias.astype(bf16).astype(f32)
    bl = (bias - bh).astype(bf16).astype(f32)
    bl2 = bias - bh - bl
    row8 = lax.broadcasted_iota(jnp.int32, (8, D), 0)
    ext = jnp.where(row8 == 0, bh,
                    jnp.where(row8 == 1, bl, jnp.where(row8 == 2, bl2, 0.0)))
    wf = w.astype(f32)
    wr = cat([wf[2 * KH:], ext, jnp.zeros((56, D), f32)], axis=0)
    wg = wf[:2 * KH].T * g[:, :2 * KH]
    gr = cat([g[:, 2 * KH:], jnp.ones((1, 64), f32)], axis=1)
    a1 = _sa(wg[0:H, 0:KH], wg[0:H, KH:], wg[H:, 0:KH], wg[H:, KH:])
    for i in range(1, 8):
        top, bot = a1[i - 1][0:Q], a1[i - 1][Q:]
        if i in PERM:
            top, bot = bot, top
        a2 = _sa(top[:, 0:128], top[:, 128:], bot[:, 0:128], bot[:, 128:])
        a_ref[:, (i - 1) * PW:i * PW] = pltpu.bitcast(
            cat(a2, axis=0).astype(bf16), u32)
    arv = (wr.T * gr).astype(bf16)
    ar_ref[:, 0:PW] = pltpu.bitcast(arv[0:H], u32)
    ar_ref[:, PW:] = pltpu.bitcast(arv[H:], u32)

    cin_quad(0).wait()
    _norm_quad(xbuf[zs[2], :, 0:W4].astype(f32),
               *_stats_quad(xbuf[zs[0], :, 0:W4].astype(f32), []), ps[0], [])

    def run(s, fresh, waits, tasks, hooks, bubble, valu, vst, ratio, tweak):
        k1 = s + zs[0]
        k2 = s + zs[2]
        never = {n: lax.broadcasted_iota(
            jnp.int32, (8, n * PW) if n else (16, PW), 0) < zs[1]
                 for n in (0, 1, 2)}
        zero = pl.multiple_of(zs[3], 8)
        nq = 4
        nr = 65
        free = [max(valu - _VT[r], 0) for r in range(nr)]
        tn = _TWEAK_N if tweak else [1] * 65
        ts = _TWEAK_S if tweak else [1] * 65
        wn = [(min(free[r], max(vst - _ST[r], 0) * ratio) + 0.01)
              * tn[r] for r in range(nr)]
        sc = sum(_NCOST) * nq / sum(wn)
        ws = [(max(free[r] - wn[r] * sc, 0) + 0.01) * ts[r]
              for r in range(nr)]

        def xload(k, q):
            t, c = divmod(q, 2)
            return xbuf[jnp.minimum(k + t, S - 1), :,
                        c * W4:(c + 1) * W4].astype(f32)

        def make_gate(e):
            if e is None:
                return lambda v, n: v

            def gate(v, n):
                z = e[0][e[1]:e[1] + 8]
                if n != 1:
                    z = cat([z, z], axis=1 if n else 0)
                return lax.select(never[n], z, v)
            return gate

        mr = {}
        first = {}
        todo = list(tasks)

        def flush(now):
            for task in [t for t in todo if t[3] <= now + 1e-9]:
                todo.remove(task)
                kind, q, t0, t1 = task
                wt = wn if kind == "N" else ws
                cand = []
                a = 0.0
                if t0 == 0 or t0 in waits:
                    cand.append((0.0, None))
                    a += bubble[kind]
                for r in range(int(t0), nr):
                    for e in range(NPER):
                        if t0 - 1e-9 <= r + e / NPER < t1 - 1e-9:
                            cand.append(
                                (a, (first[r], Q * e // NPER // 8 * 8)))
                            a += wt[r] / NPER
                costs = _NCOST if kind == "N" else [1] * (D // 4)
                done = 0
                gates = []
                for x in costs:
                    tgt = a * done / sum(costs)
                    gates.append(make_gate(
                        [e for (c, e) in cand if c <= tgt + 1e-9][-1]))
                    done += x
                if kind == "N":
                    _norm_quad(xload(k2, q), *mr.pop(q), ps[q % 4], gates)
                else:
                    mr[q] = _stats_quad(xload(k1, q), gates)

        count = [0]

        def mxu(lhs, rhs):
            r, o = divmod(count[0], 4)
            if o == 0 and r in waits:
                flush(r)
                waits[r]()
            v = jnp.dot(lhs(), rhs(), preferred_element_type=f32)
            if o == 0:
                first[r] = v
            count[0] += 1
            return v

        def get(i):
            return us[i][pl.ds(zero, H), :]

        def get_sub(i, hr, hc):
            return us[i][pl.ds(pl.multiple_of(zero + hr * Q, 8), Q),
                         hc * PW:(hc + 1) * PW]

        def quad(p):
            sl = s + p // 2
            c0 = (p % 2) * W4
            p_ref = ps[p % 4]
            if p in fresh:
                p_ref = p_ref.at[pl.ds(zero, BROWS), :]

            def hook(name):
                if (p, name) in hooks:
                    hooks[(p, name)]()

            def dot(i, j):
                r1, c1 = _ppos(i, j)
                return mxu(
                    lambda: pltpu.bitcast(
                        a_ref[(j - 1) * 72:j * 72, (i - 1) * PW:i * PW], bf16),
                    lambda: pltpu.bitcast(
                        p_ref[r1:r1 + 64, c1:c1 + PW], bf16))

            def rem(half, cc, hr, hc):
                r1, c1 = _rpos(2 * cc + hc)
                return mxu(
                    lambda: pltpu.bitcast(
                        ar_ref[hr * 72:(hr + 1) * 72,
                               half * PW:(half + 1) * PW], bf16)[:, :KR],
                    lambda: pltpu.bitcast(
                        p_ref[r1:r1 + 40, c1:c1 + PW], bf16))

            def prod(i, o=None, sep=None, plus=(), minus=()):
                sw = 1 if i in PERM else 0

                def blk(c):
                    rows = [cat([c["11"], c["12"]], axis=1),
                            cat([c["21"], c["22"]], axis=1)]
                    return cat(rows[::-1] if sw else rows, axis=0)

                kind = "sep" if i in (4, 5) else "merge" if o else "put"
                seq = _ORDER[("early" if sep else kind, count[0] % 4)].split()
                acc = {}
                sign = {}
                sep = dict(sep or {})
                for n, nm in enumerate(seq):
                    if nm[0] == "m":
                        v = dot(i, int(nm[1]))
                    else:
                        v = rem(o[0], o[1], (int(nm[1]) - 1) ^ sw,
                                int(nm[2]) - 1)
                        sep[nm[1:]] = v
                    for k, terms in _TERMS.items():
                        sg = terms.get(nm)
                        if kind == "merge" and nm == "r" + k:
                            sg = 1
                        if sg is None:
                            continue
                        if k not in acc:
                            acc[k], sign[k] = v, sg
                        elif sign[k] < 0:
                            acc[k], sign[k] = v - acc[k], 1
                        else:
                            acc[k] = acc[k] + v if sg > 0 else acc[k] - v
                    if plus and n == len(seq) - 5:
                        for k in _TERMS:
                            hr, hc = (int(k[0]) - 1) ^ sw, int(k[1]) - 1
                            for u in plus:
                                acc[k] = acc[k] + get_sub(u, hr, hc)
                            for u in minus:
                                acc[k] = acc[k] - get_sub(u, hr, hc)
                return blk(acc), blk(sep) if kind == "sep" else None

            def out(i, o, plus, minus=(), sep=None):
                if i == 6 and p == nq - 1:
                    val, v = prod(i, o, None, plus, minus)
                    plus = minus = ()
                else:
                    val, v = prod(i, o, sep)
                if o == (1, 1):
                    hook("m6")
                v = val if v is None else val + v
                for u in plus:
                    v = v + get(u)
                for u in minus:
                    v = v - get(u)
                obuf[sl, o[0] * H:(o[0] + 1) * H,
                     c0 + o[1] * W2:c0 + (o[1] + 1) * W2] = v.astype(bf16)
                return val

            early = None
            if p == 0:
                early = {k: rem(0, 1, (int(k[0]) - 1) ^ 1, int(k[1]) - 1)
                         for k in _TERMS}
            us[0][...] = prod(3)[0]
            hook("m3")
            us[1][...] = out(5, (0, 1), [0], sep=early)
            us[2][...] = prod(2)[0]
            hook("m2")
            m4 = out(4, (1, 0), [2])
            us[3][...] = m4 - get(1)
            us[4][...] = prod(1)[0]
            hook("m1")
            out(7, (0, 0), [3, 4])
            out(6, (1, 1), [0, 4], [2])

        for p in range(nq):
            flush(-(-count[0] // 4))
            quad(p)
        flush(nr)

    def wait_quads(ns):
        return lambda: [cin_quad(n).wait() for n in ns]

    cin_quad(1).wait()
    run(0, (1, 2, 3), {r: wait_quads(ns) for r, ns in _FIRST_WAITS.items()},
        _FIRST_TASKS, {}, {"N": 125, "S": 176}, 467, 125, 4.61, False)

    j_flush = (DEFER - 2) // 2

    def write_part(half, cc):
        for k in range(2):
            cout(S - 1, half * H, (half + 1) * H, 4 + 2 * cc + k)

    def body(j, carry):
        s = 2 + 2 * j

        @pl.when(j < NI - 1)
        def _():
            cin_pair(j).wait()

        @pl.when(j == NI - 1)
        def _():
            cin_last().wait()

        def write_prev(p):
            def fn():
                if p == 0:
                    @pl.when(j == j_flush)
                    def _():
                        for ct in range(8):
                            cout(pl.ds(0, DEFER), 0, D, ct)

                @pl.when(j > j_flush if p == 0 else j >= j_flush)
                def _():
                    cout_quad(s + (p - 1) // 2, (p - 1) % 2)
            return fn

        def write_last(half, cc):
            return lambda: pl.when(j == NI - 1)(
                lambda: write_part(half, cc))

        hooks = {(p, "m3"): write_prev(p) for p in range(4)}
        hooks.update({(3, "m2"): write_last(0, 1), (3, "m1"): write_last(1, 0),
                      (3, "m6"): write_last(0, 0)})
        run(s, (2, 3), {}, _LOOP_TASKS, hooks, {"N": 0.01, "S": 550},
            441, 121, 5.86, True)
        return carry

    lax.fori_loop(0, NI, body, 0)
    write_part(1, 1)
    pltpu.make_async_copy(obuf, o_hbm, sout.at[0]).wait()


@jax.jit
def pallas_standalone__layernorm_linear__sampling_kernel(
    x: jax.Array,
    g: jax.Array,
    b: jax.Array,
    w: jax.Array,
):
    assert x.shape == (B, S, D) and w.shape == (D, D)
    xt = jnp.transpose(x, (1, 2, 0))
    out = pl.pallas_call(
        _kernel,
        in_specs=[pl.BlockSpec(memory_space=pl.ANY)] * 4,
        out_specs=pl.BlockSpec(memory_space=pl.ANY),
        out_shape=jax.ShapeDtypeStruct((S, D, B), x.dtype),
        scratch_shapes=[
            pltpu.VMEM((S, D, B), bf16),
            pltpu.VMEM((S, D, B), bf16),
        ] + [pltpu.VMEM((BROWS, W2), u32)] * 4
        + [pltpu.VMEM((H, W2), f32)] * 5
        + [
            pltpu.VMEM((D,), bf16),
            pltpu.VMEM((D,), bf16),
            pltpu.VMEM((D, D), bf16),
            pltpu.VMEM((7 * 72, 7 * PW), u32),
            pltpu.VMEM((144, W2), u32),
            pltpu.SMEM((4,), jnp.int32),
            pltpu.SemaphoreType.DMA((NI + 3 + NH,)),
            pltpu.SemaphoreType.DMA((1,)),
        ],
        compiler_params=pltpu.CompilerParams(
            vmem_limit_bytes=110 * 1024 * 1024,
            disable_bounds_checks=True,
            disable_semaphore_checks=True,
        ),
    )(xt, g, b, w)
    return jnp.transpose(out, (2, 0, 1))
```

```python
import jax
import jax.numpy as jnp
from jax import lax
import jax.experimental.pallas as pl
import jax.experimental.pallas.tpu as pltpu

EPS = 1e-5
D = 576
S = 32
B = 1024
H = D // 2
Q = D // 4
KH = 256
KR = 80
PW = 128
W2 = 2 * PW
W4 = 4 * PW
NH = 6
NI = 15
DEFER = 14
NPER = 18
f32 = jnp.float32
bf16 = jnp.bfloat16
u32 = jnp.uint32
cat = jnp.concatenate
PERM = (3, 5, 6, 7)
RROW = 28 * 64
BROWS = RROW + 80


def _sa(a11, a12, a21, a22):
    return [a11 + a22, a21 + a22, a11, a22, a11 + a12, a21 - a11, a12 - a22]


def _sb(b11, b12, b21, b22):
    return [b11 + b22, b11, b12 - b22, b21 - b11, b22, b11 + b12, b21 + b22]


def _ppos(i, j):
    return ((j - 1) * 4 + (i - 1) // 2) * 64, ((i - 1) % 2) * PW


def _rpos(ct):
    return RROW + (ct // 2) * 40, (ct % 2) * PW


_VT = [
    69, 74, 88, 142, 97, 108, 86, 159, 180, 74, 74, 71, 177, 165, 54, 224,
    205, 111, 54, 159, 110, 74, 73, 124, 197, 115, 102, 54, 173, 166, 75, 210,
    186, 112, 69, 140, 144, 74, 74, 122, 180, 98, 114, 61, 173, 181, 60, 206,
    202, 79, 73, 90, 160, 108, 108, 71, 196, 128, 74, 90, 53, 190, 169, 207,
    216]
_ST = [
    17, 54, 35, 55, 19, 52, 59, 40, 54, 18, 54, 10, 17, 19, 12, 21, 55, 56,
    23, 55, 39, 40, 41, 73, 53, 44, 56, 2, 16, 18, 12, 17, 19, 53, 56, 40, 54,
    19, 54, 59, 55, 20, 53, 20, 16, 18, 2, 16, 21, 40, 42, 54, 53, 43, 56, 43,
    53, 41, 45, 38, 9, 17, 46, 19, 18]
_TWEAK_N = [
    1.0, 1.0, 1.0, 1.0, 1.0, 1.0, 1.0, 1.0, 1.0, 1.0, 1.0, 1.0, 1.0, 1.0, 1.0,
    1.0, 1.0, 1.0, 1.0, 1.0, 1.0, 1.0, 1.0, 1.0, 1.0, 1.0, 1.0, 1.0, 1.0, 1.0,
    1.0, 1.0, 1.0, 1.0, 1.0, 1.0, 1.0, 1.0, 1.0, 1.0, 1.0, 1.0, 1.0, 1.0, 1.0,
    1.0, 1.0, 1.0, 0.8928, 1.0, 1.1072, 1.0, 1.0, 1.0, 1.0, 1.0, 1.0, 1.0,
    0.7203, 1.2478, 1.0424, 1.0, 1.2017, 0.7983, 1.0]
_TWEAK_S = [
    1.0, 1.0, 1.0, 1.0, 1.0, 1.0, 1.0, 1.0, 1.0, 1.0, 1.0, 1.0, 1.0, 1.0, 1.0,
    1.0, 0.7353, 0.7965, 1.0, 1.0, 1.0, 1.0, 1.0, 1.0, 1.0, 1.0, 1.0, 1.0,
    1.0, 1.0, 1.0, 1.0, 1.0, 1.0, 1.0, 1.0, 1.0, 1.0, 1.0, 1.1102, 0.9512,
    0.9332, 1.0, 1.0, 1.0, 1.0445, 0.7247, 1.1393, 1.0824, 1.0, 1.0, 1.0,
    1.0425, 1.0, 0.9575, 1.0, 1.0, 1.0, 1.0, 1.0, 1.1749, 0.8251, 1.0, 1.0,
    1.0]
_NCOST = []
for _k in range(8):
    _NCOST += [13, 13, 9, 12, 17, 17, 9, 12, 17, 17, 9, 12, 17, 12, 9, 12, 17,
               17, 9, 12, 17, 12] + ([16, 16] if _k % 2 == 0 else [])

_FIRST_WAITS = {17: (2, 3), 39: (4, 5)}
_FIRST_TASKS = [
    ("S", 1, 0, 5.21),
    ("N", 1, 5.21, 14.69),
    ("S", 2, 17, 19.63),
    ("N", 2, 19.63, 30.2835),
    ("S", 3, 19.63, 29.7835),
    ("N", 3, 30.2835, 39),
    ("S", 4, 39, 42.84),
    ("S", 5, 42.84, 53.1984),
    ("N", 4, 42.84, 53.6984),
    ("N", 5, 53.6984, 65),
]
_LOOP_TASKS = [
    ("S", 2, 0, 4.97),
    ("S", 3, 4.97, 14.0775),
    ("N", 2, 4.97, 19.9775),
    ("S", 4, 14.0775, 29.085),
    ("N", 3, 19.9775, 34.985),
    ("S", 5, 29.085, 44.0925),
    ("N", 4, 34.985, 49.9925),
    ("N", 5, 49.9925, 65.0),
]

_ORDER = {
    ("put", 0): "m1 m2 m4 m6 m3 m5 m7",
    ("put", 1): "m1 m2 m4 m3 m5 m6 m7",
    ("put", 2): "m1 m6 m2 m3 m4 m5 m7",
    ("put", 3): "m2 m1 m3 m5 m6 m4 m7",
    ("sep", 0): "m1 m2 m4 m7 m3 m5 r11 r12 m6 r21 r22",
    ("sep", 1): "m1 m2 m4 m3 m6 r21 r22 m5 m7 r11 r12",
    ("sep", 2): "m3 m4 m1 m2 m6 r21 m5 m7 r11 r12 r22",
    ("sep", 3): "m3 m1 m2 m4 m6 m5 m7 r11 r12 r21 r22",
    ("merge", 0): "m3 m6 r12 r22 m1 m2 m4 r21 m5 m7 r11",
    ("merge", 1): "m3 m6 r22 m1 m2 m4 r21 m5 m7 r11 r12",
    ("merge", 2): "m6 r22 m4 m7 r11 r21 m1 m3 m5 r12 m2",
    ("merge", 3): "m1 m3 m6 r12 r22 m2 m4 m7 r21 m5 r11",
    ("early", 3): "m3 m1 m2 m4 m6 m5 m7",
}
_TERMS = {"11": {"m1": 1, "m7": 1, "m5": -1, "m4": 1},
          "12": {"m3": 1, "m5": 1},
          "21": {"m2": 1, "m4": 1},
          "22": {"m1": 1, "m3": 1, "m6": 1, "m2": -1}}


def _stats_pair(x, gates):
    c = jnp.broadcast_to(x[0:1, :], (8, W2))
    a1 = a2 = None
    if gates:
        for k in range(D // 8):
            v = x[k * 8:(k + 1) * 8] - gates[k](c, 2)
            a1 = v if a1 is None else a1 + v
            a2 = v * v if a2 is None else a2 + v * v
    else:
        c4 = cat([c] * 4, axis=0)
        for k in range(D // 32):
            v = x[k * 32:(k + 1) * 32] - c4
            sq = v * v
            if a1 is not None:
                v = cat([a1, v], axis=0)
                sq = cat([a2, sq], axis=0)
            a1 = jnp.sum(v.reshape(-1, 8, W2), axis=0)
            a2 = jnp.sum(sq.reshape(-1, 8, W2), axis=0)
    a1 = jnp.sum(a1, axis=0, keepdims=True) * (1.0 / D)
    a2 = jnp.sum(a2, axis=0, keepdims=True) * (1.0 / D)
    m = c[0:1] + a1
    var = jnp.maximum(a2 - a1 * a1, 0.0)
    r = lax.rsqrt(var + EPS)
    return jnp.broadcast_to(m, (8, W2)), jnp.broadcast_to(r, (8, W2))


def _stats_quad(x, gates):
    h = len(gates) // 2
    ma, ra = _stats_pair(x[:, 0:W2], gates[:h])
    mb, rb = _stats_pair(x[:, W2:], gates[h:])
    return cat([ma, mb], axis=1), cat([ra, rb], axis=1)


def _norm_quad(x, m, r, p_ref, gates):
    def tiles(v, tc):
        return cat([v[:, tc * PW:(tc + 1) * PW],
                    v[:, (tc + 2) * PW:(tc + 3) * PW]], axis=1)

    def wide(v):
        return cat([cat([v, v], axis=1)] * 2, axis=0)

    xt = [tiles(x, 0), tiles(x, 1)]
    mt = [tiles(m, 0), tiles(m, 1)]
    rt = [wide(tiles(r, 0)), wide(tiles(r, 1))]
    ms = [m[:, c * PW:(c + 1) * PW] for c in range(4)]
    r16 = cat([r, r], axis=0)
    it = iter(gates)

    def sub(k, kr, tc):
        mg = mt[tc]
        if gates:
            mg = cat([next(it)(ms[tc], 1), next(it)(ms[tc + 2], 1)], axis=1)
        r0 = kr * 128 + k * 16
        xb = cat([xt[tc][r0:r0 + 16], xt[tc][KH + r0:KH + r0 + 16]], axis=1)
        return (xb - wide(mg)) * rt[tc]

    def emit(k, j, v):
        q = [v[:, i * PW:(i + 1) * PW] for i in range(4)]
        if gates:
            q[0] = next(it)(q[0], 0)
            q[3] = next(it)(q[3], 0)
        ops = _sb(*q)
        for i0 in range(0, 7, 2):
            grp = ops[i0:i0 + 2]
            r0 = _ppos(i0 + 1, j)[0] + k * 8
            p_ref[r0:r0 + 8, 0:len(grp) * PW] = pltpu.bitcast(
                cat(grp, axis=1).astype(bf16), u32)

    for k in range(8):
        b11 = sub(k, 0, 0)
        emit(k, 2, b11)
        b12 = sub(k, 0, 1)
        emit(k, 6, b11 + b12)
        b22 = sub(k, 1, 1)
        emit(k, 3, b12 - b22)
        emit(k, 1, b11 + b22)
        emit(k, 5, b22)
        b21 = sub(k, 1, 0)
        emit(k, 4, b21 - b11)
        emit(k, 7, b21 + b22)
        if k % 2 == 0:
            mg = m
            if gates:
                mg = cat([next(it)(m[:, 0:W2], 2), next(it)(m[:, W2:], 2)],
                         axis=1)
            r0 = 2 * KH + k * 8
            v = (x[r0:r0 + 16] - cat([mg, mg], axis=0)) * r16
            for c0 in (0, 2):
                r1 = _rpos(c0)[0] + k * 4
                p_ref[r1:r1 + 8, :] = pltpu.bitcast(
                    v[:, c0 * PW:(c0 + 2) * PW].astype(bf16), u32)


def _kernel(x_hbm, g_hbm, b_hbm, w_hbm, o_hbm, xbuf, obuf,
            p0, p1, p2, p3, u0, u1, u2, u3, u4,
            g_ref, b_ref, w_ref, a_ref, ar_ref, zs, sin, sout):
    ps = [p0, p1, p2, p3]
    us = [u0, u1, u2, u3, u4]
    for i in range(4):
        zs[i] = 0

    def cin_last():
        return pltpu.make_async_copy(
            x_hbm.at[S - 1], xbuf.at[S - 1], sin.at[NI - 1])

    def cin_pair(j):
        rows = pl.ds(3 + 2 * j, 2)
        return pltpu.make_async_copy(x_hbm.at[rows], xbuf.at[rows], sin.at[j])

    def cin_quad(n):
        t, c = divmod(n, 2)
        return pltpu.make_async_copy(
            x_hbm.at[t, :, c * W4:(c + 1) * W4],
            xbuf.at[t, :, c * W4:(c + 1) * W4], sin.at[NI + 3 + n])

    def cout(sl, r0, r1, ct):
        idx = (sl, slice(r0, r1), slice(ct * PW, (ct + 1) * PW))
        pltpu.make_async_copy(
            obuf.at[idx], o_hbm.at[idx], sout.at[0]).start(priority=ct % 2)

    def cout_quad(t, c):
        for ct in range(4):
            cout(t, 0, D, 4 * c + ct)

    cw = pltpu.make_async_copy(w_hbm, w_ref, sin.at[NI])
    cg = pltpu.make_async_copy(g_hbm, g_ref, sin.at[NI + 1])
    cb = pltpu.make_async_copy(b_hbm, b_ref, sin.at[NI + 2])
    cg.start()
    cb.start()
    cw.start()
    for n in range(NH):
        cin_quad(n).start()
    for j in range(NI - 1):
        cin_pair(j).start()
    cin_last().start()

    row16 = lax.broadcasted_iota(jnp.int32, (16, W2), 0)
    ones = pltpu.bitcast(jnp.where(row16 < 3, 1.0, 0.0).astype(bf16), u32)
    for p_ref in ps:
        for c0 in (0, 2):
            r1 = _rpos(c0)[0] + 32
            p_ref[r1:r1 + 8, :] = ones

    cg.wait()
    cb.wait()
    cw.wait()
    g = g_ref[...].astype(f32).reshape(1, D)
    w = w_ref[...]
    b16 = jnp.broadcast_to(b_ref[...].reshape(1, D), (16, D))
    bias = jnp.dot(b16, w, preferred_element_type=f32)[0:8]
    bh = bias.astype(bf16).astype(f32)
    bl = (bias - bh).astype(bf16).astype(f32)
    bl2 = bias - bh - bl
    row8 = lax.broadcasted_iota(jnp.int32, (8, D), 0)
    ext = jnp.where(row8 == 0, bh,
                    jnp.where(row8 == 1, bl, jnp.where(row8 == 2, bl2, 0.0)))
    wf = w.astype(f32)
    wr = cat([wf[2 * KH:], ext, jnp.zeros((56, D), f32)], axis=0)
    wg = wf[:2 * KH].T * g[:, :2 * KH]
    gr = cat([g[:, 2 * KH:], jnp.ones((1, 64), f32)], axis=1)
    a1 = _sa(wg[0:H, 0:KH], wg[0:H, KH:], wg[H:, 0:KH], wg[H:, KH:])
    for i in range(1, 8):
        top, bot = a1[i - 1][0:Q], a1[i - 1][Q:]
        if i in PERM:
            top, bot = bot, top
        a2 = _sa(top[:, 0:128], top[:, 128:], bot[:, 0:128], bot[:, 128:])
        a_ref[:, (i - 1) * PW:i * PW] = pltpu.bitcast(
            cat(a2, axis=0).astype(bf16), u32)
    arv = (wr.T * gr).astype(bf16)
    ar_ref[:, 0:PW] = pltpu.bitcast(arv[0:H], u32)
    ar_ref[:, PW:] = pltpu.bitcast(arv[H:], u32)

    cin_quad(0).wait()
    _norm_quad(xbuf[zs[2], :, 0:W4].astype(f32),
               *_stats_quad(xbuf[zs[0], :, 0:W4].astype(f32), []), ps[0], [])

    def run(s, fresh, waits, tasks, hooks, bubble, valu, vst, ratio, tweak):
        k1 = s + zs[0]
        k2 = s + zs[2]
        never = {n: lax.broadcasted_iota(
            jnp.int32, (8, n * PW) if n else (16, PW), 0) < zs[1]
                 for n in (0, 1, 2)}
        zero = pl.multiple_of(zs[3], 8)
        nq = 4
        nr = 65
        free = [max(valu - _VT[r], 0) for r in range(nr)]
        tn = _TWEAK_N if tweak else [1] * 65
        ts = _TWEAK_S if tweak else [1] * 65
        wn = [(min(free[r], max(vst - _ST[r], 0) * ratio) + 0.01)
              * tn[r] for r in range(nr)]
        sc = sum(_NCOST) * nq / sum(wn)
        ws = [(max(free[r] - wn[r] * sc, 0) + 0.01) * ts[r]
              for r in range(nr)]

        def xload(k, q):
            t, c = divmod(q, 2)
            return xbuf[jnp.minimum(k + t, S - 1), :,
                        c * W4:(c + 1) * W4].astype(f32)

        cache = {}

        def event(e, n):
            if (e, n) not in cache:
                if n == 1:
                    cache[e, n] = first[e[0]][e[1]:e[1] + 8]
                else:
                    cache[e, n] = cat([event(e, 1)] * 2, axis=1 if n else 0)
            return cache[e, n]

        def make_gate(e):
            if e is None:
                return lambda v, n: v
            return lambda v, n: lax.select(never[n], event(e, n), v)

        mr = {}
        first = {}
        todo = list(tasks)

        def flush(now):
            for task in [t for t in todo if t[3] <= now + 1e-9]:
                todo.remove(task)
                kind, q, t0, t1 = task
                wt = wn if kind == "N" else ws
                cand = []
                a = 0.0
                if t0 == 0 or t0 in waits:
                    cand.append((0.0, None))
                    a += bubble[kind]
                for r in range(int(t0), nr):
                    for e in range(NPER):
                        if t0 - 1e-9 <= r + e / NPER < t1 - 1e-9:
                            cand.append((a, (r, Q * e // NPER // 8 * 8)))
                            a += wt[r] / NPER
                costs = _NCOST if kind == "N" else [1] * (D // 4)
                done = 0
                gates = []
                for x in costs:
                    tgt = a * done / sum(costs)
                    gates.append(make_gate(
                        [e for (c, e) in cand if c <= tgt + 1e-9][-1]))
                    done += x
                if kind == "N":
                    _norm_quad(xload(k2, q), *mr.pop(q), ps[q % 4], gates)
                else:
                    mr[q] = _stats_quad(xload(k1, q), gates)

        count = [0]

        def mxu(lhs, rhs):
            r, o = divmod(count[0], 4)
            if o == 0 and r in waits:
                flush(r)
                waits[r]()
            v = jnp.dot(lhs(), rhs(), preferred_element_type=f32)
            if o == 0:
                first[r] = v
            count[0] += 1
            return v

        def get(i):
            return us[i][pl.ds(zero, H), :]

        def get_sub(i, hr, hc):
            return us[i][pl.ds(pl.multiple_of(zero + hr * Q, 8), Q),
                         hc * PW:(hc + 1) * PW]

        def quad(p):
            sl = s + p // 2
            c0 = (p % 2) * W4
            p_ref = ps[p % 4]
            if p in fresh:
                p_ref = p_ref.at[pl.ds(zero, BROWS), :]

            def hook(name):
                if (p, name) in hooks:
                    hooks[(p, name)]()

            def dot(i, j):
                r1, c1 = _ppos(i, j)
                return mxu(
                    lambda: pltpu.bitcast(
                        a_ref[(j - 1) * 72:j * 72, (i - 1) * PW:i * PW], bf16),
                    lambda: pltpu.bitcast(
                        p_ref[r1:r1 + 64, c1:c1 + PW], bf16))

            def rem(half, cc, hr, hc):
                r1, c1 = _rpos(2 * cc + hc)
                return mxu(
                    lambda: pltpu.bitcast(
                        ar_ref[hr * 72:(hr + 1) * 72,
                               half * PW:(half + 1) * PW], bf16)[:, :KR],
                    lambda: pltpu.bitcast(
                        p_ref[r1:r1 + 40, c1:c1 + PW], bf16))

            def prod(i, o=None, sep=None, plus=(), minus=()):
                sw = 1 if i in PERM else 0

                def blk(c):
                    rows = [cat([c["11"], c["12"]], axis=1),
                            cat([c["21"], c["22"]], axis=1)]
                    return cat(rows[::-1] if sw else rows, axis=0)

                kind = "sep" if i in (4, 5) else "merge" if o else "put"
                seq = _ORDER[("early" if sep else kind, count[0] % 4)].split()
                acc = {}
                sign = {}
                sep = dict(sep or {})
                for n, nm in enumerate(seq):
                    if nm[0] == "m":
                        v = dot(i, int(nm[1]))
                    else:
                        v = rem(o[0], o[1], (int(nm[1]) - 1) ^ sw,
                                int(nm[2]) - 1)
                        sep[nm[1:]] = v
                    for k, terms in _TERMS.items():
                        sg = terms.get(nm)
                        if kind == "merge" and nm == "r" + k:
                            sg = 1
                        if sg is None:
                            continue
                        if k not in acc:
                            acc[k], sign[k] = v, sg
                        elif sign[k] < 0:
                            acc[k], sign[k] = v - acc[k], 1
                        else:
                            acc[k] = acc[k] + v if sg > 0 else acc[k] - v
                    if plus and n == len(seq) - 5:
                        for k in _TERMS:
                            hr, hc = (int(k[0]) - 1) ^ sw, int(k[1]) - 1
                            for u in plus:
                                acc[k] = acc[k] + get_sub(u, hr, hc)
                            for u in minus:
                                acc[k] = acc[k] - get_sub(u, hr, hc)
                return blk(acc), blk(sep) if kind == "sep" else None

            def out(i, o, plus, minus=(), sep=None):
                if i == 6 and p == nq - 1:
                    val, v = prod(i, o, None, plus, minus)
                    plus = minus = ()
                else:
                    val, v = prod(i, o, sep)
                if o == (1, 1):
                    hook("m6")
                v = val if v is None else val + v
                for u in plus:
                    v = v + get(u)
                for u in minus:
                    v = v - get(u)
                obuf[sl, o[0] * H:(o[0] + 1) * H,
                     c0 + o[1] * W2:c0 + (o[1] + 1) * W2] = v.astype(bf16)
                return val

            early = None
            if p == 0:
                early = {k: rem(0, 1, (int(k[0]) - 1) ^ 1, int(k[1]) - 1)
                         for k in _TERMS}
            us[0][...] = prod(3)[0]
            hook("m3")
            us[1][...] = out(5, (0, 1), [0], sep=early)
            us[2][...] = prod(2)[0]
            hook("m2")
            m4 = out(4, (1, 0), [2])
            us[3][...] = m4 - get(1)
            us[4][...] = prod(1)[0]
            hook("m1")
            out(7, (0, 0), [3, 4])
            out(6, (1, 1), [0, 4], [2])

        for p in range(nq):
            flush(-(-count[0] // 4))
            quad(p)
        flush(nr)

    def wait_quads(ns):
        return lambda: [cin_quad(n).wait() for n in ns]

    cin_quad(1).wait()
    run(0, (1, 2, 3), {r: wait_quads(ns) for r, ns in _FIRST_WAITS.items()},
        _FIRST_TASKS, {}, {"N": 125, "S": 176}, 467, 125, 4.61, False)

    j_flush = (DEFER - 2) // 2

    def write_part(half, cc):
        for k in range(2):
            cout(S - 1, half * H, (half + 1) * H, 4 + 2 * cc + k)

    def body(j, carry):
        s = 2 + 2 * j

        @pl.when(j < NI - 1)
        def _():
            cin_pair(j).wait()

        @pl.when(j == NI - 1)
        def _():
            cin_last().wait()

        def write_prev(p):
            def fn():
                if p == 0:
                    @pl.when(j == j_flush)
                    def _():
                        for ct in range(8):
                            cout(pl.ds(0, DEFER), 0, D, ct)

                @pl.when(j > j_flush if p == 0 else j >= j_flush)
                def _():
                    cout_quad(s + (p - 1) // 2, (p - 1) % 2)
            return fn

        def write_last(half, cc):
            return lambda: pl.when(j == NI - 1)(
                lambda: write_part(half, cc))

        hooks = {(p, "m3"): write_prev(p) for p in range(4)}
        hooks.update({(3, "m2"): write_last(0, 1), (3, "m1"): write_last(1, 0),
                      (3, "m6"): write_last(0, 0)})
        run(s, (2, 3), {}, _LOOP_TASKS, hooks, {"N": 0.01, "S": 550},
            441, 121, 5.86, True)
        return carry

    lax.fori_loop(0, NI, body, 0)
    write_part(1, 1)
    pltpu.make_async_copy(obuf, o_hbm, sout.at[0]).wait()


@jax.jit
def pallas_standalone__layernorm_linear__sampling_kernel(
    x: jax.Array,
    g: jax.Array,
    b: jax.Array,
    w: jax.Array,
):
    assert x.shape == (B, S, D) and w.shape == (D, D)
    xt = jnp.transpose(x, (1, 2, 0))
    out = pl.pallas_call(
        _kernel,
        in_specs=[pl.BlockSpec(memory_space=pl.ANY)] * 4,
        out_specs=pl.BlockSpec(memory_space=pl.ANY),
        out_shape=jax.ShapeDtypeStruct((S, D, B), x.dtype),
        scratch_shapes=[
            pltpu.VMEM((S, D, B), bf16),
            pltpu.VMEM((S, D, B), bf16),
        ] + [pltpu.VMEM((BROWS, W2), u32)] * 4
        + [pltpu.VMEM((H, W2), f32)] * 5
        + [
            pltpu.VMEM((D,), bf16),
            pltpu.VMEM((D,), bf16),
            pltpu.VMEM((D, D), bf16),
            pltpu.VMEM((7 * 72, 7 * PW), u32),
            pltpu.VMEM((144, W2), u32),
            pltpu.SMEM((4,), jnp.int32),
            pltpu.SemaphoreType.DMA((NI + 3 + NH,)),
            pltpu.SemaphoreType.DMA((1,)),
        ],
        compiler_params=pltpu.CompilerParams(
            vmem_limit_bytes=110 * 1024 * 1024,
            disable_bounds_checks=True,
            disable_semaphore_checks=True,
        ),
    )(xt, g, b, w)
    return jnp.transpose(out, (2, 0, 1))
```

```python
import jax
import jax.numpy as jnp
from jax import lax
import jax.experimental.pallas as pl
import jax.experimental.pallas.tpu as pltpu

EPS = 1e-5
D = 576
S = 32
B = 1024
H = D // 2
Q = D // 4
KH = 256
KR = 80
PW = 128
W2 = 2 * PW
W4 = 4 * PW
NH = 6
NI = 15
DEFER = 14
NPER = 18
f32 = jnp.float32
bf16 = jnp.bfloat16
u32 = jnp.uint32
cat = jnp.concatenate
PERM = (3, 5, 6, 7)
RROW = 28 * 64
BROWS = RROW + 80


def _sa(a11, a12, a21, a22):
    return [a11 + a22, a21 + a22, a11, a22, a11 + a12, a21 - a11, a12 - a22]


def _sb(b11, b12, b21, b22):
    return [b11 + b22, b11, b12 - b22, b21 - b11, b22, b11 + b12, b21 + b22]


def _ppos(i, j):
    return ((j - 1) * 4 + (i - 1) // 2) * 64, ((i - 1) % 2) * PW


def _rpos(ct):
    return RROW + (ct // 2) * 40, (ct % 2) * PW


_VT = [
    69, 74, 88, 142, 97, 108, 86, 159, 180, 74, 74, 71, 177, 165, 54, 224,
    205, 111, 54, 159, 110, 74, 73, 124, 197, 115, 102, 54, 173, 166, 75, 210,
    186, 112, 69, 140, 144, 74, 74, 122, 180, 98, 114, 61, 173, 181, 60, 206,
    202, 79, 73, 90, 160, 108, 108, 71, 196, 128, 74, 90, 53, 190, 169, 207,
    216]
_ST = [
    17, 54, 35, 55, 19, 52, 59, 40, 54, 18, 54, 10, 17, 19, 12, 21, 55, 56,
    23, 55, 39, 40, 41, 73, 53, 44, 56, 2, 16, 18, 12, 17, 19, 53, 56, 40, 54,
    19, 54, 59, 55, 20, 53, 20, 16, 18, 2, 16, 21, 40, 42, 54, 53, 43, 56, 43,
    53, 41, 45, 38, 9, 17, 46, 19, 18]
_TWEAK_N = [
    1.0, 1.0, 1.0, 1.0, 1.0, 1.0, 1.0, 1.0, 1.0, 1.0, 1.0, 1.0, 1.0, 1.0, 1.0,
    1.0, 1.0, 1.0, 1.0, 1.0, 1.0, 1.0, 1.0, 1.0, 1.0, 1.0, 1.0, 1.0, 1.0, 1.0,
    1.0, 1.0, 1.0, 1.0, 1.0, 1.0, 1.0, 1.0, 1.0, 1.0, 1.0, 1.0, 1.0, 1.0, 1.0,
    1.0, 1.0, 1.0, 0.8928, 1.0, 1.1072, 1.0, 1.0, 1.0, 1.0, 1.0, 1.0, 1.0,
    0.7203, 1.2478, 1.0424, 1.0, 1.2017, 0.7983, 1.0]
_TWEAK_S = [
    1.0, 1.0, 1.0, 1.0, 1.0, 1.0, 1.0, 1.0, 1.0, 1.0, 1.0, 1.0, 1.0, 1.0, 1.0,
    1.0, 0.7353, 0.7965, 1.0, 1.0, 1.0, 1.0, 1.0, 1.0, 1.0, 1.0, 1.0, 1.0,
    1.0, 1.0, 1.0, 1.0, 1.0, 1.0, 1.0, 1.0, 1.0, 1.0, 1.0, 1.1102, 0.9512,
    0.9332, 1.0, 1.0, 1.0, 1.0445, 0.7247, 1.1393, 1.0824, 1.0, 1.0, 1.0,
    1.0425, 1.0, 0.9575, 1.0, 1.0, 1.0, 1.0, 1.0, 1.1749, 0.8251, 1.0, 1.0,
    1.0]
_NCOST = []
for _k in range(8):
    _NCOST += [13, 13, 9, 12, 17, 17, 9, 12, 17, 17, 9, 12, 17, 12, 9, 12, 17,
               17, 9, 12, 17, 12] + ([16, 16] if _k % 2 == 0 else [])

_FIRST_WAITS = {15: (2, 3), 35: (4, 5)}
_FIRST_VT = [70, 80, 90, 150, 110, 90, 160, 150, 75, 90, 170, 120] + _VT[16:]
_FIRST_ST = [30, 54, 45, 55, 40, 55, 50, 50, 30, 40, 20, 25] + _ST[16:]
_FIRST_TASKS = [
    ("S", 1, 0, 3.49),
    ("N", 1, 3.49, 10.99),
    ("S", 2, 15, 17.66),
    ("N", 2, 17.66, 26.33),
    ("S", 3, 17.66, 25.83),
    ("N", 3, 26.33, 35),
    ("S", 4, 35, 39.3),
    ("S", 5, 39.3, 50.301),
    ("N", 4, 39.3, 50.801),
    ("N", 5, 50.801, 61),
]
_LOOP_TASKS = [
    ("S", 2, 0, 4.97),
    ("S", 3, 4.97, 14.0775),
    ("N", 2, 4.97, 19.9775),
    ("S", 4, 14.0775, 29.085),
    ("N", 3, 19.9775, 34.985),
    ("S", 5, 29.085, 44.0925),
    ("N", 4, 34.985, 49.9925),
    ("N", 5, 49.9925, 65.0),
]

_ORDER = {
    ("put", 0): "m1 m2 m4 m6 m3 m5 m7",
    ("put", 1): "m1 m2 m4 m3 m5 m6 m7",
    ("put", 2): "m1 m6 m2 m3 m4 m5 m7",
    ("put", 3): "m2 m1 m3 m5 m6 m4 m7",
    ("sep", 0): "m1 m2 m4 m7 m3 m5 r11 r12 m6 r21 r22",
    ("sep", 1): "m1 m2 m4 m3 m6 r21 r22 m5 m7 r11 r12",
    ("sep", 2): "m3 m4 m1 m2 m6 r21 m5 m7 r11 r12 r22",
    ("sep", 3): "m3 m1 m2 m4 m6 m5 m7 r11 r12 r21 r22",
    ("merge", 0): "m3 m6 r12 r22 m1 m2 m4 r21 m5 m7 r11",
    ("merge", 1): "m3 m6 r22 m1 m2 m4 r21 m5 m7 r11 r12",
    ("merge", 2): "m6 r22 m4 m7 r11 r21 m1 m3 m5 r12 m2",
    ("merge", 3): "m1 m3 m6 r12 r22 m2 m4 m7 r21 m5 r11",
    ("early", 1): "m1 m6 m7 m2 m3 m4 m5",
    ("early", 2): "m3 m6 m1 m2 m4 m7 m5",
    ("early", 3): "m3 m1 m2 m4 m6 m5 m7",
}
_OUT = {5: (0, 1), 4: (1, 0), 7: (0, 0), 6: (1, 1)}
_TERMS = {"11": {"m1": 1, "m7": 1, "m5": -1, "m4": 1},
          "12": {"m3": 1, "m5": 1},
          "21": {"m2": 1, "m4": 1},
          "22": {"m1": 1, "m3": 1, "m6": 1, "m2": -1}}


def _stats_pair(x, gates):
    c = jnp.broadcast_to(x[0:1, :], (8, W2))
    a1 = a2 = None
    for k in range(D // 8):
        v = x[k * 8:(k + 1) * 8] - (gates[k](c, 2) if gates else c)
        a1 = v if a1 is None else a1 + v
        a2 = v * v if a2 is None else a2 + v * v
    a1 = jnp.sum(a1, axis=0, keepdims=True) * (1.0 / D)
    a2 = jnp.sum(a2, axis=0, keepdims=True) * (1.0 / D)
    m = c[0:1] + a1
    var = jnp.maximum(a2 - a1 * a1, 0.0)
    r = lax.rsqrt(var + EPS)
    return jnp.broadcast_to(m, (8, W2)), jnp.broadcast_to(r, (8, W2))


def _stats_quad(x, gates):
    h = len(gates) // 2
    ma, ra = _stats_pair(x[:, 0:W2], gates[:h])
    mb, rb = _stats_pair(x[:, W2:], gates[h:])
    return cat([ma, mb], axis=1), cat([ra, rb], axis=1)


def _norm_quad(x, m, r, p_ref, gates, main=True, rest=True):
    def tiles(v, tc):
        return cat([v[:, tc * PW:(tc + 1) * PW],
                    v[:, (tc + 2) * PW:(tc + 3) * PW]], axis=1)

    def wide(v):
        return cat([cat([v, v], axis=1)] * 2, axis=0)

    xt = [tiles(x, 0), tiles(x, 1)]
    mt = [tiles(m, 0), tiles(m, 1)]
    rt = [wide(tiles(r, 0)), wide(tiles(r, 1))]
    ms = [m[:, c * PW:(c + 1) * PW] for c in range(4)]
    r16 = cat([r, r], axis=0)
    it = iter(gates)

    def sub(k, kr, tc):
        mg = mt[tc]
        if gates:
            mg = cat([next(it)(ms[tc], 1), next(it)(ms[tc + 2], 1)], axis=1)
        r0 = kr * 128 + k * 16
        xb = cat([xt[tc][r0:r0 + 16], xt[tc][KH + r0:KH + r0 + 16]], axis=1)
        return (xb - wide(mg)) * rt[tc]

    def emit(k, j, v):
        q = [v[:, i * PW:(i + 1) * PW] for i in range(4)]
        if gates:
            q[0] = next(it)(q[0], 0)
            q[3] = next(it)(q[3], 0)
        ops = _sb(*q)
        for i0 in range(0, 7, 2):
            grp = ops[i0:i0 + 2]
            r0 = _ppos(i0 + 1, j)[0] + k * 8
            p_ref[r0:r0 + 8, 0:len(grp) * PW] = pltpu.bitcast(
                cat(grp, axis=1).astype(bf16), u32)

    for k in range(8):
        if main:
            b11 = sub(k, 0, 0)
            emit(k, 2, b11)
            b12 = sub(k, 0, 1)
            emit(k, 6, b11 + b12)
            b22 = sub(k, 1, 1)
            emit(k, 3, b12 - b22)
            emit(k, 1, b11 + b22)
            emit(k, 5, b22)
            b21 = sub(k, 1, 0)
            emit(k, 4, b21 - b11)
            emit(k, 7, b21 + b22)
        if rest and k % 2 == 0:
            mg = m
            if gates:
                mg = cat([next(it)(m[:, 0:W2], 2), next(it)(m[:, W2:], 2)],
                         axis=1)
            r0 = 2 * KH + k * 8
            v = (x[r0:r0 + 16] - cat([mg, mg], axis=0)) * r16
            for c0 in (0, 2):
                r1 = _rpos(c0)[0] + k * 4
                p_ref[r1:r1 + 8, :] = pltpu.bitcast(
                    v[:, c0 * PW:(c0 + 2) * PW].astype(bf16), u32)


def _kernel(x_hbm, g_hbm, b_hbm, w_hbm, o_hbm, xbuf, obuf,
            p0, p1, p2, p3, u0, u1, u2, u3, u4,
            g_ref, b_ref, w_ref, a_ref, ar_ref, zs, sin, sout):
    ps = [p0, p1, p2, p3]
    us = [u0, u1, u2, u3, u4]
    for i in range(4):
        zs[i] = 0

    def cin_last():
        return pltpu.make_async_copy(
            x_hbm.at[S - 1], xbuf.at[S - 1], sin.at[NI - 1])

    def cin_pair(j):
        rows = pl.ds(3 + 2 * j, 2)
        return pltpu.make_async_copy(x_hbm.at[rows], xbuf.at[rows], sin.at[j])

    def cin_quad(n):
        t, c = divmod(n, 2)
        return pltpu.make_async_copy(
            x_hbm.at[t, :, c * W4:(c + 1) * W4],
            xbuf.at[t, :, c * W4:(c + 1) * W4], sin.at[NI + 3 + n])

    def cout(sl, r0, r1, ct):
        idx = (sl, slice(r0, r1), slice(ct * PW, (ct + 1) * PW))
        pltpu.make_async_copy(
            obuf.at[idx], o_hbm.at[idx], sout.at[0]).start(priority=ct % 2)

    def cout_quad(t, c):
        for ct in range(4):
            cout(t, 0, D, 4 * c + ct)

    cw = pltpu.make_async_copy(w_hbm, w_ref, sin.at[NI])
    cg = pltpu.make_async_copy(g_hbm, g_ref, sin.at[NI + 1])
    cb = pltpu.make_async_copy(b_hbm, b_ref, sin.at[NI + 2])
    cg.start()
    cb.start()
    cw.start()
    for n in range(NH):
        cin_quad(n).start()
    for j in range(NI - 1):
        cin_pair(j).start()
    cin_last().start()

    row16 = lax.broadcasted_iota(jnp.int32, (16, W2), 0)
    ones = pltpu.bitcast(jnp.where(row16 < 3, 1.0, 0.0).astype(bf16), u32)
    for p_ref in ps:
        for c0 in (0, 2):
            r1 = _rpos(c0)[0] + 32
            p_ref[r1:r1 + 8, :] = ones

    cg.wait()
    cb.wait()
    cw.wait()
    g = g_ref[...].astype(f32).reshape(1, D)
    w = w_ref[...]
    b16 = jnp.broadcast_to(b_ref[...].reshape(1, D), (16, D))
    bias = jnp.dot(b16, w, preferred_element_type=f32)[0:8]
    bh = bias.astype(bf16).astype(f32)
    bl = (bias - bh).astype(bf16).astype(f32)
    bl2 = bias - bh - bl
    row8 = lax.broadcasted_iota(jnp.int32, (8, D), 0)
    ext = jnp.where(row8 == 0, bh,
                    jnp.where(row8 == 1, bl, jnp.where(row8 == 2, bl2, 0.0)))
    wf = w.astype(f32)
    wr = cat([wf[2 * KH:], ext, jnp.zeros((56, D), f32)], axis=0)
    wg = wf[:2 * KH].T * g[:, :2 * KH]
    gr = cat([g[:, 2 * KH:], jnp.ones((1, 64), f32)], axis=1)
    a1 = _sa(wg[0:H, 0:KH], wg[0:H, KH:], wg[H:, 0:KH], wg[H:, KH:])
    for i in range(1, 8):
        top, bot = a1[i - 1][0:Q], a1[i - 1][Q:]
        if i in PERM:
            top, bot = bot, top
        a2 = _sa(top[:, 0:128], top[:, 128:], bot[:, 0:128], bot[:, 128:])
        a_ref[:, (i - 1) * PW:i * PW] = pltpu.bitcast(
            cat(a2, axis=0).astype(bf16), u32)
    arv = (wr.T * gr).astype(bf16)
    ar_ref[:, 0:PW] = pltpu.bitcast(arv[0:H], u32)
    ar_ref[:, PW:] = pltpu.bitcast(arv[H:], u32)

    def masks():
        return {n: lax.broadcasted_iota(
            jnp.int32, (8, n * PW) if n else (16, PW), 0) < zs[1]
                for n in (0, 1, 2)}

    def gate_factory(source):
        never = masks()
        cache = {}

        def event(e, n):
            if (e, n) not in cache:
                if n == 1:
                    cache[e, n] = source[e[0]][e[1]:e[1] + 8]
                else:
                    cache[e, n] = cat([event(e, 1)] * 2, axis=1 if n else 0)
            return cache[e, n]

        def make_gate(e):
            if e is None:
                return lambda v, n: v
            return lambda v, n: lax.select(never[n], event(e, n), v)
        return make_gate

    def rem_operands(p_ref, i, k):
        half, cc = _OUT[i]
        hr = (int(k[0]) - 1) ^ (1 if i in PERM else 0)
        r1, c1 = _rpos(2 * cc + int(k[1]) - 1)
        return (lambda: pltpu.bitcast(
                    ar_ref[hr * 72:(hr + 1) * 72,
                           half * PW:(half + 1) * PW], bf16)[:, :KR],
                lambda: pltpu.bitcast(p_ref[r1:r1 + 40, c1:c1 + PW], bf16))

    cin_quad(0).wait()
    m0, r0 = _stats_quad(xbuf[zs[0], :, 0:W4].astype(f32), [])
    x0 = xbuf[zs[2], :, 0:W4].astype(f32)
    _norm_quad(x0, m0, r0, ps[0], [], main=False)
    early0 = {}
    for i in (4, 7, 5, 6):
        early0[i] = {}
        for k in _TERMS:
            lhs, rhs = rem_operands(ps[0], i, k)
            early0[i][k] = jnp.dot(lhs(), rhs(), preferred_element_type=f32)
    gate0 = gate_factory([early0[i]["11"] for i in (4, 7, 5, 6)])
    _norm_quad(x0, m0, r0, ps[0],
               [gate0(None)] * 19
               + [gate0(divmod(int(u * 72 * 0.99 / 157) * 8, Q))
                  for u in range(157)], rest=False)

    def run(s, fresh, waits, tasks, hooks, early, bubble, valu, vst, ratio):
        k1 = s + zs[0]
        k2 = s + zs[2]
        first = {}
        make_gate = gate_factory(first)
        zero = pl.multiple_of(zs[3], 8)
        nq = 4
        vt, st = (_FIRST_VT, _FIRST_ST) if early else (_VT, _ST)
        nr = len(vt)
        tn = [1] * nr if early else _TWEAK_N
        ts = [1] * nr if early else _TWEAK_S
        free = [max(valu - vt[r], 0) for r in range(nr)]
        wn = [(min(free[r], max(vst - st[r], 0) * ratio) + 0.01) * tn[r]
              for r in range(nr)]
        sc = sum(_NCOST) * nr / 16.25 / sum(wn)
        ws = [(max(free[r] - wn[r] * sc, 0) + 0.01) * ts[r] for r in range(nr)]

        def xload(k, q):
            t, c = divmod(q, 2)
            return xbuf[jnp.minimum(k + t, S - 1), :,
                        c * W4:(c + 1) * W4].astype(f32)

        mr = {}
        todo = list(tasks)

        def flush(now):
            for task in [t for t in todo if t[3] <= now + 1e-9]:
                todo.remove(task)
                kind, q, t0, t1 = task
                wt = wn if kind == "N" else ws
                cand = []
                a = 0.0
                if t0 == 0 or t0 in waits:
                    cand.append((0.0, None))
                    a += bubble[kind]
                for r in range(int(t0), nr):
                    for e in range(NPER):
                        if t0 - 1e-9 <= r + e / NPER < t1 - 1e-9:
                            cand.append((a, (r, Q * e // NPER // 8 * 8)))
                            a += wt[r] / NPER
                costs = _NCOST if kind == "N" else [1] * (D // 4)
                done = 0
                gates = []
                for x in costs:
                    tgt = a * done / sum(costs)
                    gates.append(make_gate(
                        [e for (c, e) in cand if c <= tgt + 1e-9][-1]))
                    done += x
                if kind == "N":
                    _norm_quad(xload(k2, q), *mr.pop(q), ps[q % 4], gates)
                else:
                    mr[q] = _stats_quad(xload(k1, q), gates)

        count = [0]

        def mxu(lhs, rhs):
            r, o = divmod(count[0], 4)
            if o == 0 and r in waits:
                flush(r)
                waits[r]()
            v = jnp.dot(lhs(), rhs(), preferred_element_type=f32)
            if o == 0:
                first[r] = v
            count[0] += 1
            return v

        def get(i):
            return us[i][pl.ds(zero, H), :]

        def get_sub(i, hr, hc):
            return us[i][pl.ds(pl.multiple_of(zero + hr * Q, 8), Q),
                         hc * PW:(hc + 1) * PW]

        def quad(p):
            sl = s + p // 2
            c0 = (p % 2) * W4
            p_ref = ps[p % 4]
            if p in fresh:
                p_ref = p_ref.at[pl.ds(zero, BROWS), :]

            def hook(name):
                if (p, name) in hooks:
                    hooks[(p, name)]()

            def dot(i, j):
                r1, c1 = _ppos(i, j)
                return mxu(
                    lambda: pltpu.bitcast(
                        a_ref[(j - 1) * 72:j * 72, (i - 1) * PW:i * PW], bf16),
                    lambda: pltpu.bitcast(
                        p_ref[r1:r1 + 64, c1:c1 + PW], bf16))

            def rem(i, k):
                return mxu(*rem_operands(p_ref, i, k))

            def prod(i, sep=None, plus=(), minus=()):
                sw = 1 if i in PERM else 0

                def blk(c):
                    rows = [cat([c["11"], c["12"]], axis=1),
                            cat([c["21"], c["22"]], axis=1)]
                    return cat(rows[::-1] if sw else rows, axis=0)

                kind = ("put" if i not in _OUT else
                        "sep" if sep or i in (4, 5) else "merge")
                seq = _ORDER[("early" if sep else kind, count[0] % 4)].split()
                acc = {}
                sign = {}
                sep = dict(sep or {})
                for n, nm in enumerate(seq):
                    if nm[0] == "m":
                        v = dot(i, int(nm[1]))
                    else:
                        v = rem(i, nm[1:])
                        sep[nm[1:]] = v
                    for k, terms in _TERMS.items():
                        sg = terms.get(nm)
                        if kind == "merge" and nm == "r" + k:
                            sg = 1
                        if sg is None:
                            continue
                        if k not in acc:
                            acc[k], sign[k] = v, sg
                        elif sign[k] < 0:
                            acc[k], sign[k] = v - acc[k], 1
                        else:
                            acc[k] = acc[k] + v if sg > 0 else acc[k] - v
                    if plus and n == len(seq) - 5:
                        for k in _TERMS:
                            hr, hc = (int(k[0]) - 1) ^ sw, int(k[1]) - 1
                            for u in plus:
                                acc[k] = acc[k] + get_sub(u, hr, hc)
                            for u in minus:
                                acc[k] = acc[k] - get_sub(u, hr, hc)
                return blk(acc), blk(sep) if kind == "sep" else None

            def out(i, plus, minus=()):
                o = _OUT[i]
                if i == 6 and p == nq - 1:
                    val, v = prod(i, None, plus, minus)
                    plus = minus = ()
                else:
                    val, v = prod(i, done.get(i))
                if i == 6:
                    hook("m6")
                v = val if v is None else val + v
                for u in plus:
                    v = v + get(u)
                for u in minus:
                    v = v - get(u)
                obuf[sl, o[0] * H:(o[0] + 1) * H,
                     c0 + o[1] * W2:c0 + (o[1] + 1) * W2] = v.astype(bf16)
                return val

            done = {}
            if p == 0:
                done = early or {5: {k: rem(5, k) for k in _TERMS}}
            us[0][...] = prod(3)[0]
            hook("m3")
            us[1][...] = out(5, [0])
            us[2][...] = prod(2)[0]
            hook("m2")
            m4 = out(4, [2])
            us[3][...] = m4 - get(1)
            us[4][...] = prod(1)[0]
            hook("m1")
            out(7, [3, 4])
            out(6, [0, 4], [2])

        for p in range(nq):
            flush(-(-count[0] // 4))
            quad(p)
        flush(nr)

    def wait_quads(ns):
        return lambda: [cin_quad(n).wait() for n in ns]

    cin_quad(1).wait()
    run(0, (1, 2, 3), {r: wait_quads(ns) for r, ns in _FIRST_WAITS.items()},
        _FIRST_TASKS, {}, early0, {"N": 293, "S": 396}, 509, 138, 4.92)

    j_flush = (DEFER - 2) // 2

    def write_part(half, cc):
        for k in range(2):
            cout(S - 1, half * H, (half + 1) * H, 4 + 2 * cc + k)

    def body(j, carry):
        s = 2 + 2 * j

        @pl.when(j < NI - 1)
        def _():
            cin_pair(j).wait()

        @pl.when(j == NI - 1)
        def _():
            cin_last().wait()

        def write_prev(p):
            def fn():
                if p == 0:
                    @pl.when(j == j_flush)
                    def _():
                        for ct in range(8):
                            cout(pl.ds(0, DEFER), 0, D, ct)

                @pl.when(j > j_flush if p == 0 else j >= j_flush)
                def _():
                    cout_quad(s + (p - 1) // 2, (p - 1) % 2)
            return fn

        def write_last(half, cc):
            return lambda: pl.when(j == NI - 1)(
                lambda: write_part(half, cc))

        hooks = {(p, "m3"): write_prev(p) for p in range(4)}
        hooks.update({(3, "m2"): write_last(0, 1), (3, "m1"): write_last(1, 0),
                      (3, "m6"): write_last(0, 0)})
        run(s, (2, 3), {}, _LOOP_TASKS, hooks, None, {"N": 0.01, "S": 550},
            441, 121, 5.86)
        return carry

    lax.fori_loop(0, NI, body, 0)
    write_part(1, 1)
    pltpu.make_async_copy(obuf, o_hbm, sout.at[0]).wait()


@jax.jit
def pallas_standalone__layernorm_linear__sampling_kernel(
    x: jax.Array,
    g: jax.Array,
    b: jax.Array,
    w: jax.Array,
):
    assert x.shape == (B, S, D) and w.shape == (D, D)
    xt = jnp.transpose(x, (1, 2, 0))
    out = pl.pallas_call(
        _kernel,
        in_specs=[pl.BlockSpec(memory_space=pl.ANY)] * 4,
        out_specs=pl.BlockSpec(memory_space=pl.ANY),
        out_shape=jax.ShapeDtypeStruct((S, D, B), x.dtype),
        scratch_shapes=[
            pltpu.VMEM((S, D, B), bf16),
            pltpu.VMEM((S, D, B), bf16),
        ] + [pltpu.VMEM((BROWS, W2), u32)] * 4
        + [pltpu.VMEM((H, W2), f32)] * 5
        + [
            pltpu.VMEM((D,), bf16),
            pltpu.VMEM((D,), bf16),
            pltpu.VMEM((D, D), bf16),
            pltpu.VMEM((7 * 72, 7 * PW), u32),
            pltpu.VMEM((144, W2), u32),
            pltpu.SMEM((4,), jnp.int32),
            pltpu.SemaphoreType.DMA((NI + 3 + NH,)),
            pltpu.SemaphoreType.DMA((1,)),
        ],
        compiler_params=pltpu.CompilerParams(
            vmem_limit_bytes=110 * 1024 * 1024,
            disable_bounds_checks=True,
            disable_semaphore_checks=True,
        ),
    )(xt, g, b, w)
    return jnp.transpose(out, (2, 0, 1))
```

```python
import jax
import jax.numpy as jnp
from jax import lax
import jax.experimental.pallas as pl
import jax.experimental.pallas.tpu as pltpu

EPS = 1e-5
D = 576
S = 32
B = 1024
H = D // 2
Q = D // 4
KH = 256
KR = 80
PW = 128
W2 = 2 * PW
W4 = 4 * PW
NH = 6
NI = 15
DEFER = 14
NPER = 18
f32 = jnp.float32
bf16 = jnp.bfloat16
u32 = jnp.uint32
cat = jnp.concatenate
PERM = (3, 5, 6, 7)
RROW = 28 * 64
BROWS = RROW + 80


def _sa(a11, a12, a21, a22):
    return [a11 + a22, a21 + a22, a11, a22, a11 + a12, a21 - a11, a12 - a22]


def _sb(b11, b12, b21, b22):
    return [b11 + b22, b11, b12 - b22, b21 - b11, b22, b11 + b12, b21 + b22]


def _ppos(i, j):
    return ((j - 1) * 4 + (i - 1) // 2) * 64, ((i - 1) % 2) * PW


def _rpos(ct):
    return RROW + (ct // 2) * 40, (ct % 2) * PW


_VT = [
    69, 74, 88, 142, 97, 108, 86, 159, 180, 74, 74, 71, 177, 165, 54, 224,
    205, 111, 54, 159, 110, 74, 73, 124, 197, 115, 102, 54, 173, 166, 75, 210,
    186, 112, 69, 140, 144, 74, 74, 122, 180, 98, 114, 61, 173, 181, 60, 206,
    202, 79, 73, 90, 160, 108, 108, 71, 196, 128, 74, 90, 53, 190, 169, 207,
    216]
_ST = [
    17, 54, 35, 55, 19, 52, 59, 40, 54, 18, 54, 10, 17, 19, 12, 21, 55, 56,
    23, 55, 39, 40, 41, 73, 53, 44, 56, 2, 16, 18, 12, 17, 19, 53, 56, 40, 54,
    19, 54, 59, 55, 20, 53, 20, 16, 18, 2, 16, 21, 40, 42, 54, 53, 43, 56, 43,
    53, 41, 45, 38, 9, 17, 46, 19, 18]
_TWEAK_N = [
    1.0, 1.0, 1.0, 1.0341, 1.0, 0.9659, 1.0, 1.0, 1.0, 1.0, 1.0, 1.0, 1.0,
    1.0, 1.0, 1.0, 1.0, 1.0, 1.0, 1.0, 1.0, 1.0, 1.0, 1.0, 1.0, 1.0, 1.0, 1.0,
    1.0, 1.0, 1.0, 1.0, 1.0, 1.0, 1.0, 1.0, 1.0, 1.0, 1.0, 1.0, 1.0, 1.0, 1.0,
    1.0, 1.0, 1.0, 1.0, 1.0, 0.8928, 1.0, 1.1072, 1.0, 1.0, 1.0, 1.0, 1.0,
    1.0, 1.0, 0.7203, 1.2478, 1.0424, 1.0, 1.2017, 0.7983, 1.0]
_TWEAK_S = [
    1.0, 1.0, 1.0, 1.0, 1.0, 1.0, 1.0, 1.0, 0.7016, 1.0, 1.0, 1.0, 1.0, 1.0,
    1.0, 1.0, 0.7353, 0.7965, 1.0, 1.0, 1.0, 1.0, 1.0, 1.0, 1.0, 1.0, 1.0,
    1.0, 1.0, 1.0, 1.0, 1.0, 1.0, 1.0, 1.0, 1.0, 1.0, 1.0, 1.0, 1.1102,
    0.9512, 0.9332, 0.9577, 1.0, 1.0423, 0.7687, 0.9161, 1.0032, 1.0824, 1.0,
    1.0, 1.0, 1.0425, 1.0, 0.7235, 1.2128, 1.0, 1.0, 1.0, 1.0, 1.1749, 0.8251,
    1.0, 1.0, 1.0]
_NCOST = []
for _k in range(8):
    _NCOST += [13, 13, 9, 12, 17, 17, 9, 12, 17, 17, 9, 12, 17, 12, 9, 12, 17,
               17, 9, 12, 17, 12] + ([16, 16] if _k % 2 == 0 else [])

_FIRST_WAITS = {15: (2, 3), 35: (4, 5)}
_FIRST_VT = [70, 80, 90, 150, 110, 90, 160, 150, 75, 90, 170, 120] + _VT[16:]
_FIRST_ST = [30, 54, 45, 55, 40, 55, 50, 50, 30, 40, 20, 25] + _ST[16:]
_FIRST_TASKS = [
    ("S", 1, 0, 3.49),
    ("N", 1, 3.49, 10.99),
    ("S", 2, 15, 17.66),
    ("N", 2, 17.66, 26.33),
    ("S", 3, 17.66, 25.83),
    ("N", 3, 26.33, 35),
    ("S", 4, 35, 39.3),
    ("S", 5, 39.3, 50.301),
    ("N", 4, 39.3, 50.801),
    ("N", 5, 50.801, 61),
]
_LOOP_TASKS = [
    ("S", 2, 0, 4.132),
    ("S", 3, 4.132, 14.0775),
    ("N", 2, 4.132, 19.9775),
    ("S", 4, 14.0775, 29.085),
    ("N", 3, 19.9775, 34.985),
    ("S", 5, 29.085, 44.092),
    ("N", 4, 34.985, 49.9925),
    ("N", 5, 49.9925, 65),
]

_ORDER = {
    ("put", 0): "m1 m2 m4 m6 m3 m5 m7",
    ("put", 1): "m1 m2 m4 m3 m5 m6 m7",
    ("put", 2): "m1 m6 m2 m3 m4 m5 m7",
    ("put", 3): "m2 m1 m3 m5 m6 m4 m7",
    ("sep", 0): "m1 m2 m4 m7 m3 m5 r11 r12 m6 r21 r22",
    ("sep", 1): "m1 m2 m4 m3 m6 r21 r22 m5 m7 r11 r12",
    ("sep", 2): "m3 m4 m1 m2 m6 r21 m5 m7 r11 r12 r22",
    ("sep", 3): "m3 m1 m2 m4 m6 m5 m7 r11 r12 r21 r22",
    ("merge", 0): "m3 m6 r12 r22 m1 m2 m4 r21 m5 m7 r11",
    ("merge", 1): "m3 m6 r22 m1 m2 m4 r21 m5 m7 r11 r12",
    ("merge", 2): "m6 r22 m4 m7 r11 r21 m1 m3 m5 r12 m2",
    ("merge", 3): "m1 m3 m6 r12 r22 m2 m4 m7 r21 m5 r11",
    ("early", 1): "m1 m6 m7 m2 m3 m4 m5",
    ("early", 2): "m3 m6 m1 m2 m4 m7 m5",
    ("early", 3): "m3 m1 m2 m4 m6 m5 m7",
}
_OUT = {5: (0, 1), 4: (1, 0), 7: (0, 0), 6: (1, 1)}
_TERMS = {"11": {"m1": 1, "m7": 1, "m5": -1, "m4": 1},
          "12": {"m3": 1, "m5": 1},
          "21": {"m2": 1, "m4": 1},
          "22": {"m1": 1, "m3": 1, "m6": 1, "m2": -1}}


def _stats_pair(x, gates):
    c = jnp.broadcast_to(x[0:1, :], (8, W2))
    a1 = a2 = None
    for k in range(D // 8):
        v = x[k * 8:(k + 1) * 8] - (gates[k](c, 2) if gates else c)
        a1 = v if a1 is None else a1 + v
        a2 = v * v if a2 is None else a2 + v * v
    a1 = jnp.sum(a1, axis=0, keepdims=True) * (1.0 / D)
    a2 = jnp.sum(a2, axis=0, keepdims=True) * (1.0 / D)
    m = c[0:1] + a1
    var = jnp.maximum(a2 - a1 * a1, 0.0)
    r = lax.rsqrt(var + EPS)
    return jnp.broadcast_to(m, (8, W2)), jnp.broadcast_to(r, (8, W2))


def _stats_quad(x, gates):
    h = len(gates) // 2
    ma, ra = _stats_pair(x[:, 0:W2], gates[:h])
    mb, rb = _stats_pair(x[:, W2:], gates[h:])
    return cat([ma, mb], axis=1), cat([ra, rb], axis=1)


def _norm_quad(x, m, r, p_ref, gates, main=True, rest=True):
    def tiles(v, tc):
        return cat([v[:, tc * PW:(tc + 1) * PW],
                    v[:, (tc + 2) * PW:(tc + 3) * PW]], axis=1)

    def wide(v):
        return cat([cat([v, v], axis=1)] * 2, axis=0)

    xt = [tiles(x, 0), tiles(x, 1)]
    mt = [tiles(m, 0), tiles(m, 1)]
    rt = [wide(tiles(r, 0)), wide(tiles(r, 1))]
    ms = [m[:, c * PW:(c + 1) * PW] for c in range(4)]
    r16 = cat([r, r], axis=0)
    it = iter(gates)

    def sub(k, kr, tc):
        mg = mt[tc]
        if gates:
            mg = cat([next(it)(ms[tc], 1), next(it)(ms[tc + 2], 1)], axis=1)
        r0 = kr * 128 + k * 16
        xb = cat([xt[tc][r0:r0 + 16], xt[tc][KH + r0:KH + r0 + 16]], axis=1)
        return (xb - wide(mg)) * rt[tc]

    def emit(k, j, v):
        q = [v[:, i * PW:(i + 1) * PW] for i in range(4)]
        if gates:
            q[0] = next(it)(q[0], 0)
            q[3] = next(it)(q[3], 0)
        ops = _sb(*q)
        for i0 in range(0, 7, 2):
            grp = ops[i0:i0 + 2]
            r0 = _ppos(i0 + 1, j)[0] + k * 8
            p_ref[r0:r0 + 8, 0:len(grp) * PW] = pltpu.bitcast(
                cat(grp, axis=1).astype(bf16), u32)

    for k in range(8):
        if main:
            b11 = sub(k, 0, 0)
            emit(k, 2, b11)
            b12 = sub(k, 0, 1)
            emit(k, 6, b11 + b12)
            b22 = sub(k, 1, 1)
            emit(k, 3, b12 - b22)
            emit(k, 1, b11 + b22)
            emit(k, 5, b22)
            b21 = sub(k, 1, 0)
            emit(k, 4, b21 - b11)
            emit(k, 7, b21 + b22)
        if rest and k % 2 == 0:
            mg = m
            if gates:
                mg = cat([next(it)(m[:, 0:W2], 2), next(it)(m[:, W2:], 2)],
                         axis=1)
            r0 = 2 * KH + k * 8
            v = (x[r0:r0 + 16] - cat([mg, mg], axis=0)) * r16
            for c0 in (0, 2):
                r1 = _rpos(c0)[0] + k * 4
                p_ref[r1:r1 + 8, :] = pltpu.bitcast(
                    v[:, c0 * PW:(c0 + 2) * PW].astype(bf16), u32)


def _kernel(x_hbm, g_hbm, b_hbm, w_hbm, o_hbm, xbuf, obuf,
            p0, p1, p2, p3, u0, u1, u2, u3, u4,
            g_ref, b_ref, w_ref, a_ref, ar_ref, zs, sin, sout):
    ps = [p0, p1, p2, p3]
    us = [u0, u1, u2, u3, u4]
    for i in range(4):
        zs[i] = 0

    def cin_last():
        return pltpu.make_async_copy(
            x_hbm.at[S - 1], xbuf.at[S - 1], sin.at[NI - 1])

    def cin_pair(j):
        rows = pl.ds(3 + 2 * jnp.minimum(j, NI - 2), 2)
        return pltpu.make_async_copy(x_hbm.at[rows], xbuf.at[rows], sin.at[j])

    def cin_quad(n):
        t, c = divmod(n, 2)
        return pltpu.make_async_copy(
            x_hbm.at[t, :, c * W4:(c + 1) * W4],
            xbuf.at[t, :, c * W4:(c + 1) * W4], sin.at[NI + 3 + n])

    def cout(sl, r0, r1, ct):
        idx = (sl, slice(r0, r1), slice(ct * PW, (ct + 1) * PW))
        pltpu.make_async_copy(
            obuf.at[idx], o_hbm.at[idx], sout.at[0]).start(priority=ct % 2)

    def cout_quad(t, c):
        for ct in range(4):
            cout(t, 0, D, 4 * c + ct)

    cw = pltpu.make_async_copy(w_hbm, w_ref, sin.at[NI])
    cg = pltpu.make_async_copy(g_hbm, g_ref, sin.at[NI + 1])
    cb = pltpu.make_async_copy(b_hbm, b_ref, sin.at[NI + 2])
    cg.start()
    cb.start()
    cw.start()
    for n in range(NH):
        cin_quad(n).start()
    for j in range(NI - 1):
        pltpu.make_async_copy(x_hbm.at[3 + 2 * j:5 + 2 * j],
                              xbuf.at[3 + 2 * j:5 + 2 * j], sin.at[j]).start()
    cin_last().start()

    row16 = lax.broadcasted_iota(jnp.int32, (16, W2), 0)
    ones = pltpu.bitcast(jnp.where(row16 < 3, 1.0, 0.0).astype(bf16), u32)
    for p_ref in ps:
        for c0 in (0, 2):
            r1 = _rpos(c0)[0] + 32
            p_ref[r1:r1 + 8, :] = ones

    cg.wait()
    cb.wait()
    cw.wait()
    g = g_ref[...].astype(f32).reshape(1, D)
    w = w_ref[...]
    b16 = jnp.broadcast_to(b_ref[...].reshape(1, D), (16, D))
    bias = jnp.dot(b16, w, preferred_element_type=f32)[0:8]
    bh = bias.astype(bf16).astype(f32)
    bl = (bias - bh).astype(bf16).astype(f32)
    bl2 = bias - bh - bl
    row8 = lax.broadcasted_iota(jnp.int32, (8, D), 0)
    ext = jnp.where(row8 == 0, bh,
                    jnp.where(row8 == 1, bl, jnp.where(row8 == 2, bl2, 0.0)))
    wf = w.astype(f32)
    wr = cat([wf[2 * KH:], ext, jnp.zeros((56, D), f32)], axis=0)
    wg = wf[:2 * KH].T * g[:, :2 * KH]
    gr = cat([g[:, 2 * KH:], jnp.ones((1, 64), f32)], axis=1)
    a1 = _sa(wg[0:H, 0:KH], wg[0:H, KH:], wg[H:, 0:KH], wg[H:, KH:])
    for i in range(1, 8):
        top, bot = a1[i - 1][0:Q], a1[i - 1][Q:]
        if i in PERM:
            top, bot = bot, top
        a2 = _sa(top[:, 0:128], top[:, 128:], bot[:, 0:128], bot[:, 128:])
        a_ref[:, (i - 1) * PW:i * PW] = pltpu.bitcast(
            cat(a2, axis=0).astype(bf16), u32)
    arv = (wr.T * gr).astype(bf16)
    ar_ref[:, 0:PW] = pltpu.bitcast(arv[0:H], u32)
    ar_ref[:, PW:] = pltpu.bitcast(arv[H:], u32)

    def masks():
        return {n: lax.broadcasted_iota(
            jnp.int32, (8, n * PW) if n else (16, PW), 0) < zs[1]
                for n in (0, 1, 2)}

    def gate_factory(source):
        never = masks()
        cache = {}

        def event(e, n):
            if (e, n) not in cache:
                if n == 1:
                    cache[e, n] = source[e[0]][e[1]:e[1] + 8]
                else:
                    cache[e, n] = cat([event(e, 1)] * 2, axis=1 if n else 0)
            return cache[e, n]

        def make_gate(e):
            if e is None:
                return lambda v, n: v
            return lambda v, n: lax.select(never[n], event(e, n), v)
        return make_gate

    def rem_operands(p_ref, i, k):
        half, cc = _OUT[i]
        hr = (int(k[0]) - 1) ^ (1 if i in PERM else 0)
        r1, c1 = _rpos(2 * cc + int(k[1]) - 1)
        return (lambda: pltpu.bitcast(
                    ar_ref[hr * 72:(hr + 1) * 72,
                           half * PW:(half + 1) * PW], bf16)[:, :KR],
                lambda: pltpu.bitcast(p_ref[r1:r1 + 40, c1:c1 + PW], bf16))

    cin_quad(0).wait()
    m0, r0 = _stats_quad(xbuf[zs[0], :, 0:W4].astype(f32), [])
    x0 = xbuf[zs[2], :, 0:W4].astype(f32)
    _norm_quad(x0, m0, r0, ps[0], [], main=False)
    early0 = {}
    for i in (4, 7, 5, 6):
        early0[i] = {}
        for k in _TERMS:
            lhs, rhs = rem_operands(ps[0], i, k)
            early0[i][k] = jnp.dot(lhs(), rhs(), preferred_element_type=f32)
    gate0 = gate_factory([early0[i]["11"] for i in (4, 7, 5, 6)])
    _norm_quad(x0, m0, r0, ps[0],
               [gate0(None)] * 19
               + [gate0(divmod(int(u * 72 * 0.99 / 157) * 8, Q))
                  for u in range(157)], rest=False)

    def run(s, fresh, waits, tasks, hooks, early, bubble, valu, vst, ratio):
        k1 = s + zs[0]
        k2 = s + zs[2]
        first = {}
        make_gate = gate_factory(first)
        zero = pl.multiple_of(zs[3], 8)
        nq = 4
        vt, st = (_FIRST_VT, _FIRST_ST) if early else (_VT, _ST)
        nr = len(vt)
        tn = [1] * nr if early else _TWEAK_N
        ts = [1] * nr if early else _TWEAK_S
        free = [max(valu - vt[r], 0) for r in range(nr)]
        wn = [(min(free[r], max(vst - st[r], 0) * ratio) + 0.01) * tn[r]
              for r in range(nr)]
        sc = sum(_NCOST) * nr / 16.25 / sum(wn)
        ws = [(max(free[r] - wn[r] * sc, 0) + 0.01) * ts[r] for r in range(nr)]

        def xload(k, q):
            t, c = divmod(q, 2)
            return xbuf[jnp.minimum(k + t, S - 1), :,
                        c * W4:(c + 1) * W4].astype(f32)

        mr = {}
        todo = list(tasks)

        def flush(now):
            for task in [t for t in todo if t[3] <= now + 1e-9]:
                todo.remove(task)
                kind, q, t0, t1 = task
                wt = wn if kind == "N" else ws
                cand = []
                a = 0.0
                if t0 == 0 or t0 in waits:
                    cand.append((0.0, None))
                    a += bubble[kind]
                for r in range(int(t0), nr):
                    for e in range(NPER):
                        if t0 - 1e-9 <= r + e / NPER < t1 - 1e-9:
                            cand.append((a, (r, Q * e // NPER // 8 * 8)))
                            a += wt[r] / NPER
                costs = _NCOST if kind == "N" else [1] * (D // 4)
                done = 0
                gates = []
                for x in costs:
                    tgt = a * done / sum(costs)
                    gates.append(make_gate(
                        [e for (c, e) in cand if c <= tgt + 1e-9][-1]))
                    done += x
                if kind == "N":
                    _norm_quad(xload(k2, q), *mr.pop(q), ps[q % 4], gates)
                else:
                    mr[q] = _stats_quad(xload(k1, q), gates)

        count = [0]

        def mxu(lhs, rhs):
            r, o = divmod(count[0], 4)
            if o == 0 and r in waits:
                flush(r)
                waits[r]()
            v = jnp.dot(lhs(), rhs(), preferred_element_type=f32)
            if o == 0:
                first[r] = v
            count[0] += 1
            return v

        def get(i):
            return us[i][pl.ds(zero, H), :]

        def get_sub(i, hr, hc):
            return us[i][pl.ds(pl.multiple_of(zero + hr * Q, 8), Q),
                         hc * PW:(hc + 1) * PW]

        def quad(p):
            sl = s + p // 2
            c0 = (p % 2) * W4
            p_ref = ps[p % 4]
            if p in fresh:
                p_ref = p_ref.at[pl.ds(zero, BROWS), :]

            def hook(name):
                if (p, name) in hooks:
                    hooks[(p, name)]()

            def dot(i, j):
                r1, c1 = _ppos(i, j)
                return mxu(
                    lambda: pltpu.bitcast(
                        a_ref[(j - 1) * 72:j * 72, (i - 1) * PW:i * PW], bf16),
                    lambda: pltpu.bitcast(
                        p_ref[r1:r1 + 64, c1:c1 + PW], bf16))

            def rem(i, k):
                return mxu(*rem_operands(p_ref, i, k))

            def prod(i, sep=None, plus=(), minus=()):
                sw = 1 if i in PERM else 0

                def blk(c):
                    rows = [cat([c["11"], c["12"]], axis=1),
                            cat([c["21"], c["22"]], axis=1)]
                    return cat(rows[::-1] if sw else rows, axis=0)

                kind = ("put" if i not in _OUT else
                        "sep" if sep or i in (4, 5) else "merge")
                seq = _ORDER[("early" if sep else kind, count[0] % 4)].split()
                acc = {}
                sign = {}
                sep = dict(sep or {})
                for n, nm in enumerate(seq):
                    if nm[0] == "m":
                        v = dot(i, int(nm[1]))
                    else:
                        v = rem(i, nm[1:])
                        sep[nm[1:]] = v
                    for k, terms in _TERMS.items():
                        sg = terms.get(nm)
                        if kind == "merge" and nm == "r" + k:
                            sg = 1
                        if sg is None:
                            continue
                        if k not in acc:
                            acc[k], sign[k] = v, sg
                        elif sign[k] < 0:
                            acc[k], sign[k] = v - acc[k], 1
                        else:
                            acc[k] = acc[k] + v if sg > 0 else acc[k] - v
                    if plus and n == len(seq) - 5:
                        for k in _TERMS:
                            hr, hc = (int(k[0]) - 1) ^ sw, int(k[1]) - 1
                            for u in plus:
                                acc[k] = acc[k] + get_sub(u, hr, hc)
                            for u in minus:
                                acc[k] = acc[k] - get_sub(u, hr, hc)
                return blk(acc), blk(sep) if kind == "sep" else None

            def out(i, plus, minus=()):
                o = _OUT[i]
                if i == 6 and p == nq - 1:
                    val, v = prod(i, None, plus, minus)
                    plus = minus = ()
                else:
                    val, v = prod(i, done.get(i))
                if i == 6:
                    hook("m6")
                v = val if v is None else val + v
                for u in plus:
                    v = v + get(u)
                for u in minus:
                    v = v - get(u)
                obuf[sl, o[0] * H:(o[0] + 1) * H,
                     c0 + o[1] * W2:c0 + (o[1] + 1) * W2] = v.astype(bf16)
                return val

            done = {}
            if p == 0:
                done = early or {5: {k: rem(5, k) for k in _TERMS}}
            us[0][...] = prod(3)[0]
            hook("m3")
            us[1][...] = out(5, [0])
            us[2][...] = prod(2)[0]
            hook("m2")
            m4 = out(4, [2])
            us[3][...] = m4 - get(1)
            us[4][...] = prod(1)[0]
            hook("m1")
            out(7, [3, 4])
            out(6, [0, 4], [2])

        for p in range(nq):
            flush(-(-count[0] // 4))
            quad(p)
        flush(nr)

    def wait_quads(ns):
        return lambda: [cin_quad(n).wait() for n in ns]

    cin_quad(1).wait()
    run(0, (1, 2, 3), {r: wait_quads(ns) for r, ns in _FIRST_WAITS.items()},
        _FIRST_TASKS, {}, early0, {"N": 293, "S": 396}, 509, 138, 4.92)

    j_flush = (DEFER - 2) // 2

    def write_part(half, cc):
        for k in range(2):
            cout(S - 1, half * H, (half + 1) * H, 4 + 2 * cc + k)

    def body(j, carry):
        s = 2 + 2 * j

        @pl.when(j < NI - 1)
        def _():
            cin_pair(j).wait()

        @pl.when(j == NI - 1)
        def _():
            cin_last().wait()

        def write_prev(p):
            def fn():
                if p == 0:
                    @pl.when(j == j_flush)
                    def _():
                        for ct in range(8):
                            cout(pl.ds(0, DEFER), 0, D, ct)

                @pl.when(j > j_flush if p == 0 else j >= j_flush)
                def _():
                    cout_quad(s + (p - 1) // 2, (p - 1) % 2)
            return fn

        def write_last(half, cc):
            return lambda: pl.when(j == NI - 1)(
                lambda: write_part(half, cc))

        hooks = {(p, "m3"): write_prev(p) for p in range(4)}
        hooks.update({(3, "m2"): write_last(0, 1), (3, "m1"): write_last(1, 0),
                      (3, "m6"): write_last(0, 0)})
        run(s, (2, 3), {}, _LOOP_TASKS, hooks, None, {"N": 0.01, "S": 550},
            441, 121, 5.86)
        return carry

    lax.fori_loop(0, NI, body, 0)
    write_part(1, 1)
    pltpu.make_async_copy(obuf, o_hbm, sout.at[0]).wait()


@jax.jit
def pallas_standalone__layernorm_linear__sampling_kernel(
    x: jax.Array,
    g: jax.Array,
    b: jax.Array,
    w: jax.Array,
):
    assert x.shape == (B, S, D) and w.shape == (D, D)
    xt = jnp.transpose(x, (1, 2, 0))
    out = pl.pallas_call(
        _kernel,
        in_specs=[pl.BlockSpec(memory_space=pl.ANY)] * 4,
        out_specs=pl.BlockSpec(memory_space=pl.ANY),
        out_shape=jax.ShapeDtypeStruct((S, D, B), x.dtype),
        scratch_shapes=[
            pltpu.VMEM((S, D, B), bf16),
            pltpu.VMEM((S, D, B), bf16),
        ] + [pltpu.VMEM((BROWS, W2), u32)] * 4
        + [pltpu.VMEM((H, W2), f32)] * 5
        + [
            pltpu.VMEM((D,), bf16),
            pltpu.VMEM((D,), bf16),
            pltpu.VMEM((D, D), bf16),
            pltpu.VMEM((7 * 72, 7 * PW), u32),
            pltpu.VMEM((144, W2), u32),
            pltpu.SMEM((4,), jnp.int32),
            pltpu.SemaphoreType.DMA((NI + 3 + NH,)),
            pltpu.SemaphoreType.DMA((1,)),
        ],
        compiler_params=pltpu.CompilerParams(
            vmem_limit_bytes=110 * 1024 * 1024,
            disable_bounds_checks=True,
            disable_semaphore_checks=True,
        ),
    )(xt, g, b, w)
    return jnp.transpose(out, (2, 0, 1))
```
